```python
import jax
import jax.numpy as jnp

def _softmax(x, axis=-1):
    return jax.nn.softmax(x, axis=axis)
def _gelu(x):
    return jax.nn.gelu(x, approximate=True)
def _silu(x):
    return jax.nn.silu(x)
def _sigmoid(x):
    return jax.nn.sigmoid(x)
def _layernorm(x, axis=-1, eps=1e-5):
    m = jnp.mean(x, axis=axis, keepdims=True)
    v = jnp.var(x, axis=axis, keepdims=True)
    return (x - m) / jnp.sqrt(v + eps)
def _scatter_add(tgt, idx, src, axis=0):
    return tgt.at[idx].add(src)
def _segment_sum(src, seg, n):
    return jax.ops.segment_sum(src, seg, n)
class _Rng:
    def __init__(self, key):
        self._k = key
    def _next(self):
        self._k, sub = jax.random.split(self._k)
        return sub
    def normal(self, shape):
        return jax.random.normal(self._next(), shape, dtype=jnp.bfloat16)
    def randint(self, lo, hi, shape):
        return jax.random.randint(self._next(), shape, lo, hi, dtype=jnp.int32)
    def uniform(self, shape, lo=0.0, hi=1.0):
        return jax.random.uniform(self._next(), shape, jnp.bfloat16, lo, hi)
    def permutation(self, n):
        return jax.random.permutation(self._next(), n)


kernel_name = 'gated_mix__ssm_conv_h3__sliding_local_dilated__prompt'

def setup_inputs():
    _rng = _Rng(jax.random.key(int.from_bytes(__import__("os").urandom(4), "little")))
    _w = (lambda a: (lambda t: t.astype(jnp.bfloat16) if jnp.issubdtype(t.dtype, jnp.floating) else t)(jnp.asarray(a)))
    def _A_setup():
        B, S, D = 1, 2048, 640
        ks = 4
        return {
            "q": _w((lambda *s: _rng.normal(s) * 0.05)(B, S, D)),
            "k": _w((lambda *s: _rng.normal(s) * 0.05)(B, S, D)),
            "v": _w((lambda *s: _rng.normal(s) * 0.05)(B, S, D)),
            "shift_k": _w((lambda *s: _rng.normal(s) * 0.05)(D, ks) * 0.5),
            "ssm_k": _w((lambda *s: _rng.normal(s) * 0.05)(D, S) * (1.0 / S ** 0.5)),
            "ssm_D": _w((lambda *s: _rng.normal(s) * 0.05)(D)),
        }
    _A_in = _A_setup()

    def _B_setup():
        B, S, D = 1, 2048, 640
        return {
            "x": _w((lambda *s: _rng.normal(s) * 0.05)(B, S, D)),
            "wqkv": _w((lambda *s: _rng.normal(s) * 0.05)(D, 3 * D)),
            "wo": _w((lambda *s: _rng.normal(s) * 0.05)(D, D)),
        }
    _B_in = _B_setup()

    return {
        "A_q": _A_in["q"],
        "A_k": _A_in["k"],
        "A_v": _A_in["v"],
        "A_shift_k": _A_in["shift_k"],
        "A_ssm_k": _A_in["ssm_k"],
        "A_ssm_D": _A_in["ssm_D"],
        "B_x": _B_in["x"],
        "B_wqkv": _B_in["wqkv"],
        "B_wo": _B_in["wo"],
        "gate_w": _w((lambda *s: _rng.normal(s) * 0.05)(640)),
    }

def reference(A_q, A_k, A_v, A_shift_k, A_ssm_k, A_ssm_D, B_x, B_wqkv, B_wo, gate_w):
    def _A_ref(q, k, v, shift_k, ssm_k, ssm_D):
        B, S, D = q.shape
        ks = shift_k.shape[-1]
        k_pad = jnp.pad(k, ((0, 0), (ks - 1, 0), (0, 0)))
        k_shift = jnp.zeros_like(k)
        for t in range(ks):
            k_shift = k_shift + k_pad[:, t:t + S, :] * shift_k[:, ks - 1 - t][None, None, :]
        kv = k_shift * v
        L = 2 * S
        kv_pad = jnp.pad(kv, ((0, 0), (0, S), (0, 0)))
        kf_pad = jnp.pad(ssm_k, ((0, 0), (0, S)))
        kv_f = (lambda x, axes=(-2,-1): jnp.fft.rfft2(x.astype(jnp.float32), axes=axes))(kv_pad[:, None, :, :], axes=(1, 2))
        kf_f = (lambda x, axes=(-2,-1): jnp.fft.rfft2(x.astype(jnp.float32), axes=axes))(kf_pad[:, None, :], axes=(1, 2))
        kf_f = (lambda x, *d: x.transpose(*d))(kf_f, 1, 2, 0)
        y_f = kv_f * kf_f[None, :, :, :]
        y = (lambda x, s, axes=(-2,-1): jnp.fft.irfft2(x, s=s, axes=axes).astype(jnp.bfloat16))(y_f, (1, L), axes=(1, 2))[:, 0, :S, :]
        y = y + kv * ssm_D[None, None, :]
        return q * y

    def _B_ref(x, wqkv, wo):
        B, S, D = x.shape
        H = 32; Dh = D // H
        W, dil = 8, 2
        qkv = (lambda x, *d: x.transpose(*d))((x @ wqkv).reshape(B, S, 3, H, Dh), 2, 0, 3, 1, 4)
        q, k, v = qkv[0], qkv[1], qkv[2]
        scale = Dh ** -0.5
        pos = jnp.arange(S)
        off = jnp.arange(W) * dil
        idx = pos[:, None] - off[None, :]
        mask = idx >= 0
        idx_c = jnp.where(mask, idx, 0).reshape(-1)
        kg = k[:, :, idx_c, :].reshape(B, H, S, W, Dh)
        vg = v[:, :, idx_c, :].reshape(B, H, S, W, Dh)
        logits = jnp.einsum("bhsd,bhswd->bhsw", q, kg) * scale
        logits = jnp.where(mask[None, None, :, :], logits, -1e9)
        attn = _softmax(logits, axis=-1)
        o = jnp.einsum("bhsw,bhswd->bhsd", attn, vg)
        return (lambda x, *d: x.transpose(*d))(o, 0, 2, 1, 3).reshape(B, S, D) @ wo

    x = A_q
    g = _sigmoid((x * gate_w).sum(-1, keepdims=True))
    a = _A_ref(x, A_k, A_v, A_shift_k, A_ssm_k, A_ssm_D)
    b = _B_ref(x, B_wqkv, B_wo)
    return g * a + (1 - g) * b
```

```python
import numpy as np
import jax
import jax.numpy as jnp
import jax.experimental.pallas as pl
import jax.experimental.pallas.tpu as pltpu

S, D = 2048, 640
H, DH = 32, 20
WIN, DIL = 8, 2
KS = 4
LT = D // 128
BLK = 256
NB = S // BLK
HALO = 16
SQRT2 = float(np.sqrt(2.0))
F32, BF16 = jnp.float32, jnp.bfloat16


def _dft_matrices():
    n = np.arange(128)[None, :]
    m = np.arange(64)[:, None]
    fwd, inv = [], []
    for f in (4 * m, 4 * m + 2, 8 * m + 1, 8 * m + 3):
        ang = 2.0 * np.pi * ((f * n) % 512) / 512.0
        a = np.concatenate([np.cos(ang), -np.sin(ang)], axis=0)
        wgt = np.full((128, 1), 2.0 / 512.0)
        if not fwd:
            a[64] = np.cos(np.pi * n[0])
            wgt[0] = wgt[64] = 1.0 / 512.0
        fwd.append(a)
        inv.append((a * wgt).T)
    return np.stack(fwd + inv).astype(np.float32)


_DFT = _dft_matrices()


def _nt(a, b):
    return jax.lax.dot_general(a, b, (((1,), (1,)), ((), ())),
                               preferred_element_type=F32)


def _kernel(x_hbm, k_hbm, v_hbm, h_hbm, w_hbm, wo_hbm,
            shift_ref, dvec_ref, gate_ref, dft_ref,
            out_hbm,
            x_v, k_v, v_v, h_v, w_v, wo_v,
            tmp_s, wp_s, wop_s, q_s, ka_s, va_s, kf_s, o_s, gq_s, u_s, g_s,
            y_s, out_s, sems, out_sems):
    copies = [
        pltpu.make_async_copy(src, dst, sems.at[n])
        for n, (src, dst) in enumerate((
            (w_hbm, w_v), (x_hbm, x_v), (k_hbm, k_v), (v_hbm, v_v),
            (wo_hbm, wo_v), (h_hbm, h_v)))
    ]
    cp_w, cp_x, cp_k, cp_v, cp_wo, cp_h = copies
    cp_w.start()
    cp_x.start()

    cp_w.wait()
    for c in (cp_k, cp_v, cp_wo, cp_h):
        c.start()

    def permute_w(kt, carry):
        r0 = pl.multiple_of(kt * 128, 128)
        for ct in range(3 * LT):
            t = w_v[pl.ds(r0, 128), ct * 128:(ct + 1) * 128].astype(F32)
            tmp_s[ct * 128:(ct + 1) * 128, :] = t.T
        for p in range(3):
            for d in range(DH):
                rows = tmp_s[pl.ds(p * D + d, H, stride=DH), :]
                wp_s[kt, p * D + d * H:p * D + (d + 1) * H, :] = rows.astype(BF16)
        return carry

    jax.lax.fori_loop(0, LT, permute_w, 0)

    zeros = jnp.zeros((HALO, 128), F32)
    for t in range(LT):
        ka_s[t, 0:HALO, :] = zeros
        va_s[t, 0:HALO, :] = zeros
        kf_s[t, 0:8, :] = zeros[0:8]

    cp_x.wait()
    cp_k.wait()
    cp_v.wait()

    shift = shift_ref[...].astype(F32)
    gate = gate_ref[...].astype(F32)
    qscale = float(DH ** -0.5 * np.log2(np.e))

    def project(i):
        r0 = pl.multiple_of(i * BLK, BLK)
        xb = x_v[pl.ds(r0, BLK), :]
        for ct in range(3 * LT):
            acc = None
            for kt in range(LT):
                part = _nt(xb[:, kt * 128:(kt + 1) * 128],
                           wp_s[kt, ct * 128:(ct + 1) * 128, :])
                acc = part if acc is None else acc + part
            p, t = divmod(ct, LT)
            if p == 0:
                q_s[t] = acc * qscale
            elif p == 1:
                ka_s[t, pl.ds(r0 + HALO, BLK), :] = acc
            else:
                va_s[t, pl.ds(r0 + HALO, BLK), :] = acc

    def attend(i):
        r0 = pl.multiple_of(i * BLK, BLK)
        rc = 16
        for c in range(BLK // rc):
            row = c * rc
            xs = [x_v[pl.ds(r0 + row, rc), t * 128:(t + 1) * 128].astype(F32)
                  for t in range(LT)]
            z = xs[0] * gate[:, 0:128]
            for t in range(1, LT):
                z = z + xs[t] * gate[:, t * 128:(t + 1) * 128]
            g = jax.nn.sigmoid(jnp.sum(z, axis=-1, keepdims=True))
            for t in range(LT):
                gq_s[t, pl.ds(r0 + row, rc), :] = xs[t] * g
            qs = [q_s[t, row:row + rc, :] for t in range(LT)]
            logits = []
            for w in range(WIN):
                a = None
                for t in range(LT):
                    kk = ka_s[t, pl.ds(r0 + (row + HALO - DIL * w), rc), :]
                    a = qs[t] * kk if a is None else a + qs[t] * kk
                a = a + pltpu.roll(a, 64, 1)
                a = a + pltpu.roll(a, 32, 1)
                if row < DIL * w:
                    pos = r0 + row + jax.lax.broadcasted_iota(jnp.int32, (rc, 128), 0)
                    a = jnp.where(pos >= DIL * w, a, -1e9)
                logits.append(a)
            m = logits[0]
            for w in range(1, WIN):
                m = jnp.maximum(m, logits[w])
            es = [jnp.exp2(a - m) for a in logits]
            den = es[0]
            for w in range(1, WIN):
                den = den + es[w]
            norm = (1.0 - g) / den
            for t in range(LT):
                a = None
                for w in range(WIN):
                    vv = va_s[t, pl.ds(r0 + (row + HALO - DIL * w), rc), :]
                    a = es[w] * vv if a is None else a + es[w] * vv
                o_s[pl.ds(r0 + row, rc), t * 128:(t + 1) * 128] = (a * norm).astype(BF16)

    def conv_forward(i):
        r0 = pl.multiple_of(i * BLK, BLK)
        for t in range(LT):
            lanes = slice(t * 128, (t + 1) * 128)
            kf_s[t, pl.ds(r0 + 8, BLK), :] = k_v[pl.ds(r0, BLK), lanes].astype(F32)
            xs = []
            for b in range(4):
                ks = None
                for j in range(KS):
                    kk = kf_s[t, pl.ds(r0 + (8 + 64 * b - j), 64), :]
                    term = kk * shift[j:j + 1, lanes]
                    ks = term if ks is None else ks + term
                xs.append(ks * v_v[pl.ds(r0 + 64 * b, 64), lanes].astype(F32))
            x0, x1, x2, x3 = xs
            t0, t1 = x0 - x2, x1 + x3
            w0, w1 = SQRT2 * x3, SQRT2 * x2
            res = ((x0 + x2, t1), (t0, x1 - x3), (t0 - w0, t1 + w1), (t0 + w0, t1 - w1))
            for cl in range(4):
                r = jnp.concatenate(res[cl], axis=0).astype(BF16)
                u_s[t, i, cl] = jnp.dot(dft_ref[cl], r, preferred_element_type=F32)

    def phase1(i, carry):
        project(i)
        conv_forward(i)
        attend(i)
        return carry

    jax.lax.fori_loop(0, NB, phase1, 0)

    cp_wo.wait()
    for t in range(LT):
        tmp_s[0:D, :] = wo_v[:, t * 128:(t + 1) * 128].astype(F32)
        for d in range(DH):
            rows = tmp_s[pl.ds(d, H, stride=DH), :]
            wop_s[t, d * H:(d + 1) * H, :] = rows.astype(BF16)
    cp_h.wait()

    lane = jax.lax.broadcasted_iota(jnp.int32, (128, 128), 1)
    sign = jnp.where(lane < 64, -1.0, 1.0).astype(F32)
    slot0 = jax.lax.broadcasted_iota(jnp.int32, (16, 128), 0) == 0

    def out_copy(j):
        return pltpu.make_async_copy(
            out_s.at[j], out_hbm.at[:, pl.ds(pl.multiple_of(j * 128, 128), 128)],
            out_sems.at[j])

    def phase2(j, carry):
        c0 = pl.multiple_of(j * 128, 128)
        prev = None
        for a in range(NB):
            lo = h_v[pl.ds(c0, 128), a * BLK:a * BLK + 128].astype(F32)
            hi = h_v[pl.ds(c0, 128), a * BLK + 128:(a + 1) * BLK].astype(F32)
            if a == 0:
                lo = lo + jnp.where(lane == 0, dvec_ref[pl.ds(c0, 128), :].astype(F32), 0.0)
                elo, ehi, olo, ohi = lo, hi, lo, hi
            else:
                elo, ehi = lo + prev[0], hi + prev[1]
                olo, ohi = lo - prev[0], hi - prev[1]
            prev = (lo, hi)
            tt = olo + sign * ohi
            ww = (SQRT2 * sign) * pltpu.roll(ohi, 64, 1)
            res = (elo + ehi, elo - ehi, tt + ww, tt - ww)
            for cl in range(4):
                g_s[a, cl] = _nt(dft_ref[cl], res[cl].astype(BF16))

        for m in range(NB):
            for cl in range(4):
                for r in range(4):
                    re = slice(16 * r, 16 * r + 16)
                    im = slice(64 + 16 * r, 64 + 16 * r + 16)
                    yr = yi = None
                    for a in range(m + 1):
                        gr, gi = g_s[a, cl, re, :], g_s[a, cl, im, :]
                        ur, ui = u_s[j, m - a, cl, re, :], u_s[j, m - a, cl, im, :]
                        if cl == 0 and r == 0:
                            ga = jnp.where(slot0, 0.0, gi)
                            gb = jnp.where(slot0, gi, gr)
                        else:
                            ga, gb = gi, gr
                        pr = ur * gr - ui * ga
                        pi = ur * ga + ui * gb
                        yr = pr if yr is None else yr + pr
                        yi = pi if yi is None else yi + pi
                    y_s[m, cl, re, :] = yr.astype(BF16)
                    y_s[m, cl, im, :] = yi.astype(BF16)
            rho = [jnp.dot(dft_ref[4 + cl], y_s[m, cl], preferred_element_type=F32)
                   for cl in range(4)]
            (a0, a1), (b0, b1), (p0, p1), (n0, n1) = [(z[:64], z[64:]) for z in rho]
            s0, s1, d0, d1 = p0 + n0, p1 + n1, p0 - n0, p1 - n1
            ys = (a0 + b0 + s0, a1 + b1 + s1,
                  a0 - b0 - s0 + SQRT2 * d1, a1 - b1 + s1 - SQRT2 * d0)
            bb = jnp.dot(o_s[m * BLK:(m + 1) * BLK, :], wop_s[j],
                         preferred_element_type=F32)
            for b in range(4):
                rows = slice(m * BLK + 64 * b, m * BLK + 64 * (b + 1))
                res = gq_s[j, rows, :] * ys[b] + bb[64 * b:64 * (b + 1)]
                out_s[j, rows, :] = res.astype(BF16)
        out_copy(j).start()
        return carry

    jax.lax.fori_loop(0, LT, phase2, 0)
    for j in range(LT):
        out_copy(j).wait()


@jax.jit
def pallas_gated_mix__ssm_conv_h3__sliding_local_dilated__prompt_kernel(
    A_q: jax.Array,
    A_k: jax.Array,
    A_v: jax.Array,
    A_shift_k: jax.Array,
    A_ssm_k: jax.Array,
    A_ssm_D: jax.Array,
    B_x: jax.Array,
    B_wqkv: jax.Array,
    B_wo: jax.Array,
    gate_w: jax.Array,
):
    del B_x
    hbm = pl.BlockSpec(memory_space=pl.ANY)
    vmem = pl.BlockSpec(memory_space=pltpu.VMEM)
    out = pl.pallas_call(
        _kernel,
        out_shape=jax.ShapeDtypeStruct((S, D), BF16),
        in_specs=[hbm] * 6 + [vmem] * 4,
        out_specs=hbm,
        scratch_shapes=[
            pltpu.VMEM((S, D), BF16),
            pltpu.VMEM((S, D), BF16),
            pltpu.VMEM((S, D), BF16),
            pltpu.VMEM((D, S), BF16),
            pltpu.VMEM((D, 3 * D), BF16),
            pltpu.VMEM((D, D), BF16),
            pltpu.VMEM((3 * D, 128), F32),
            pltpu.VMEM((LT, 3 * D, 128), BF16),
            pltpu.VMEM((LT, D, 128), BF16),
            pltpu.VMEM((LT, BLK, 128), F32),
            pltpu.VMEM((LT, HALO + S, 128), F32),
            pltpu.VMEM((LT, HALO + S, 128), F32),
            pltpu.VMEM((LT, 8 + S, 128), F32),
            pltpu.VMEM((S, D), BF16),
            pltpu.VMEM((LT, S, 128), F32),
            pltpu.VMEM((LT, NB, 4, 128, 128), F32),
            pltpu.VMEM((NB, 4, 128, 128), F32),
            pltpu.VMEM((NB, 4, 128, 128), BF16),
            pltpu.VMEM((LT, S, 128), BF16),
            pltpu.SemaphoreType.DMA((6,)),
            pltpu.SemaphoreType.DMA((LT,)),
        ],
        compiler_params=pltpu.CompilerParams(vmem_limit_bytes=100 * 2**20),
    )(A_q.reshape(S, D), A_k.reshape(S, D), A_v.reshape(S, D), A_ssm_k, B_wqkv, B_wo,
      A_shift_k.T, A_ssm_D.reshape(D, 1), gate_w.reshape(1, D),
      jnp.asarray(_DFT, BF16))
    return out.reshape(1, S, D)
```

```python
import functools

import numpy as np
import jax
import jax.numpy as jnp
import jax.experimental.pallas as pl
import jax.experimental.pallas.tpu as pltpu

S, D = 2048, 640
H, DH = 32, 20
WIN, DIL = 8, 2
KS = 4
LT = D // 128
BLK = 256
NB = S // BLK
HALO = 16
SQRT2 = float(np.sqrt(2.0))
F32, BF16, U32 = jnp.float32, jnp.bfloat16, jnp.uint32


def _dft_matrices():
    n = np.arange(128)[None, :]
    m = np.arange(64)[:, None]
    order = np.arange(128).reshape(2, 8, 8).transpose(1, 0, 2).reshape(-1)
    fwd, inv = [], []
    for f in (4 * m, 4 * m + 2, 8 * m + 1, 8 * m + 3):
        ang = 2.0 * np.pi * ((f * n) % 512) / 512.0
        a = np.concatenate([np.cos(ang), -np.sin(ang)], axis=0)
        wgt = np.full((128, 1), 2.0 / 512.0)
        if not fwd:
            a[64] = np.cos(np.pi * n[0])
            wgt[0] = wgt[64] = 1.0 / 512.0
        fwd.append(a[order])
        inv.append((a * wgt)[order].T)
    lane = np.arange(128)
    same_head = (lane[:, None] % H == lane[None, :] % H)
    return np.stack(fwd + inv + [same_head]).astype(np.float32)


_DFT = _dft_matrices()


def _nt(a, b):
    return jax.lax.dot_general(a, b, (((1,), (1,)), ((), ())),
                               preferred_element_type=F32)


def _nn(a, b):
    return jnp.dot(a, b, preferred_element_type=F32)


def _pack(x):
    return pltpu.bitcast(x.astype(BF16), U32)


def _unpack(x):
    return pltpu.bitcast(x, BF16)


def _interleave(*streams):
    items = []
    for s in streams:
        items += [((n + 0.5) / len(s), f) for n, f in enumerate(s)]
    for _, f in sorted(items, key=lambda e: e[0]):
        f()


def _kernel(x_hbm, k_hbm, v_hbm, h_hbm, w_hbm, wo_hbm,
            shift_ref, dvec_ref, gate_ref, dft_ref,
            out_hbm,
            x_v, k_v, v_v, h_v, w_v, wo_v,
            tmp_s, wp_s, wop_s, dft_s, d_s, xp_s, q0_s, q1_s, k0_s, k1_s, v0_s, v1_s,
            kf_s, pp_s, lg_s, o_s, gq_s, u_s, g_s, y_s, rho_s, out_s,
            w_sem, x_sem, k_sem, v_sem, h_sem, wo_sem, out_sem):
    def rows_copy(src, dst, sem, n, size):
        rows = pl.ds(n * size, size)
        return pltpu.make_async_copy(src.at[rows], dst.at[rows], sem.at[n])

    cp_w = [rows_copy(w_hbm, w_v, w_sem, n, 128) for n in range(LT)]
    cp_x = [rows_copy(x_hbm, x_v, x_sem, n, BLK) for n in range(NB)]
    cp_k = [rows_copy(k_hbm, k_v, k_sem, n, BLK) for n in range(NB)]
    cp_v = [rows_copy(v_hbm, v_v, v_sem, n, BLK) for n in range(NB)]
    cp_h = pltpu.make_async_copy(h_hbm, h_v, h_sem.at[0])
    cp_wo = pltpu.make_async_copy(wo_hbm, wo_v, wo_sem.at[0])

    for c in cp_w + [cp_x[0], cp_k[0], cp_v[0]]:
        c.start()

    qkv_s = ((q0_s, k0_s, v0_s), (q1_s, k1_s, v1_s))
    zeros = jnp.zeros((HALO, 128), F32)
    for t in range(LT):
        k0_s[t, 0:HALO, :] = zeros
        v0_s[t, 0:HALO, :] = zeros
        kf_s[t, 0:8, :] = zeros[0:8]
    for n in range(9):
        dft_s[n] = pltpu.bitcast(dft_ref[n], U32)
    shift = shift_ref[...].astype(F32)
    gate = gate_ref[...].astype(F32).reshape(1, D)
    dvec = dvec_ref[...].astype(F32).reshape(1, D)
    for t in range(LT):
        d_s[t] = jnp.broadcast_to(dvec[:, t * 128:(t + 1) * 128], (8, 128))
    qscale = float(DH ** -0.5 * np.log2(np.e))

    for kt in range(LT):
        cp_w[kt].wait()
        if kt == LT - 1:
            for n in range(1, NB):
                for c in (cp_x[n], cp_k[n], cp_v[n]):
                    c.start()
            cp_wo.start()
            cp_h.start()
        for ct in range(3 * LT):
            t = w_v[kt * 128:(kt + 1) * 128, ct * 128:(ct + 1) * 128].astype(F32)
            tmp_s[ct * 128:(ct + 1) * 128, :] = t.T
        for p in range(3):
            for d in range(DH):
                rows = tmp_s[pl.ds(p * D + d, H, stride=DH), :]
                ct, r = divmod(p * D + d * H, 128)
                wp_s[ct, r // 2:(r + H) // 2, kt * 128:(kt + 1) * 128] = _pack(rows)

    def permute_wo(t):
        tmp_s[0:D, :] = wo_v[:, t * 128:(t + 1) * 128].astype(F32)
        for d in range(DH):
            rows = tmp_s[pl.ds(d, H, stride=DH), :]
            wop_s[t, d * H // 2:(d + 1) * H // 2, :] = _pack(rows)

    def project_items(i):
        q_s, ka_s, va_s = qkv_s[i % 2]

        def stage():
            xp_s[...] = pltpu.bitcast(x_v[i * BLK:(i + 1) * BLK, :], U32)

        def tile(ct):
            acc = _nt(_unpack(xp_s[...]), _unpack(wp_s[ct]))
            p, t = divmod(ct, LT)
            if p == 0:
                q_s[t] = acc * qscale
            else:
                (ka_s, va_s)[p - 1][t, HALO:HALO + BLK, :] = acc

        return [stage] + [functools.partial(tile, ct) for ct in range(3 * LT)]

    def halo_copy(i):
        for src, dst in zip(qkv_s[i % 2][1:], qkv_s[(i + 1) % 2][1:]):
            for t in range(LT):
                dst[t, 0:HALO, :] = src[t, BLK:BLK + HALO, :]

    def attend_items(i):
        q_s, ka_s, va_s = qkv_s[i % 2]
        rc = 16

        part = 64

        def scores(row):
            for sub in range(row, row + part, rc):
                qs = [q_s[t, sub:sub + rc, :] for t in range(LT)]
                for w in range(WIN):
                    lo = sub + HALO - DIL * w
                    a = qs[0] * ka_s[0, lo:lo + rc, :]
                    for t in range(1, LT):
                        a = a + qs[t] * ka_s[t, lo:lo + rc, :]
                    pp_s[row // part, (w * part + sub - row) // 2:
                         (w * part + sub - row + rc) // 2, :] = _pack(a)
            tot = _nn(_unpack(pp_s[row // part]), _unpack(dft_s[8]))
            for w in range(WIN):
                lg_s[w, row:row + part, :] = tot[w * part:(w + 1) * part]

        def chunk(row):
            r0 = i * BLK + row
            xs = [x_v[r0:r0 + rc, t * 128:(t + 1) * 128].astype(F32) for t in range(LT)]
            z = xs[0] * gate[:, 0:128]
            for t in range(1, LT):
                z = z + xs[t] * gate[:, t * 128:(t + 1) * 128]
            th = 0.5 * jnp.tanh(0.5 * jnp.sum(z, axis=-1, keepdims=True))
            g = 0.5 + th
            for t in range(LT):
                gq_s[t, r0:r0 + rc, :] = xs[t] * g
            logits = []
            for w in range(WIN):
                a = lg_s[w, row:row + rc, :]
                if r0 < DIL * w:
                    pos = r0 + jax.lax.broadcasted_iota(jnp.int32, (rc, 128), 0)
                    a = jnp.where(pos >= DIL * w, a, -1e9)
                logits.append(a)
            m = logits[0]
            for w in range(1, WIN):
                m = jnp.maximum(m, logits[w])
            es = [jnp.exp2(a - m) for a in logits]
            den = es[0]
            for w in range(1, WIN):
                den = den + es[w]
            inv = pl.reciprocal(den, approx=True)
            inv = inv * (2.0 - den * inv)
            norm = (0.5 - th) * inv
            for t in range(LT):
                a = None
                for w in range(WIN):
                    lo = row + HALO - DIL * w
                    term = es[w] * va_s[t, lo:lo + rc, :]
                    a = term if a is None else a + term
                o_s[r0 // 2:(r0 + rc) // 2, t * 128:(t + 1) * 128] = _pack(a * norm)

        items = []
        for row in range(0, BLK + part, part):
            if row < BLK:
                items.append(functools.partial(scores, row))
            if row > 0:
                items += [functools.partial(chunk, r) for r in range(row - part, row, rc)]
        return items

    def conv_forward_items(i):
        r0 = i * BLK

        def tile(t):
            lanes = slice(t * 128, (t + 1) * 128)
            kf_s[t, r0 + 8:r0 + 8 + BLK, :] = k_v[r0:r0 + BLK, lanes].astype(F32)
            xs = []
            for b in range(4):
                ks = None
                for j in range(KS):
                    lo = r0 + 8 + 64 * b - j
                    term = kf_s[t, lo:lo + 64, :] * shift[j:j + 1, lanes]
                    ks = term if ks is None else ks + term
                xs.append(ks * v_v[r0 + 64 * b:r0 + 64 * (b + 1), lanes].astype(F32))
            x0, x1, x2, x3 = xs
            t0, t1 = x0 - x2, x1 + x3
            w0, w1 = SQRT2 * x3, SQRT2 * x2
            res = ((x0 + x2, t1), (t0, x1 - x3), (t0 - w0, t1 + w1), (t0 + w0, t1 - w1))
            for cl in range(4):
                r = jnp.concatenate(res[cl], axis=0).astype(BF16)
                u_s[t, i, cl] = _nn(_unpack(dft_s[cl]), r)

        return [functools.partial(tile, t) for t in range(LT)]

    for i in range(NB + 1):
        streams = []
        if i < NB:
            cp_x[i].wait()
            cp_k[i].wait()
            cp_v[i].wait()
            streams += [project_items(i), conv_forward_items(i)]
        else:
            cp_wo.wait()
            streams.append([functools.partial(permute_wo, t) for t in range(LT)])
        if i > 0:
            streams.append(attend_items(i - 1))
        _interleave(*streams)
        if i + 1 < NB:
            halo_copy(i)
    cp_h.wait()

    def out_copy(j):
        return pltpu.make_async_copy(
            out_s.at[j], out_hbm.at[:, pl.ds(pl.multiple_of(j * 128, 128), 128)],
            out_sem.at[j])

    def phase2(j, carry):
        c0 = pl.multiple_of(j * 128, 128)
        lane = jax.lax.broadcasted_iota(jnp.int32, (128, 128), 1)
        sign = jnp.where(lane < 64, -1.0, 1.0).astype(F32)
        slot0 = jax.lax.broadcasted_iota(jnp.int32, (8, 128), 0) == 0

        def filter_block(a):
            def half(n):
                return h_v[pl.ds(c0, 128), n * 128:(n + 1) * 128].astype(F32)
            lo, hi = half(2 * a), half(2 * a + 1)
            if a == 0:
                elo, ehi, olo, ohi = lo, hi, lo, hi
            else:
                plo, phi = half(2 * a - 2), half(2 * a - 1)
                elo, ehi, olo, ohi = lo + plo, hi + phi, lo - plo, hi - phi
            tt = olo + sign * ohi
            ww = (SQRT2 * sign) * pltpu.roll(ohi, 64, 1)
            res = (elo + ehi, elo - ehi, tt + ww, tt - ww)
            for cl in range(4):
                g_s[a, cl] = _nt(_unpack(dft_s[cl]), res[cl].astype(BF16))

        def pointwise(cl, r):
            re, im = slice(16 * r, 16 * r + 8), slice(16 * r + 8, 16 * r + 16)
            special = cl == 0 and r == 0
            dd = d_s[j]
            gs = []
            for a in range(NB):
                gr, gi = g_s[a, cl, re, :], g_s[a, cl, im, :]
                if a < 2:
                    sd = dd if (a == 0 or cl < 2) else -dd
                    gr = gr + sd
                    if special:
                        gi = gi + jnp.where(slot0, sd, 0.0)
                if special:
                    gs.append((gr, jnp.where(slot0, 0.0, gi), jnp.where(slot0, gi, gr)))
                else:
                    gs.append((gr, gi, gr))
            us = [(u_s[j, a, cl, re, :], u_s[j, a, cl, im, :]) for a in range(NB)]
            for m in range(NB):
                yr = yi = None
                for a in range(m + 1):
                    (gr, ga, gb), (ur, ui) = gs[a], us[m - a]
                    pr = ur * gr - ui * ga
                    pi = ur * ga + ui * gb
                    yr = pr if yr is None else yr + pr
                    yi = pi if yi is None else yi + pi
                y_s[m, cl, 8 * r:8 * r + 8, :] = _pack(jnp.concatenate([yr, yi], axis=0))

        def inverse(cl, m):
            rho_s[m, cl] = _nn(_unpack(dft_s[4 + cl]), _unpack(y_s[m, cl]))

        def finish(m):
            bb = _nn(_unpack(o_s[m * BLK // 2:(m + 1) * BLK // 2, :]), _unpack(wop_s[j]))
            (a0, a1), (b0, b1), (p0, p1), (n0, n1) = [
                (rho_s[m, cl, 0:64, :], rho_s[m, cl, 64:128, :]) for cl in range(4)]
            s0, s1, d0, d1 = p0 + n0, p1 + n1, p0 - n0, p1 - n1
            ys = (a0 + b0 + s0, a1 + b1 + s1,
                  a0 - b0 - s0 + SQRT2 * d1, a1 - b1 + s1 - SQRT2 * d0)
            for b in range(4):
                lo = m * BLK + 64 * b
                res = gq_s[j, lo:lo + 64, :] * ys[b] + bb[64 * b:64 * (b + 1)]
                out_s[j, lo:lo + 64, :] = res.astype(BF16)

        for a in range(NB):
            filter_block(a)
        for cl in range(4):
            streams = [[functools.partial(pointwise, cl, r) for r in range(8)]]
            if cl > 0:
                streams.append([functools.partial(inverse, cl - 1, m) for m in range(NB)])
            _interleave(*streams)
        for m in range(NB):
            inverse(3, m)
        for m in range(NB):
            finish(m)
        out_copy(j).start()
        return carry

    jax.lax.fori_loop(0, LT, phase2, 0)
    for j in range(LT):
        out_copy(j).wait()


@jax.jit
def pallas_gated_mix__ssm_conv_h3__sliding_local_dilated__prompt_kernel(
    A_q: jax.Array,
    A_k: jax.Array,
    A_v: jax.Array,
    A_shift_k: jax.Array,
    A_ssm_k: jax.Array,
    A_ssm_D: jax.Array,
    B_x: jax.Array,
    B_wqkv: jax.Array,
    B_wo: jax.Array,
    gate_w: jax.Array,
):
    del B_x
    hbm = pl.BlockSpec(memory_space=pl.ANY)
    vmem = pl.BlockSpec(memory_space=pltpu.VMEM)
    qkv = [pltpu.VMEM((LT, BLK, 128), F32)] * 2 + [pltpu.VMEM((LT, HALO + BLK, 128), F32)] * 4
    out = pl.pallas_call(
        _kernel,
        out_shape=jax.ShapeDtypeStruct((S, D), BF16),
        in_specs=[hbm] * 6 + [vmem] * 4,
        out_specs=hbm,
        scratch_shapes=[
            pltpu.VMEM((S, D), BF16),
            pltpu.VMEM((S, D), BF16),
            pltpu.VMEM((S, D), BF16),
            pltpu.VMEM((D, S), BF16),
            pltpu.VMEM((D, 3 * D), BF16),
            pltpu.VMEM((D, D), BF16),
            pltpu.VMEM((3 * D, 128), F32),
            pltpu.VMEM((3 * LT, 64, D), U32),
            pltpu.VMEM((LT, D // 2, 128), U32),
            pltpu.VMEM((9, 64, 128), U32),
            pltpu.VMEM((LT, 8, 128), F32),
            pltpu.VMEM((BLK // 2, D), U32),
            *qkv,
            pltpu.VMEM((LT, 8 + S, 128), F32),
            pltpu.VMEM((4, WIN * 32, 128), U32),
            pltpu.VMEM((WIN, BLK, 128), F32),
            pltpu.VMEM((S // 2, D), U32),
            pltpu.VMEM((LT, S, 128), F32),
            pltpu.VMEM((LT, NB, 4, 128, 128), F32),
            pltpu.VMEM((NB, 4, 128, 128), F32),
            pltpu.VMEM((NB, 4, 64, 128), U32),
            pltpu.VMEM((NB, 4, 128, 128), F32),
            pltpu.VMEM((LT, S, 128), BF16),
            pltpu.SemaphoreType.DMA((LT,)),
            pltpu.SemaphoreType.DMA((NB,)),
            pltpu.SemaphoreType.DMA((NB,)),
            pltpu.SemaphoreType.DMA((NB,)),
            pltpu.SemaphoreType.DMA((1,)),
            pltpu.SemaphoreType.DMA((1,)),
            pltpu.SemaphoreType.DMA((LT,)),
        ],
        compiler_params=pltpu.CompilerParams(vmem_limit_bytes=100 * 2**20),
    )(A_q.reshape(S, D), A_k.reshape(S, D), A_v.reshape(S, D), A_ssm_k, B_wqkv, B_wo,
      A_shift_k.T, A_ssm_D, gate_w, jnp.asarray(_DFT, BF16))
    return out.reshape(1, S, D)
```

```python
import functools

import numpy as np
import jax
import jax.numpy as jnp
import jax.experimental.pallas as pl
import jax.experimental.pallas.tpu as pltpu

S, D = 2048, 640
H, DH = 32, 20
WIN, DIL = 8, 2
KS = 4
LT = D // 128
BLK = 256
NB = S // BLK
HALO = 16
SQRT2 = float(np.sqrt(2.0))
F32, BF16, U32 = jnp.float32, jnp.bfloat16, jnp.uint32


def _dft_matrices():
    n = np.arange(128)[None, :]
    m = np.arange(64)[:, None]
    order = np.arange(128).reshape(2, 8, 8).transpose(1, 0, 2).reshape(-1)
    fwd, inv = [], []
    for f in (4 * m, 4 * m + 2, 8 * m + 1, 8 * m + 3):
        ang = 2.0 * np.pi * ((f * n) % 512) / 512.0
        a = np.concatenate([np.cos(ang), -np.sin(ang)], axis=0)
        wgt = np.full((128, 1), 2.0 / 512.0)
        if not fwd:
            a[64] = np.cos(np.pi * n[0])
            wgt[0] = wgt[64] = 1.0 / 512.0
        fwd.append(a[order])
        inv.append((a * wgt)[order].T)
    lane = np.arange(128)
    same_head = (lane[:, None] % H == lane[None, :] % H)
    return np.stack(fwd + inv + [same_head]).astype(np.float32)


_DFT = _dft_matrices()


def _nt(a, b):
    return jax.lax.dot_general(a, b, (((1,), (1,)), ((), ())),
                               preferred_element_type=F32)


def _nn(a, b):
    return jnp.dot(a, b, preferred_element_type=F32)


def _pack(x):
    return pltpu.bitcast(x.astype(BF16), U32)


def _unpack(x):
    return pltpu.bitcast(x, BF16)


def _interleave(*streams):
    items = []
    for s in streams:
        total, done = sum(c for c, _ in s), 0.0
        for c, f in s:
            items.append(((done + 0.5 * c) / total, f))
            done += c
    for _, f in sorted(items, key=lambda e: e[0]):
        f()


def _kernel(x_hbm, k_hbm, v_hbm, h_hbm, w_hbm, wo_hbm,
            shift_ref, dvec_ref, gate_ref, dft_ref,
            out_hbm,
            x_v, k_v, v_v, h_v, w_v, wo_v,
            tmp_s, wp_s, wop_s, dft_s, xp_s, q0_s, q1_s, k0_s, k1_s, v0_s, v1_s,
            kf_s, pp_s, lg_s, o0_s, o1_s, gq_s, u_s, g_s, y_s, out_s,
            w_sem, x_sem, k_sem, v_sem, h_sem, wo_sem, out_sem):
    part_fn = functools.partial

    def rows_copy(src, dst, sem, n):
        rows = pl.ds(n * BLK, BLK)
        return pltpu.make_async_copy(src.at[rows], dst.at[rows], sem.at[n])

    def cols_copy(src, dst, sem, n, size):
        cols = pl.ds(n * size, size)
        return pltpu.make_async_copy(src.at[:, cols], dst.at[:, cols], sem.at[n])

    cp_w = [cols_copy(w_hbm, w_v, w_sem, n, D) for n in range(3)]
    cp_x = [rows_copy(x_hbm, x_v, x_sem, n) for n in range(NB)]
    cp_k = [rows_copy(k_hbm, k_v, k_sem, n) for n in range(NB)]
    cp_v = [rows_copy(v_hbm, v_v, v_sem, n) for n in range(NB)]
    cp_h = [cols_copy(h_hbm, h_v, h_sem, n, BLK) for n in range(NB)]
    cp_wo = pltpu.make_async_copy(wo_hbm, wo_v, wo_sem.at[0])
    cp_out = [rows_copy(out_s, out_hbm, out_sem, n) for n in range(NB)]

    cp_w[0].start()
    cp_x[0].start()

    qkv_s = ((q0_s, k0_s, v0_s), (q1_s, k1_s, v1_s))
    o_s = (o0_s, o1_s)
    zeros = jnp.zeros((HALO, 128), F32)
    for t in range(LT):
        k0_s[t, 0:HALO, :] = zeros
        v0_s[t, 0:HALO, :] = zeros
        kf_s[t, 0:8, :] = zeros[0:8]
    for n in range(9):
        dft_s[n] = pltpu.bitcast(dft_ref[n], U32)
    shift = shift_ref[...].astype(F32)
    gate = gate_ref[...].astype(F32).reshape(1, D)
    dvec = dvec_ref[...].astype(F32).reshape(1, D)
    qscale = float(DH ** -0.5 * np.log2(np.e))

    def lanes(t):
        return slice(t * 128, (t + 1) * 128)

    def permute_w_items(p):
        def ktile(kt):
            for t in range(LT):
                blk = w_v[lanes(kt), lanes(p * LT + t)].astype(F32)
                tmp_s[kt, lanes(t), :] = blk.T
            for d in range(DH):
                rows = tmp_s[kt, pl.ds(d, H, stride=DH), :]
                ct, r = divmod(p * D + d * H, 128)
                wp_s[ct, r // 2:(r + H) // 2, lanes(kt)] = _pack(rows)

        return [(1, part_fn(ktile, kt)) for kt in range(LT)]

    def permute_wo_items():
        def ntile(t):
            tmp_s[t] = wo_v[:, lanes(t)].astype(F32)
            for d in range(DH):
                rows = tmp_s[t, pl.ds(d, H, stride=DH), :]
                wop_s[t, d * H // 2:(d + 1) * H // 2, :] = _pack(rows)

        return [(1, part_fn(ntile, t)) for t in range(LT)]

    def stage_x(i):
        xp_s[...] = pltpu.bitcast(x_v[i * BLK:(i + 1) * BLK, :], U32)

    def project_items(i, parts=(0, 1, 2)):
        def tile(p, t):
            acc = _nt(_unpack(xp_s[...]), _unpack(wp_s[p * LT + t]))
            if p == 0:
                qkv_s[i % 2][0][t] = acc * qscale
            else:
                qkv_s[i % 2][p][t, HALO:HALO + BLK, :] = acc

        return [(1, part_fn(tile, p, t)) for p in parts for t in range(LT)]

    def halo_copy(i):
        for src, dst in zip(qkv_s[i % 2][1:], qkv_s[(i + 1) % 2][1:]):
            for t in range(LT):
                dst[t, 0:HALO, :] = src[t, BLK:BLK + HALO, :]

    def attend_items(i):
        q_s, ka_s, va_s = qkv_s[i % 2]
        rc, part = 16, 64

        def scores(row):
            n, sub = divmod(row, part)
            qs = [q_s[t, row:row + rc, :] for t in range(LT)]
            for w in range(WIN):
                lo = row + HALO - DIL * w
                a = qs[0] * ka_s[0, lo:lo + rc, :]
                for t in range(1, LT):
                    a = a + qs[t] * ka_s[t, lo:lo + rc, :]
                pp_s[n, (w * part + sub) // 2:(w * part + sub + rc) // 2, :] = _pack(a)

        def head_sum(n):
            lg_s[n] = _nn(_unpack(pp_s[n]), _unpack(dft_s[8]))

        def mix(row):
            n, sub = divmod(row, part)
            r0 = i * BLK + row
            xs = [x_v[r0:r0 + rc, lanes(t)].astype(F32) for t in range(LT)]
            z = xs[0] * gate[:, lanes(0)]
            for t in range(1, LT):
                z = z + xs[t] * gate[:, lanes(t)]
            th = 0.5 * jnp.tanh(0.5 * jnp.sum(z, axis=-1, keepdims=True))
            g = 0.5 + th
            for t in range(LT):
                gq_s[t, r0:r0 + rc, :] = xs[t] * g
            logits = []
            for w in range(WIN):
                a = lg_s[n, w * part + sub:w * part + sub + rc, :]
                if r0 < DIL * w:
                    pos = r0 + jax.lax.broadcasted_iota(jnp.int32, (rc, 128), 0)
                    a = jnp.where(pos >= DIL * w, a, -1e9)
                logits.append(a)
            m = logits[0]
            for w in range(1, WIN):
                m = jnp.maximum(m, logits[w])
            es = [jnp.exp2(a - m) for a in logits]
            den = es[0]
            for w in range(1, WIN):
                den = den + es[w]
            inv = pl.reciprocal(den, approx=True)
            inv = inv * (2.0 - den * inv)
            norm = (0.5 - th) * inv
            for t in range(LT):
                a = None
                for w in range(WIN):
                    lo = row + HALO - DIL * w
                    term = es[w] * va_s[t, lo:lo + rc, :]
                    a = term if a is None else a + term
                o_s[i % 2][row // 2:(row + rc) // 2, lanes(t)] = _pack(a * norm)

        items = []
        for row in range(0, BLK + part, rc):
            if row < BLK:
                items.append((150, part_fn(scores, row)))
                if (row + rc) % part == 0:
                    items.append((30, part_fn(head_sum, row // part)))
            if row >= part:
                items.append((290, part_fn(mix, row - part)))
        return items

    def signal_items(i):
        r0 = i * BLK

        def tile(t):
            kf_s[t, r0 + 8:r0 + 8 + BLK, :] = k_v[r0:r0 + BLK, lanes(t)].astype(F32)
            xs = []
            for b in range(4):
                ks = None
                for j in range(KS):
                    lo = r0 + 8 + 64 * b - j
                    term = kf_s[t, lo:lo + 64, :] * shift[j:j + 1, lanes(t)]
                    ks = term if ks is None else ks + term
                xs.append(ks * v_v[r0 + 64 * b:r0 + 64 * (b + 1), lanes(t)].astype(F32))
            x0, x1, x2, x3 = xs
            t0, t1 = x0 - x2, x1 + x3
            w0, w1 = SQRT2 * x3, SQRT2 * x2
            res = ((x0 + x2, t1), (t0, x1 - x3), (t0 - w0, t1 + w1), (t0 + w0, t1 - w1))
            for cl in range(4):
                r = jnp.concatenate(res[cl], axis=0).astype(BF16)
                u_s[i, t, cl] = _nn(_unpack(dft_s[cl]), r)

        return [(450, part_fn(tile, t)) for t in range(LT)]

    def filter_items(a):
        def tile(t):
            lane = jax.lax.broadcasted_iota(jnp.int32, (128, 128), 1)
            sign = jnp.where(lane < 64, -1.0, 1.0).astype(F32)
            lo, hi = (h_v[lanes(t), lanes(2 * a + n)].astype(F32) for n in (0, 1))
            if a == 0:
                elo, ehi, olo, ohi = lo, hi, lo, hi
            else:
                plo, phi = (h_v[lanes(t), lanes(2 * a - 2 + n)].astype(F32) for n in (0, 1))
                elo, ehi, olo, ohi = lo + plo, hi + phi, lo - plo, hi - phi
            tt = olo + sign * ohi
            ww = (SQRT2 * sign) * pltpu.roll(ohi, 64, 1)
            res = (elo + ehi, elo - ehi, tt + ww, tt - ww)
            for cl in range(4):
                spec = _nt(_unpack(dft_s[cl]), res[cl].astype(BF16))
                if a < 2:
                    row = jax.lax.broadcasted_iota(jnp.int32, (128, 128), 0)
                    real = (row & 8) == 0
                    if cl == 0:
                        real = real | (row == 8)
                    dd = dvec[:, lanes(t)] if (a == 0 or cl < 2) else -dvec[:, lanes(t)]
                    spec = spec + jnp.where(real, dd, 0.0)
                g_s[a, t, cl] = spec

        return [(300, part_fn(tile, t)) for t in range(LT)]

    def spectrum_items(m):
        def group(t, cl):
            for r in range(8):
                re, im = slice(16 * r, 16 * r + 8), slice(16 * r + 8, 16 * r + 16)
                yr = yi = None
                for a in range(m + 1):
                    gr, gi = g_s[a, t, cl, re, :], g_s[a, t, cl, im, :]
                    ur, ui = u_s[m - a, t, cl, re, :], u_s[m - a, t, cl, im, :]
                    ga, gb = gi, gr
                    if cl == 0 and r == 0:
                        slot0 = jax.lax.broadcasted_iota(jnp.int32, (8, 128), 0) == 0
                        ga, gb = jnp.where(slot0, 0.0, gi), jnp.where(slot0, gi, gr)
                    pr = ur * gr - ui * ga
                    pi = ur * ga + ui * gb
                    yr = pr if yr is None else yr + pr
                    yi = pi if yi is None else yi + pi
                y_s[m % 2, t, cl, 8 * r:8 * r + 8, :] = _pack(jnp.concatenate([yr, yi], axis=0))

        return [(64 * (m + 1), part_fn(group, t, cl)) for t in range(LT) for cl in range(4)]

    def finish_items(m):
        def tile(t):
            rho = [_nn(_unpack(dft_s[4 + cl]), _unpack(y_s[m % 2, t, cl])) for cl in range(4)]
            (a0, a1), (b0, b1), (p0, p1), (n0, n1) = [(z[:64], z[64:]) for z in rho]
            s0, s1, d0, d1 = p0 + n0, p1 + n1, p0 - n0, p1 - n1
            ys = (a0 + b0 + s0, a1 + b1 + s1,
                  a0 - b0 - s0 + SQRT2 * d1, a1 - b1 + s1 - SQRT2 * d0)
            bb = _nn(_unpack(o_s[m % 2][...]), _unpack(wop_s[t]))
            for b in range(4):
                lo = m * BLK + 64 * b
                res = gq_s[t, lo:lo + 64, :] * ys[b] + bb[64 * b:64 * (b + 1)]
                out_s[lo:lo + 64, lanes(t)] = res.astype(BF16)

        return [(1, part_fn(tile, t)) for t in range(LT)]

    for i in range(NB + 2):
        streams = []
        if i == 0:
            cp_w[0].wait()
            for c in (cp_w[1], cp_k[0], cp_v[0], cp_h[0], cp_w[2]):
                c.start()
            _interleave(permute_w_items(0))
            cp_x[0].wait()
            stage_x(0)
            cp_w[1].wait()
            _interleave(project_items(0, (0,)), permute_w_items(1))
            for c in (cp_k[0], cp_v[0], cp_h[0], cp_w[2]):
                c.wait()
            for c in (cp_x[1], cp_k[1], cp_v[1], cp_h[1], cp_wo):
                c.start()
            _interleave(project_items(0, (1,)), permute_w_items(2), signal_items(0))
            streams += [project_items(0, (2,)), filter_items(0)]
        elif i < NB:
            for c in (cp_x[i], cp_k[i], cp_v[i], cp_h[i]):
                c.wait()
            if i + 1 < NB:
                for c in (cp_x[i + 1], cp_k[i + 1], cp_v[i + 1], cp_h[i + 1]):
                    c.start()
            stage_x(i)
            streams += [project_items(i), signal_items(i) + filter_items(i)]
        if i == 1:
            cp_wo.wait()
            streams.append(permute_wo_items())
        if 1 <= i <= NB:
            streams += [attend_items(i - 1), spectrum_items(i - 1)]
        if i >= 2:
            streams.append(finish_items(i - 2))
        _interleave(*streams)
        if i + 1 < NB:
            halo_copy(i)
        if i >= 2:
            cp_out[i - 2].start()
    for c in cp_out:
        c.wait()


@jax.jit
def pallas_gated_mix__ssm_conv_h3__sliding_local_dilated__prompt_kernel(
    A_q: jax.Array,
    A_k: jax.Array,
    A_v: jax.Array,
    A_shift_k: jax.Array,
    A_ssm_k: jax.Array,
    A_ssm_D: jax.Array,
    B_x: jax.Array,
    B_wqkv: jax.Array,
    B_wo: jax.Array,
    gate_w: jax.Array,
):
    del B_x
    hbm = pl.BlockSpec(memory_space=pl.ANY)
    vmem = pl.BlockSpec(memory_space=pltpu.VMEM)
    qkv = [pltpu.VMEM((LT, BLK, 128), F32)] * 2 + [pltpu.VMEM((LT, HALO + BLK, 128), F32)] * 4
    out = pl.pallas_call(
        _kernel,
        out_shape=jax.ShapeDtypeStruct((S, D), BF16),
        in_specs=[hbm] * 6 + [vmem] * 4,
        out_specs=hbm,
        scratch_shapes=[
            pltpu.VMEM((S, D), BF16),
            pltpu.VMEM((S, D), BF16),
            pltpu.VMEM((S, D), BF16),
            pltpu.VMEM((D, S), BF16),
            pltpu.VMEM((D, 3 * D), BF16),
            pltpu.VMEM((D, D), BF16),
            pltpu.VMEM((LT, D, 128), F32),
            pltpu.VMEM((3 * LT, 64, D), U32),
            pltpu.VMEM((LT, D // 2, 128), U32),
            pltpu.VMEM((9, 64, 128), U32),
            pltpu.VMEM((BLK // 2, D), U32),
            *qkv,
            pltpu.VMEM((LT, 8 + S, 128), F32),
            pltpu.VMEM((4, WIN * 32, 128), U32),
            pltpu.VMEM((4, WIN * 64, 128), F32),
            pltpu.VMEM((BLK // 2, D), U32),
            pltpu.VMEM((BLK // 2, D), U32),
            pltpu.VMEM((LT, S, 128), F32),
            pltpu.VMEM((NB, LT, 4, 128, 128), F32),
            pltpu.VMEM((NB, LT, 4, 128, 128), F32),
            pltpu.VMEM((2, LT, 4, 64, 128), U32),
            pltpu.VMEM((S, D), BF16),
            pltpu.SemaphoreType.DMA((3,)),
            pltpu.SemaphoreType.DMA((NB,)),
            pltpu.SemaphoreType.DMA((NB,)),
            pltpu.SemaphoreType.DMA((NB,)),
            pltpu.SemaphoreType.DMA((NB,)),
            pltpu.SemaphoreType.DMA((1,)),
            pltpu.SemaphoreType.DMA((NB,)),
        ],
        compiler_params=pltpu.CompilerParams(vmem_limit_bytes=100 * 2**20),
    )(A_q.reshape(S, D), A_k.reshape(S, D), A_v.reshape(S, D), A_ssm_k, B_wqkv, B_wo,
      A_shift_k.T, A_ssm_D, gate_w, jnp.asarray(_DFT, BF16))
    return out.reshape(1, S, D)
```

```python
import functools

import numpy as np
import jax
import jax.numpy as jnp
import jax.experimental.pallas as pl
import jax.experimental.pallas.tpu as pltpu

S, D = 2048, 640
H, DH = 32, 20
WIN, DIL = 8, 2
KS = 4
LT = D // 128
BLK = 256
NB = S // BLK
HALO = 16
SQRT2 = float(np.sqrt(2.0))
F32, BF16, U32 = jnp.float32, jnp.bfloat16, jnp.uint32


def _dft_matrices():
    n = np.arange(128)[None, :]
    m = np.arange(64)[:, None]
    order = np.arange(128).reshape(2, 8, 8).transpose(1, 0, 2).reshape(-1)
    fwd, inv = [], []
    for f in (4 * m, 4 * m + 2, 8 * m + 1, 8 * m + 3):
        ang = 2.0 * np.pi * ((f * n) % 512) / 512.0
        a = np.concatenate([np.cos(ang), -np.sin(ang)], axis=0)
        wgt = np.full((128, 1), 2.0 / 512.0)
        if not fwd:
            a[64] = np.cos(np.pi * n[0])
            wgt[0] = wgt[64] = 1.0 / 512.0
        fwd.append(a[order])
        inv.append((a * wgt)[order].T)
    lane = np.arange(128)
    same_head = (lane[:, None] % H == lane[None, :] % H)
    return np.stack(fwd + inv + [same_head]).astype(np.float32)


_DFT = _dft_matrices()


def _nt(a, b):
    return jax.lax.dot_general(a, b, (((1,), (1,)), ((), ())),
                               preferred_element_type=F32)


def _nn(a, b):
    return jnp.dot(a, b, preferred_element_type=F32)


def _pack(x):
    return pltpu.bitcast(x.astype(BF16), U32)


def _unpack(x):
    return pltpu.bitcast(x, BF16)


def _interleave(*streams):
    items = []
    for s in streams:
        total, done = sum(c for c, _ in s), 0.0
        for c, f in s:
            items.append(((done + 0.5 * c) / total, f))
            done += c
    for _, f in sorted(items, key=lambda e: e[0]):
        f()


def _kernel(x_hbm, k_hbm, v_hbm, h_hbm, w_hbm, wo_hbm,
            shift_ref, dvec_ref, gate_ref, dft_ref,
            out_hbm,
            x_v, k_v, v_v, h_v, w_v, wo_v,
            tmp_s, dft_s, xp_s, q0_s, q1_s, k0_s, k1_s, v0_s, v1_s,
            kf_s, lg_s, o0_s, o1_s, gq_s, u_s, g_s, out_s,
            w_sem, x_sem, k_sem, v_sem, h_sem, wo_sem, out_sem):
    part_fn = functools.partial

    def rows_copy(src, dst, sem, n):
        rows = pl.ds(n * BLK, BLK)
        return pltpu.make_async_copy(src.at[rows], dst.at[rows], sem.at[n])

    def cols_copy(src, dst, sem, n, size):
        cols = pl.ds(n * size, size)
        return pltpu.make_async_copy(src.at[:, cols], dst.at[:, cols], sem.at[n])

    cp_w = [cols_copy(w_hbm, w_v, w_sem, n, D) for n in range(3)]
    cp_x = [rows_copy(x_hbm, x_v, x_sem, n) for n in range(NB)]
    cp_k = [rows_copy(k_hbm, k_v, k_sem, n) for n in range(NB)]
    cp_v = [rows_copy(v_hbm, v_v, v_sem, n) for n in range(NB)]
    cp_h = [cols_copy(h_hbm, h_v, h_sem, n, BLK) for n in range(NB)]
    cp_wo = pltpu.make_async_copy(wo_hbm, wo_v, wo_sem.at[0])
    cp_out = [rows_copy(out_s, out_hbm, out_sem, n) for n in range(NB)]

    cp_w[0].start()
    cp_x[0].start()

    qkv_s = ((q0_s, k0_s, v0_s), (q1_s, k1_s, v1_s))
    o_s = (o0_s, o1_s)
    zeros = jnp.zeros((HALO, 128), F32)
    for t in range(LT):
        k0_s[t, 0:HALO, :] = zeros
        v0_s[t, 0:HALO, :] = zeros
        kf_s[t, 0:8, :] = zeros[0:8]
    for n in range(9):
        dft_s[n] = pltpu.bitcast(dft_ref[n], U32)
    shift = shift_ref[...].astype(F32)
    gate = gate_ref[...].astype(F32).reshape(1, D)
    dvec = dvec_ref[...].astype(F32).reshape(1, D)
    qscale = float(DH ** -0.5 * np.log2(np.e))

    def lanes(t):
        return slice(t * 128, (t + 1) * 128)

    w_tiles, wo_tiles, partial, spectra = {}, {}, {}, {}

    def permute_w_items(p):
        def ktile(kt):
            for t in range(LT):
                blk = w_v[lanes(kt), lanes(p * LT + t)].astype(F32)
                tmp_s[kt, lanes(t), :] = blk.T
            for t in range(LT):
                rows = [tmp_s[kt, pl.ds(4 * t + n, H, stride=DH), :] for n in range(4)]
                w_tiles[p, t, kt] = jnp.concatenate(rows, axis=0).astype(BF16)

        return [(1, part_fn(ktile, kt)) for kt in range(LT)]

    def permute_wo_items():
        def ntile(t):
            tmp_s[t] = wo_v[:, lanes(t)].astype(F32)
            rows = [tmp_s[t, pl.ds(d, H, stride=DH), :] for d in range(DH)]
            wo_tiles[t] = jnp.concatenate(rows, axis=0).astype(BF16)

        return [(1, part_fn(ntile, t)) for t in range(LT)]

    def stage_x(i):
        xp_s[...] = pltpu.bitcast(x_v[i * BLK:(i + 1) * BLK, :], U32)

    def project_items(i, parts=(0, 1, 2)):
        def tile(p, t):
            wt = jnp.concatenate([w_tiles[p, t, kt] for kt in range(LT)], axis=1)
            acc = _nt(_unpack(xp_s[...]), wt)
            if p == 0:
                qkv_s[i % 2][0][t] = acc * qscale
            else:
                qkv_s[i % 2][p][t, HALO:HALO + BLK, :] = acc

        return [(1, part_fn(tile, p, t)) for p in parts for t in range(LT)]

    def halo_copy(i):
        for src, dst in zip(qkv_s[i % 2][1:], qkv_s[(i + 1) % 2][1:]):
            for t in range(LT):
                dst[t, 0:HALO, :] = src[t, BLK:BLK + HALO, :]

    def attend_items(i):
        q_s, ka_s, va_s = qkv_s[i % 2]
        rc, part = 16, 64

        def scores(row):
            qs = [q_s[t, row:row + rc, :] for t in range(LT)]
            sums = []
            for w in range(WIN):
                lo = row + HALO - DIL * w
                a = qs[0] * ka_s[0, lo:lo + rc, :]
                for t in range(1, LT):
                    a = a + qs[t] * ka_s[t, lo:lo + rc, :]
                sums.append(a)
            partial[row] = jnp.concatenate(sums, axis=0).astype(BF16)

        def head_sum(n):
            lhs = jnp.concatenate(
                [partial[row] for row in range(n * part, (n + 1) * part, rc)], axis=0)
            lg_s[n] = _nn(lhs, _unpack(dft_s[8]))

        def mix(row):
            n, sub = divmod(row, part)
            r0 = i * BLK + row
            xs = [x_v[r0:r0 + rc, lanes(t)].astype(F32) for t in range(LT)]
            z = xs[0] * gate[:, lanes(0)]
            for t in range(1, LT):
                z = z + xs[t] * gate[:, lanes(t)]
            th = 0.5 * jnp.tanh(0.5 * jnp.sum(z, axis=-1, keepdims=True))
            g = 0.5 + th
            for t in range(LT):
                gq_s[t, r0:r0 + rc, :] = xs[t] * g
            logits = []
            for w in range(WIN):
                a = lg_s[n, sub * WIN + w * rc:sub * WIN + (w + 1) * rc, :]
                if r0 < DIL * w:
                    pos = r0 + jax.lax.broadcasted_iota(jnp.int32, (rc, 128), 0)
                    a = jnp.where(pos >= DIL * w, a, -1e9)
                logits.append(a)
            m = logits[0]
            for w in range(1, WIN):
                m = jnp.maximum(m, logits[w])
            es = [jnp.exp2(a - m) for a in logits]
            den = es[0]
            for w in range(1, WIN):
                den = den + es[w]
            inv = pl.reciprocal(den, approx=True)
            inv = inv * (2.0 - den * inv)
            norm = (0.5 - th) * inv
            for t in range(LT):
                a = None
                for w in range(WIN):
                    lo = row + HALO - DIL * w
                    term = es[w] * va_s[t, lo:lo + rc, :]
                    a = term if a is None else a + term
                o_s[i % 2][row // 2:(row + rc) // 2, lanes(t)] = _pack(a * norm)

        items = []
        for row in range(0, BLK + part, rc):
            if row < BLK:
                items.append((150, part_fn(scores, row)))
                if (row + rc) % part == 0:
                    items.append((30, part_fn(head_sum, row // part)))
            if row >= part:
                items.append((290, part_fn(mix, row - part)))
        return items

    def signal_items(i):
        r0 = i * BLK

        def tile(t):
            kf_s[t, r0 + 8:r0 + 8 + BLK, :] = k_v[r0:r0 + BLK, lanes(t)].astype(F32)
            xs = []
            for b in range(4):
                ks = None
                for j in range(KS):
                    lo = r0 + 8 + 64 * b - j
                    term = kf_s[t, lo:lo + 64, :] * shift[j:j + 1, lanes(t)]
                    ks = term if ks is None else ks + term
                xs.append(ks * v_v[r0 + 64 * b:r0 + 64 * (b + 1), lanes(t)].astype(F32))
            x0, x1, x2, x3 = xs
            t0, t1 = x0 - x2, x1 + x3
            w0, w1 = SQRT2 * x3, SQRT2 * x2
            res = ((x0 + x2, t1), (t0, x1 - x3), (t0 - w0, t1 + w1), (t0 + w0, t1 - w1))
            for cl in range(4):
                r = jnp.concatenate(res[cl], axis=0).astype(BF16)
                u_s[i, t, cl] = _nn(_unpack(dft_s[cl]), r)

        return [(450, part_fn(tile, t)) for t in range(LT)]

    def filter_items(a):
        def tile(t):
            lane = jax.lax.broadcasted_iota(jnp.int32, (128, 128), 1)
            sign = jnp.where(lane < 64, -1.0, 1.0).astype(F32)
            lo, hi = (h_v[lanes(t), lanes(2 * a + n)].astype(F32) for n in (0, 1))
            if a == 0:
                elo, ehi, olo, ohi = lo, hi, lo, hi
            else:
                plo, phi = (h_v[lanes(t), lanes(2 * a - 2 + n)].astype(F32) for n in (0, 1))
                elo, ehi, olo, ohi = lo + plo, hi + phi, lo - plo, hi - phi
            tt = olo + sign * ohi
            ww = (SQRT2 * sign) * pltpu.roll(ohi, 64, 1)
            res = (elo + ehi, elo - ehi, tt + ww, tt - ww)
            for cl in range(4):
                spec = _nt(_unpack(dft_s[cl]), res[cl].astype(BF16))
                if a < 2:
                    row = jax.lax.broadcasted_iota(jnp.int32, (128, 128), 0)
                    real = (row & 8) == 0
                    if cl == 0:
                        real = real | (row == 8)
                    dd = dvec[:, lanes(t)] if (a == 0 or cl < 2) else -dvec[:, lanes(t)]
                    spec = spec + jnp.where(real, dd, 0.0)
                g_s[a, t, cl] = spec

        return [(300, part_fn(tile, t)) for t in range(LT)]

    def spectrum_items(m):
        def group(t, cl):
            out = []
            for r in range(8):
                re, im = slice(16 * r, 16 * r + 8), slice(16 * r + 8, 16 * r + 16)
                yr = yi = None
                for a in range(m + 1):
                    gr, gi = g_s[a, t, cl, re, :], g_s[a, t, cl, im, :]
                    ur, ui = u_s[m - a, t, cl, re, :], u_s[m - a, t, cl, im, :]
                    ga, gb = gi, gr
                    if cl == 0 and r == 0:
                        slot0 = jax.lax.broadcasted_iota(jnp.int32, (8, 128), 0) == 0
                        ga, gb = jnp.where(slot0, 0.0, gi), jnp.where(slot0, gi, gr)
                    pr = ur * gr - ui * ga
                    pi = ur * ga + ui * gb
                    yr = pr if yr is None else yr + pr
                    yi = pi if yi is None else yi + pi
                out += [yr, yi]
            spectra[m, t, cl] = jnp.concatenate(out, axis=0).astype(BF16)

        return [(64 * (m + 1), part_fn(group, t, cl)) for t in range(LT) for cl in range(4)]

    def finish_items(m):
        def tile(t):
            rho = [_nn(_unpack(dft_s[4 + cl]), spectra[m, t, cl]) for cl in range(4)]
            (a0, a1), (b0, b1), (p0, p1), (n0, n1) = [(z[:64], z[64:]) for z in rho]
            s0, s1, d0, d1 = p0 + n0, p1 + n1, p0 - n0, p1 - n1
            ys = (a0 + b0 + s0, a1 + b1 + s1,
                  a0 - b0 - s0 + SQRT2 * d1, a1 - b1 + s1 - SQRT2 * d0)
            bb = _nn(_unpack(o_s[m % 2][...]), wo_tiles[t])
            for b in range(4):
                lo = m * BLK + 64 * b
                res = gq_s[t, lo:lo + 64, :] * ys[b] + bb[64 * b:64 * (b + 1)]
                out_s[lo:lo + 64, lanes(t)] = res.astype(BF16)

        return [(1, part_fn(tile, t)) for t in range(LT)]

    for i in range(NB + 2):
        streams = []
        if i == 0:
            cp_w[0].wait()
            for c in (cp_w[1], cp_k[0], cp_v[0], cp_h[0], cp_w[2]):
                c.start()
            _interleave(permute_w_items(0))
            cp_x[0].wait()
            stage_x(0)
            cp_w[1].wait()
            _interleave(project_items(0, (0,)), permute_w_items(1))
            for c in (cp_k[0], cp_v[0], cp_h[0], cp_w[2]):
                c.wait()
            for c in (cp_x[1], cp_k[1], cp_v[1], cp_h[1], cp_wo):
                c.start()
            _interleave(project_items(0, (1,)), permute_w_items(2), signal_items(0))
            streams += [project_items(0, (2,)), filter_items(0)]
        elif i < NB:
            for c in (cp_x[i], cp_k[i], cp_v[i], cp_h[i]):
                c.wait()
            if i + 1 < NB:
                for c in (cp_x[i + 1], cp_k[i + 1], cp_v[i + 1], cp_h[i + 1]):
                    c.start()
            stage_x(i)
            streams += [project_items(i), signal_items(i) + filter_items(i)]
        if i == 1:
            cp_wo.wait()
            streams.append(permute_wo_items())
        if 1 <= i <= NB:
            streams += [attend_items(i - 1), spectrum_items(i - 1)]
        if i >= 2:
            streams.append(finish_items(i - 2))
        _interleave(*streams)
        if i + 1 < NB:
            halo_copy(i)
        if i >= 2:
            cp_out[i - 2].start()
    for c in cp_out:
        c.wait()


@jax.jit
def pallas_gated_mix__ssm_conv_h3__sliding_local_dilated__prompt_kernel(
    A_q: jax.Array,
    A_k: jax.Array,
    A_v: jax.Array,
    A_shift_k: jax.Array,
    A_ssm_k: jax.Array,
    A_ssm_D: jax.Array,
    B_x: jax.Array,
    B_wqkv: jax.Array,
    B_wo: jax.Array,
    gate_w: jax.Array,
):
    del B_x
    hbm = pl.BlockSpec(memory_space=pl.ANY)
    vmem = pl.BlockSpec(memory_space=pltpu.VMEM)
    qkv = [pltpu.VMEM((LT, BLK, 128), F32)] * 2 + [pltpu.VMEM((LT, HALO + BLK, 128), F32)] * 4
    out = pl.pallas_call(
        _kernel,
        out_shape=jax.ShapeDtypeStruct((S, D), BF16),
        in_specs=[hbm] * 6 + [vmem] * 4,
        out_specs=hbm,
        scratch_shapes=[
            pltpu.VMEM((S, D), BF16),
            pltpu.VMEM((S, D), BF16),
            pltpu.VMEM((S, D), BF16),
            pltpu.VMEM((D, S), BF16),
            pltpu.VMEM((D, 3 * D), BF16),
            pltpu.VMEM((D, D), BF16),
            pltpu.VMEM((LT, D, 128), F32),
            pltpu.VMEM((9, 64, 128), U32),
            pltpu.VMEM((BLK // 2, D), U32),
            *qkv,
            pltpu.VMEM((LT, 8 + S, 128), F32),
            pltpu.VMEM((4, WIN * 64, 128), F32),
            pltpu.VMEM((BLK // 2, D), U32),
            pltpu.VMEM((BLK // 2, D), U32),
            pltpu.VMEM((LT, S, 128), F32),
            pltpu.VMEM((NB, LT, 4, 128, 128), F32),
            pltpu.VMEM((NB, LT, 4, 128, 128), F32),
            pltpu.VMEM((S, D), BF16),
            pltpu.SemaphoreType.DMA((3,)),
            pltpu.SemaphoreType.DMA((NB,)),
            pltpu.SemaphoreType.DMA((NB,)),
            pltpu.SemaphoreType.DMA((NB,)),
            pltpu.SemaphoreType.DMA((NB,)),
            pltpu.SemaphoreType.DMA((1,)),
            pltpu.SemaphoreType.DMA((NB,)),
        ],
        compiler_params=pltpu.CompilerParams(vmem_limit_bytes=100 * 2**20),
    )(A_q.reshape(S, D), A_k.reshape(S, D), A_v.reshape(S, D), A_ssm_k, B_wqkv, B_wo,
      A_shift_k.T, A_ssm_D, gate_w, jnp.asarray(_DFT, BF16))
    return out.reshape(1, S, D)
```

```python
import functools

import numpy as np
import jax
import jax.numpy as jnp
import jax.experimental.pallas as pl
import jax.experimental.pallas.tpu as pltpu

S, D = 2048, 640
H, DH = 32, 20
WIN, DIL = 8, 2
KS = 4
LT = D // 128
BLK = 256
NB = S // BLK
HALO = 16
SQRT2 = float(np.sqrt(2.0))
F32, BF16, U32 = jnp.float32, jnp.bfloat16, jnp.uint32


def _dft_matrices():
    n = np.arange(128)[None, :]
    m = np.arange(64)[:, None]
    order = np.arange(128).reshape(2, 8, 8).transpose(1, 0, 2).reshape(-1)
    fwd, inv = [], []
    for f in (4 * m, 4 * m + 2, 8 * m + 1, 8 * m + 3):
        ang = 2.0 * np.pi * ((f * n) % 512) / 512.0
        a = np.concatenate([np.cos(ang), -np.sin(ang)], axis=0)
        wgt = np.full((128, 1), 2.0 / 512.0)
        if not fwd:
            a[64] = np.cos(np.pi * n[0])
            wgt[0] = wgt[64] = 1.0 / 512.0
        fwd.append(a[order])
        inv.append((a * wgt)[order].T)
    lane = np.arange(128)
    same_head = (lane[:, None] % H == lane[None, :] % H)
    return np.stack(fwd + inv + [same_head]).astype(np.float32)


_DFT = _dft_matrices()


def _nt(a, b):
    return jax.lax.dot_general(a, b, (((1,), (1,)), ((), ())),
                               preferred_element_type=F32)


def _nn(a, b):
    return jnp.dot(a, b, preferred_element_type=F32)


def _pack(x):
    return pltpu.bitcast(x.astype(BF16), U32)


def _unpack(x):
    return pltpu.bitcast(x, BF16)


def _interleave(*streams):
    items = []
    for s in streams:
        total, done = sum(c for c, _ in s), 0.0
        for c, f in s:
            items.append(((done + 0.5 * c) / total, f))
            done += c
    for _, f in sorted(items, key=lambda e: e[0]):
        f()


def _kernel(x_hbm, k_hbm, v_hbm, h_hbm, w_hbm, wo_hbm,
            shift_ref, dvec_ref, gate_ref, dft_ref,
            out_hbm,
            x_v, k_v, v_v, h_v, w_v, wo_v,
            tmp_s, dft_s, xp_s, q0_s, q1_s, k0_s, k1_s, v0_s, v1_s,
            kf_s, lg_s, o0_s, o1_s, gq_s, u_s, g_s, out_s,
            w_sem, x_sem, k_sem, v_sem, h_sem, wo_sem, out_sem):
    part_fn = functools.partial

    def rows_copy(src, dst, sem, n):
        rows = pl.ds(n * BLK, BLK)
        return pltpu.make_async_copy(src.at[rows], dst.at[rows], sem.at[n])

    def cols_copy(src, dst, sem, n, size):
        cols = pl.ds(n * size, size)
        return pltpu.make_async_copy(src.at[:, cols], dst.at[:, cols], sem.at[n])

    cp_w = [cols_copy(w_hbm, w_v, w_sem, n, D) for n in range(3)]
    cp_x = [rows_copy(x_hbm, x_v, x_sem, n) for n in range(NB)]
    cp_k = [rows_copy(k_hbm, k_v, k_sem, n) for n in range(NB)]
    cp_v = [rows_copy(v_hbm, v_v, v_sem, n) for n in range(NB)]
    cp_h = [cols_copy(h_hbm, h_v, h_sem, n, BLK) for n in range(NB)]
    cp_wo = pltpu.make_async_copy(wo_hbm, wo_v, wo_sem.at[0])
    cp_out = [rows_copy(out_s, out_hbm, out_sem, n) for n in range(NB)]

    for c in (cp_w[0], cp_x[0], cp_w[1], cp_w[2], cp_k[0], cp_v[0], cp_h[0]):
        c.start()

    qkv_s = ((q0_s, k0_s, v0_s), (q1_s, k1_s, v1_s))
    o_s = (o0_s, o1_s)
    zeros = jnp.zeros((HALO, 128), F32)
    for t in range(LT):
        k0_s[t, 0:HALO, :] = zeros
        v0_s[t, 0:HALO, :] = zeros
        kf_s[t, 0:8, :] = zeros[0:8]
    for n in range(9):
        dft_s[n] = pltpu.bitcast(dft_ref[n], U32)
    shift = shift_ref[...].astype(F32)
    gate = gate_ref[...].astype(F32).reshape(1, D)
    dvec = dvec_ref[...].astype(F32).reshape(1, D)
    qscale = float(DH ** -0.5 * np.log2(np.e))

    def lanes(t):
        return slice(t * 128, (t + 1) * 128)

    w_tiles, wo_tiles, partial, spectra = {}, {}, {}, {}

    def permute_w_items(p):
        def ktile(kt):
            for t in range(LT):
                blk = w_v[lanes(kt), lanes(p * LT + t)].astype(F32)
                tmp_s[kt, lanes(t), :] = blk.T
            for t in range(LT):
                rows = [tmp_s[kt, pl.ds(4 * t + n, H, stride=DH), :] for n in range(4)]
                w_tiles[p, t, kt] = _pack(jnp.concatenate(rows, axis=0))

        return [(1, part_fn(ktile, kt)) for kt in range(LT)]

    def permute_wo_items():
        def ntile(t):
            tmp_s[t] = wo_v[:, lanes(t)].astype(F32)
            rows = [tmp_s[t, pl.ds(d, H, stride=DH), :] for d in range(DH)]
            wo_tiles[t] = jnp.concatenate(rows, axis=0).astype(BF16)

        return [(1, part_fn(ntile, t)) for t in range(LT)]

    def stage_x(i):
        xp_s[...] = pltpu.bitcast(x_v[i * BLK:(i + 1) * BLK, :], U32)

    def project_items(i, parts=(0, 1, 2)):
        def tile(p, t):
            wt = jnp.concatenate([w_tiles[p, t, kt] for kt in range(LT)], axis=1)
            acc = _nt(_unpack(xp_s[...]), _unpack(wt))
            if p == 0:
                qkv_s[i % 2][0][t] = acc * qscale
            else:
                qkv_s[i % 2][p][t, HALO:HALO + BLK, :] = acc

        return [(1, part_fn(tile, p, t)) for p in parts for t in range(LT)]

    def halo_copy(i):
        for src, dst in zip(qkv_s[i % 2][1:], qkv_s[(i + 1) % 2][1:]):
            for t in range(LT):
                dst[t, 0:HALO, :] = src[t, BLK:BLK + HALO, :]

    def attend_items(i):
        q_s, ka_s, va_s = qkv_s[i % 2]
        rc, part = 16, 64

        def scores(row):
            qs = [q_s[t, row:row + rc, :] for t in range(LT)]
            sums = []
            for w in range(WIN):
                lo = row + HALO - DIL * w
                a = qs[0] * ka_s[0, lo:lo + rc, :]
                for t in range(1, LT):
                    a = a + qs[t] * ka_s[t, lo:lo + rc, :]
                sums.append(a)
            partial[row] = _pack(jnp.concatenate(sums, axis=0))

        def head_sum(n):
            lhs = jnp.concatenate(
                [partial[row] for row in range(n * part, (n + 1) * part, rc)], axis=0)
            lg_s[n] = _nn(_unpack(lhs), _unpack(dft_s[8]))

        def mix(row):
            n, sub = divmod(row, part)
            r0 = i * BLK + row
            xs = [x_v[r0:r0 + rc, lanes(t)].astype(F32) for t in range(LT)]
            z = xs[0] * gate[:, lanes(0)]
            for t in range(1, LT):
                z = z + xs[t] * gate[:, lanes(t)]
            th = 0.5 * jnp.tanh(0.5 * jnp.sum(z, axis=-1, keepdims=True))
            g = 0.5 + th
            for t in range(LT):
                gq_s[t, r0:r0 + rc, :] = xs[t] * g
            logits = []
            for w in range(WIN):
                a = lg_s[n, sub * WIN + w * rc:sub * WIN + (w + 1) * rc, :]
                if r0 < DIL * w:
                    pos = r0 + jax.lax.broadcasted_iota(jnp.int32, (rc, 128), 0)
                    a = jnp.where(pos >= DIL * w, a, -1e9)
                logits.append(a)
            m = logits[0]
            for w in range(1, WIN):
                m = jnp.maximum(m, logits[w])
            es = [jnp.exp2(a - m) for a in logits]
            den = es[0]
            for w in range(1, WIN):
                den = den + es[w]
            inv = pl.reciprocal(den, approx=True)
            inv = inv * (2.0 - den * inv)
            norm = (0.5 - th) * inv
            for t in range(LT):
                a = None
                for w in range(WIN):
                    lo = row + HALO - DIL * w
                    term = es[w] * va_s[t, lo:lo + rc, :]
                    a = term if a is None else a + term
                o_s[i % 2][row // 2:(row + rc) // 2, lanes(t)] = _pack(a * norm)

        items = []
        for row in range(0, BLK + part, rc):
            if row < BLK:
                items.append((150, part_fn(scores, row)))
                if (row + rc) % part == 0:
                    items.append((30, part_fn(head_sum, row // part)))
            if row >= part:
                items.append((290, part_fn(mix, row - part)))
        return items

    def signal_items(i):
        r0 = i * BLK

        def tile(t):
            kf_s[t, r0 + 8:r0 + 8 + BLK, :] = k_v[r0:r0 + BLK, lanes(t)].astype(F32)
            xs = []
            for b in range(4):
                ks = None
                for j in range(KS):
                    lo = r0 + 8 + 64 * b - j
                    term = kf_s[t, lo:lo + 64, :] * shift[j:j + 1, lanes(t)]
                    ks = term if ks is None else ks + term
                xs.append(ks * v_v[r0 + 64 * b:r0 + 64 * (b + 1), lanes(t)].astype(F32))
            x0, x1, x2, x3 = xs
            t0, t1 = x0 - x2, x1 + x3
            w0, w1 = SQRT2 * x3, SQRT2 * x2
            res = ((x0 + x2, t1), (t0, x1 - x3), (t0 - w0, t1 + w1), (t0 + w0, t1 - w1))
            for cl in range(4):
                r = jnp.concatenate(res[cl], axis=0).astype(BF16)
                u_s[i, t, cl] = _nn(_unpack(dft_s[cl]), r)

        return [(450, part_fn(tile, t)) for t in range(LT)]

    def filter_items(a):
        def tile(t):
            lane = jax.lax.broadcasted_iota(jnp.int32, (128, 128), 1)
            sign = jnp.where(lane < 64, -1.0, 1.0).astype(F32)
            lo, hi = (h_v[lanes(t), lanes(2 * a + n)].astype(F32) for n in (0, 1))
            if a == 0:
                elo, ehi, olo, ohi = lo, hi, lo, hi
            else:
                plo, phi = (h_v[lanes(t), lanes(2 * a - 2 + n)].astype(F32) for n in (0, 1))
                elo, ehi, olo, ohi = lo + plo, hi + phi, lo - plo, hi - phi
            tt = olo + sign * ohi
            ww = (SQRT2 * sign) * pltpu.roll(ohi, 64, 1)
            res = (elo + ehi, elo - ehi, tt + ww, tt - ww)
            for cl in range(4):
                spec = _nt(_unpack(dft_s[cl]), res[cl].astype(BF16))
                if a < 2:
                    row = jax.lax.broadcasted_iota(jnp.int32, (128, 128), 0)
                    real = (row & 8) == 0
                    if cl == 0:
                        real = real | (row == 8)
                    dd = dvec[:, lanes(t)] if (a == 0 or cl < 2) else -dvec[:, lanes(t)]
                    spec = spec + jnp.where(real, dd, 0.0)
                g_s[a, t, cl] = spec

        return [(300, part_fn(tile, t)) for t in range(LT)]

    def spectrum_items(m):
        def group(t, cl):
            out = []
            for r in range(8):
                re, im = slice(16 * r, 16 * r + 8), slice(16 * r + 8, 16 * r + 16)
                yr = yi = None
                for a in range(m + 1):
                    gr, gi = g_s[a, t, cl, re, :], g_s[a, t, cl, im, :]
                    ur, ui = u_s[m - a, t, cl, re, :], u_s[m - a, t, cl, im, :]
                    ga, gb = gi, gr
                    if cl == 0 and r == 0:
                        slot0 = jax.lax.broadcasted_iota(jnp.int32, (8, 128), 0) == 0
                        ga, gb = jnp.where(slot0, 0.0, gi), jnp.where(slot0, gi, gr)
                    pr = ur * gr - ui * ga
                    pi = ur * ga + ui * gb
                    yr = pr if yr is None else yr + pr
                    yi = pi if yi is None else yi + pi
                out += [yr, yi]
            spectra[m, t, cl] = jnp.concatenate(out, axis=0).astype(BF16)

        return [(64 * (m + 1), part_fn(group, t, cl)) for t in range(LT) for cl in range(4)]

    def finish_items(m):
        def tile(t):
            rho = [_nn(_unpack(dft_s[4 + cl]), spectra[m, t, cl]) for cl in range(4)]
            (a0, a1), (b0, b1), (p0, p1), (n0, n1) = [(z[:64], z[64:]) for z in rho]
            s0, s1, d0, d1 = p0 + n0, p1 + n1, p0 - n0, p1 - n1
            ys = (a0 + b0 + s0, a1 + b1 + s1,
                  a0 - b0 - s0 + SQRT2 * d1, a1 - b1 + s1 - SQRT2 * d0)
            bb = _nn(_unpack(o_s[m % 2][...]), wo_tiles[t])
            for b in range(4):
                lo = m * BLK + 64 * b
                res = gq_s[t, lo:lo + 64, :] * ys[b] + bb[64 * b:64 * (b + 1)]
                out_s[lo:lo + 64, lanes(t)] = res.astype(BF16)

        return [(1, part_fn(tile, t)) for t in range(LT)]

    def fetch(n):
        for c in (cp_x[n], cp_k[n], cp_v[n], cp_h[n]):
            c.start()

    for i in range(NB + 2):
        streams = []
        if i == 0:
            cp_w[0].wait()
            _interleave(permute_w_items(0))
            cp_x[0].wait()
            stage_x(0)
            cp_w[1].wait()
            _interleave(project_items(0, (0,)), permute_w_items(1))
            cp_w[2].wait()
            fetch(1)
            _interleave(project_items(0, (1,)), permute_w_items(2))
            for c in (cp_k[0], cp_v[0], cp_h[0]):
                c.wait()
            cp_wo.start()
            streams.append(project_items(0, (2,)))
        elif i < NB:
            for c in (cp_x[i], cp_k[i], cp_v[i], cp_h[i]):
                c.wait()
            if i + 1 < NB:
                fetch(i + 1)
            stage_x(i)
            streams.append(project_items(i))
        if i < NB:
            sig, fil, spec = signal_items(i), filter_items(i), spectrum_items(i)
            conv = []
            for t in range(LT + 1):
                if t < LT:
                    conv += [sig[t], fil[t]]
                if t > 0:
                    conv += spec[4 * (t - 1):4 * t]
            streams.append(conv)
        if i == 1:
            cp_wo.wait()
            streams.append(permute_wo_items())
        if 1 <= i <= NB:
            streams.append(attend_items(i - 1))
        if i >= 2:
            streams.append(finish_items(i - 2))
        _interleave(*streams)
        if i + 1 < NB:
            halo_copy(i)
        if i >= 2:
            cp_out[i - 2].start()
    for c in cp_out:
        c.wait()


@jax.jit
def pallas_gated_mix__ssm_conv_h3__sliding_local_dilated__prompt_kernel(
    A_q: jax.Array,
    A_k: jax.Array,
    A_v: jax.Array,
    A_shift_k: jax.Array,
    A_ssm_k: jax.Array,
    A_ssm_D: jax.Array,
    B_x: jax.Array,
    B_wqkv: jax.Array,
    B_wo: jax.Array,
    gate_w: jax.Array,
):
    del B_x
    hbm = pl.BlockSpec(memory_space=pl.ANY)
    vmem = pl.BlockSpec(memory_space=pltpu.VMEM)
    qkv = [pltpu.VMEM((LT, BLK, 128), F32)] * 2 + [pltpu.VMEM((LT, HALO + BLK, 128), F32)] * 4
    out = pl.pallas_call(
        _kernel,
        out_shape=jax.ShapeDtypeStruct((S, D), BF16),
        in_specs=[hbm] * 6 + [vmem] * 4,
        out_specs=hbm,
        scratch_shapes=[
            pltpu.VMEM((S, D), BF16),
            pltpu.VMEM((S, D), BF16),
            pltpu.VMEM((S, D), BF16),
            pltpu.VMEM((D, S), BF16),
            pltpu.VMEM((D, 3 * D), BF16),
            pltpu.VMEM((D, D), BF16),
            pltpu.VMEM((LT, D, 128), F32),
            pltpu.VMEM((9, 64, 128), U32),
            pltpu.VMEM((BLK // 2, D), U32),
            *qkv,
            pltpu.VMEM((LT, 8 + S, 128), F32),
            pltpu.VMEM((4, WIN * 64, 128), F32),
            pltpu.VMEM((BLK // 2, D), U32),
            pltpu.VMEM((BLK // 2, D), U32),
            pltpu.VMEM((LT, S, 128), F32),
            pltpu.VMEM((NB, LT, 4, 128, 128), F32),
            pltpu.VMEM((NB, LT, 4, 128, 128), F32),
            pltpu.VMEM((S, D), BF16),
            pltpu.SemaphoreType.DMA((3,)),
            pltpu.SemaphoreType.DMA((NB,)),
            pltpu.SemaphoreType.DMA((NB,)),
            pltpu.SemaphoreType.DMA((NB,)),
            pltpu.SemaphoreType.DMA((NB,)),
            pltpu.SemaphoreType.DMA((1,)),
            pltpu.SemaphoreType.DMA((NB,)),
        ],
        compiler_params=pltpu.CompilerParams(vmem_limit_bytes=100 * 2**20),
    )(A_q.reshape(S, D), A_k.reshape(S, D), A_v.reshape(S, D), A_ssm_k, B_wqkv, B_wo,
      A_shift_k.T, A_ssm_D, gate_w, jnp.asarray(_DFT, BF16))
    return out.reshape(1, S, D)
```

```python
import functools

import numpy as np
import jax
import jax.numpy as jnp
import jax.experimental.pallas as pl
import jax.experimental.pallas.tpu as pltpu

S, D = 2048, 640
H, DH = 32, 20
WIN, DIL = 8, 2
KS = 4
LT = D // 128
BLK = 256
NB = S // BLK
HS = 64
PM = 128
HALO = 16
SQRT2 = float(np.sqrt(2.0))
F32, BF16, U32 = jnp.float32, jnp.bfloat16, jnp.uint32


def _dft_matrices():
    n = np.arange(128)[None, :]
    m = np.arange(64)[:, None]
    order = np.arange(128).reshape(2, 8, 8).transpose(1, 0, 2).reshape(-1)
    fwd, inv = [], []
    for f in (4 * m, 4 * m + 2, 8 * m + 1, 8 * m + 3):
        ang = 2.0 * np.pi * ((f * n) % 512) / 512.0
        a = np.concatenate([np.cos(ang), -np.sin(ang)], axis=0)
        wgt = np.full((128, 1), 2.0 / 512.0)
        if not fwd:
            a[64] = np.cos(np.pi * n[0])
            wgt[0] = wgt[64] = 1.0 / 512.0
        fwd.append(a[order])
        inv.append((a * wgt)[order].T)
    lane = np.arange(128)
    same_head = (lane[:, None] % H == lane[None, :] % H)
    return np.stack(fwd + inv + [same_head]).astype(np.float32)


_DFT = _dft_matrices()


def _nt(a, b):
    return jax.lax.dot_general(a, b, (((1,), (1,)), ((), ())),
                               preferred_element_type=F32)


def _nn(a, b):
    return jnp.dot(a, b, preferred_element_type=F32)


def _pack_rows(even, odd):
    return pltpu.pack_elementwise([even, odd], packed_dtype=BF16)


def _unpack(x):
    return pltpu.bitcast(x, BF16)


def _interleave(*streams):
    items = []
    for s in streams:
        total, done = sum(c for c, _ in s), 0.0
        for c, f in s:
            items.append(((done + 0.5 * c) / total, f))
            done += c
    for _, f in sorted(items, key=lambda e: e[0]):
        f()


def _kernel(x_hbm, k_hbm, v_hbm, h_hbm, w_hbm, wo_hbm,
            shift_ref, dvec_ref, gate_ref, dft_ref,
            out_hbm,
            x_v, k_v, v_v, h_v, w_v, wo_v,
            tmp_s, dft_s, xp_s, q0_s, q1_s, k0_s, k1_s, v0_s, v1_s,
            kf_s, lg_s, o0_s, o1_s, gq_s, u_s, g_s, out_s,
            w_sem, x_sem, k_sem, v_sem, h_sem, wo_sem, out_sem):
    part_fn = functools.partial

    def rows_copy(src, dst, sem, n):
        rows = pl.ds(n * BLK, BLK)
        return pltpu.make_async_copy(src.at[rows], dst.at[rows], sem.at[n])

    def cols_copy(src, dst, sem, n, size):
        cols = pl.ds(n * size, size)
        return pltpu.make_async_copy(src.at[:, cols], dst.at[:, cols], sem.at[n])

    cp_w = [cols_copy(w_hbm, w_v, w_sem, n, D) for n in range(3)]
    cp_x = [rows_copy(x_hbm, x_v, x_sem, n) for n in range(NB)]
    cp_k = [rows_copy(k_hbm, k_v, k_sem, n) for n in range(NB)]
    cp_v = [rows_copy(v_hbm, v_v, v_sem, n) for n in range(NB)]
    cp_h = [cols_copy(h_hbm, h_v, h_sem, n, BLK) for n in range(NB)]
    cp_wo = pltpu.make_async_copy(wo_hbm, wo_v, wo_sem.at[0])
    cp_out = [rows_copy(out_s, out_hbm, out_sem, n) for n in range(NB)]

    for c in (cp_w[0], cp_x[0], cp_w[1], cp_w[2], cp_k[0], cp_v[0], cp_h[0]):
        c.start()

    qkv_s = ((q0_s, k0_s, v0_s), (q1_s, k1_s, v1_s))
    o_s = (o0_s, o1_s)
    zeros = jnp.zeros((HALO, 128), F32)
    for t in range(LT):
        k0_s[t, 0:HALO, :] = zeros
        v0_s[t, 0:HALO, :] = zeros
        kf_s[t, 0:8, :] = zeros[0:8]
    for n in range(9):
        dft_s[n] = pltpu.bitcast(dft_ref[n], U32)
    shift = shift_ref[...].astype(F32)
    gate = gate_ref[...].astype(F32).reshape(1, D)
    dvec = dvec_ref[...].astype(F32).reshape(1, D)
    qscale = float(DH ** -0.5 * np.log2(np.e))

    def lanes(t):
        return slice(t * 128, (t + 1) * 128)

    w_tiles, wo_tiles, spectra = {}, {}, {}

    def permute_w_items(p):
        def ktile(kt):
            for t in range(LT):
                blk = w_v[lanes(kt), lanes(p * LT + t)].astype(F32)
                tmp_s[kt, lanes(t), :] = blk.T
            for t in range(LT):
                w_tiles[p, t, kt] = jnp.concatenate([
                    _pack_rows(*(tmp_s[kt, pl.ds(d + odd * DH, H // 2, stride=2 * DH), :]
                                 for odd in (0, 1)))
                    for d in range(4 * t, 4 * t + 4)], axis=0)

        return [(1, part_fn(ktile, kt)) for kt in range(LT)]

    def permute_wo_items():
        def ntile(t):
            tmp_s[t] = wo_v[:, lanes(t)].astype(F32)
            rows = [tmp_s[t, pl.ds(d, H, stride=DH), :] for d in range(DH)]
            wo_tiles[t] = jnp.concatenate(rows, axis=0).astype(BF16)

        return [(1, part_fn(ntile, t)) for t in range(LT)]

    def stage_x(i):
        xp_s[...] = pltpu.bitcast(x_v[i * BLK:(i + 1) * BLK, :], U32)

    def project_items(i, parts=(0, 1, 2)):
        def tile(p, t, row):
            wt = jnp.concatenate([w_tiles[p, t, kt] for kt in range(LT)], axis=1)
            acc = _nt(_unpack(xp_s[row // 2:(row + PM) // 2, :]), _unpack(wt))
            if p == 0:
                qkv_s[i % 2][0][t, row:row + PM, :] = acc * qscale
            else:
                qkv_s[i % 2][p][t, HALO + row:HALO + row + PM, :] = acc

        return [(1, part_fn(tile, p, t, row)) for p in parts for t in range(LT)
                for row in range(0, BLK, PM)]

    def halo_copy(i):
        for src, dst in zip(qkv_s[i % 2][1:], qkv_s[(i + 1) % 2][1:]):
            for t in range(LT):
                dst[t, 0:HALO, :] = src[t, BLK:BLK + HALO, :]

    def attend_items(i):
        q_s, ka_s, va_s = qkv_s[i % 2]
        rc, part = 16, 64
        keep, pending = {}, []

        def scores(row):
            qs = [q_s[t, row:row + rc, :] for t in range(LT)]
            sums = []
            for w in range(WIN):
                lo = row + HALO - DIL * w
                a = qs[0] * ka_s[0, lo:lo + rc, :]
                for t in range(1, LT):
                    a = a + qs[t] * ka_s[t, lo:lo + rc, :]
                sums.append(a)
            pending.extend(sums)
            if (row + rc) % HS == 0:
                lo = (row + rc - HS) * WIN
                lg_s[lo:lo + HS * WIN, :] = _nn(
                    jnp.concatenate(pending, axis=0).astype(BF16), _unpack(dft_s[8]))
                pending.clear()

        def gating(row):
            r0 = i * BLK + row
            xs = [x_v[r0:r0 + rc, lanes(t)].astype(F32) for t in range(LT)]
            z = xs[0] * gate[:, lanes(0)]
            for t in range(1, LT):
                z = z + xs[t] * gate[:, lanes(t)]
            th = 0.5 * jnp.tanh(0.5 * jnp.sum(z, axis=-1, keepdims=True))
            g = 0.5 + th
            for t in range(LT):
                gq_s[t, r0:r0 + rc, :] = xs[t] * g
            keep[row] = 0.5 - th

        def mix(row):
            r0 = i * BLK + row
            logits = []
            for w in range(WIN):
                a = lg_s[row * WIN + w * rc:row * WIN + (w + 1) * rc, :]
                if r0 < DIL * w:
                    pos = r0 + jax.lax.broadcasted_iota(jnp.int32, (rc, 128), 0)
                    a = jnp.where(pos >= DIL * w, a, -1e9)
                logits.append(a)
            m = logits[0]
            for w in range(1, WIN):
                m = jnp.maximum(m, logits[w])
            es = [jnp.exp2(a - m) for a in logits]
            den = es[0]
            for w in range(1, WIN):
                den = den + es[w]
            inv = pl.reciprocal(den, approx=True)
            inv = inv * (2.0 - den * inv)
            norm = keep[row] * inv
            for t in range(LT):
                a = None
                for w in range(WIN):
                    lo = row + HALO - DIL * w
                    term = es[w] * va_s[t, lo:lo + rc, :]
                    a = term if a is None else a + term
                o_s[i % 2][row // 2:(row + rc) // 2, lanes(t)] = pltpu.bitcast((a * norm).astype(BF16), U32)

        items = []
        for row in range(0, BLK + part, rc):
            if row < BLK:
                items.append((75, part_fn(gating, row)))
                items.append((155, part_fn(scores, row)))
            if row >= part:
                items.append((215, part_fn(mix, row - part)))
        return items

    def signal_items(i):
        r0 = i * BLK

        def tile(t):
            kf_s[t, r0 + 8:r0 + 8 + BLK, :] = k_v[r0:r0 + BLK, lanes(t)].astype(F32)
            pieces = [[None] * 8 for _ in range(4)]
            for r in range(4):
                xs = []
                for b in range(4):
                    at = r0 + 64 * b + 16 * r
                    ks = None
                    for j in range(KS):
                        term = kf_s[t, at + 8 - j:at + 24 - j, :] * shift[j:j + 1, lanes(t)]
                        ks = term if ks is None else ks + term
                    xs.append(ks * v_v[at:at + 16, lanes(t)].astype(F32))
                x0, x1, x2, x3 = xs
                t0, t1 = x0 - x2, x1 + x3
                w0, w1 = SQRT2 * x3, SQRT2 * x2
                res = ((x0 + x2, t1), (t0, x1 - x3),
                       (t0 - w0, t1 + w1), (t0 + w0, t1 - w1))
                for cl in range(4):
                    pieces[cl][r], pieces[cl][4 + r] = res[cl]
            for cl in range(4):
                rhs = jnp.concatenate(pieces[cl], axis=0).astype(BF16)
                u_s[i, t, cl] = _nn(_unpack(dft_s[cl]), rhs)

        return [(450, part_fn(tile, t)) for t in range(LT)]

    def filter_items(a):
        def tile(t):
            lane = jax.lax.broadcasted_iota(jnp.int32, (16, 128), 1)
            sign = jnp.where(lane < 64, -1.0, 1.0).astype(F32)
            pieces = [[] for _ in range(4)]
            for r in range(8):
                rows = slice(t * 128 + 16 * r, t * 128 + 16 * (r + 1))
                lo, hi = (h_v[rows, lanes(2 * a + n)].astype(F32) for n in (0, 1))
                if a == 0:
                    elo, ehi, olo, ohi = lo, hi, lo, hi
                else:
                    plo, phi = (h_v[rows, lanes(2 * a - 2 + n)].astype(F32) for n in (0, 1))
                    elo, ehi, olo, ohi = lo + plo, hi + phi, lo - plo, hi - phi
                tt = olo + sign * ohi
                ww = (SQRT2 * sign) * pltpu.roll(ohi, 64, 1)
                for cl, res in enumerate((elo + ehi, elo - ehi, tt + ww, tt - ww)):
                    pieces[cl].append(res)
            for cl in range(4):
                spec = _nt(_unpack(dft_s[cl]), jnp.concatenate(pieces[cl], axis=0).astype(BF16))
                if a < 2:
                    row = jax.lax.broadcasted_iota(jnp.int32, (128, 128), 0)
                    real = (row & 8) == 0
                    if cl == 0:
                        real = real | (row == 8)
                    dd = dvec[:, lanes(t)] if (a == 0 or cl < 2) else -dvec[:, lanes(t)]
                    spec = spec + jnp.where(real, dd, 0.0)
                g_s[a, t, cl] = spec

        return [(300, part_fn(tile, t)) for t in range(LT)]

    def spectrum_items(m):
        def group(t, cl):
            out = []
            for r in range(8):
                re, im = slice(16 * r, 16 * r + 8), slice(16 * r + 8, 16 * r + 16)
                yr = yi = None
                for a in range(m + 1):
                    gr, gi = g_s[a, t, cl, re, :], g_s[a, t, cl, im, :]
                    ur, ui = u_s[m - a, t, cl, re, :], u_s[m - a, t, cl, im, :]
                    ga, gb = gi, gr
                    if cl == 0 and r == 0:
                        slot0 = jax.lax.broadcasted_iota(jnp.int32, (8, 128), 0) == 0
                        ga, gb = jnp.where(slot0, 0.0, gi), jnp.where(slot0, gi, gr)
                    pr = ur * gr - ui * ga
                    pi = ur * ga + ui * gb
                    yr = pr if yr is None else yr + pr
                    yi = pi if yi is None else yi + pi
                out += [yr, yi]
            spectra[m, t, cl] = jnp.concatenate(out, axis=0).astype(BF16)

        return [(64 * (m + 1), part_fn(group, t, cl)) for t in range(LT) for cl in range(4)]

    def finish_items(m):
        def tile(t):
            rho = [_nn(_unpack(dft_s[4 + cl]), spectra[m, t, cl]) for cl in range(4)]
            (a0, a1), (b0, b1), (p0, p1), (n0, n1) = [(z[:64], z[64:]) for z in rho]
            s0, s1, d0, d1 = p0 + n0, p1 + n1, p0 - n0, p1 - n1
            ys = (a0 + b0 + s0, a1 + b1 + s1,
                  a0 - b0 - s0 + SQRT2 * d1, a1 - b1 + s1 - SQRT2 * d0)
            for row in range(0, BLK, PM):
                bb = _nn(_unpack(o_s[m % 2][row // 2:(row + PM) // 2, :]), wo_tiles[t])
                for at in range(0, PM, 64):
                    lo = m * BLK + row + at
                    res = gq_s[t, lo:lo + 64, :] * ys[(row + at) // 64] + bb[at:at + 64]
                    out_s[lo:lo + 64, lanes(t)] = res.astype(BF16)

        return [(1, part_fn(tile, t)) for t in range(LT)]

    def fetch(n):
        for c in (cp_x[n], cp_k[n], cp_v[n], cp_h[n]):
            c.start()

    for i in range(NB + 2):
        streams = []
        if i == 0:
            cp_w[0].wait()
            _interleave(permute_w_items(0))
            cp_x[0].wait()
            stage_x(0)
            cp_w[1].wait()
            _interleave(project_items(0, (0,)), permute_w_items(1))
            cp_w[2].wait()
            fetch(1)
            _interleave(project_items(0, (1,)), permute_w_items(2))
            for c in (cp_k[0], cp_v[0], cp_h[0]):
                c.wait()
            cp_wo.start()
            streams.append(project_items(0, (2,)))
        elif i < NB:
            for c in (cp_x[i], cp_k[i], cp_v[i], cp_h[i]):
                c.wait()
            if i + 1 < NB:
                fetch(i + 1)
            stage_x(i)
            streams.append(project_items(i))
        if i < NB:
            sig, fil, spec = signal_items(i), filter_items(i), spectrum_items(i)
            conv = []
            for t in range(LT + 1):
                if t < LT:
                    conv += [sig[t], fil[t]]
                if t > 0:
                    conv += spec[4 * (t - 1):4 * t]
            streams.append(conv)
        if i == 1:
            cp_wo.wait()
            streams.append(permute_wo_items())
        if 1 <= i <= NB:
            streams.append(attend_items(i - 1))
        if i >= 2:
            streams.append(finish_items(i - 2))
        _interleave(*streams)
        if i + 1 < NB:
            halo_copy(i)
        if i >= 2:
            cp_out[i - 2].start()
    for c in cp_out:
        c.wait()


@jax.jit
def pallas_gated_mix__ssm_conv_h3__sliding_local_dilated__prompt_kernel(
    A_q: jax.Array,
    A_k: jax.Array,
    A_v: jax.Array,
    A_shift_k: jax.Array,
    A_ssm_k: jax.Array,
    A_ssm_D: jax.Array,
    B_x: jax.Array,
    B_wqkv: jax.Array,
    B_wo: jax.Array,
    gate_w: jax.Array,
):
    del B_x
    hbm = pl.BlockSpec(memory_space=pl.ANY)
    vmem = pl.BlockSpec(memory_space=pltpu.VMEM)
    qkv = [pltpu.VMEM((LT, BLK, 128), F32)] * 2 + [pltpu.VMEM((LT, HALO + BLK, 128), F32)] * 4
    out = pl.pallas_call(
        _kernel,
        out_shape=jax.ShapeDtypeStruct((S, D), BF16),
        in_specs=[hbm] * 6 + [vmem] * 4,
        out_specs=hbm,
        scratch_shapes=[
            pltpu.VMEM((S, D), BF16),
            pltpu.VMEM((S, D), BF16),
            pltpu.VMEM((S, D), BF16),
            pltpu.VMEM((D, S), BF16),
            pltpu.VMEM((D, 3 * D), BF16),
            pltpu.VMEM((D, D), BF16),
            pltpu.VMEM((LT, D, 128), F32),
            pltpu.VMEM((9, 64, 128), U32),
            pltpu.VMEM((BLK // 2, D), U32),
            *qkv,
            pltpu.VMEM((LT, 8 + S, 128), F32),
            pltpu.VMEM((BLK * WIN, 128), F32),
            pltpu.VMEM((BLK // 2, D), U32),
            pltpu.VMEM((BLK // 2, D), U32),
            pltpu.VMEM((LT, S, 128), F32),
            pltpu.VMEM((NB, LT, 4, 128, 128), F32),
            pltpu.VMEM((NB, LT, 4, 128, 128), F32),
            pltpu.VMEM((S, D), BF16),
            pltpu.SemaphoreType.DMA((3,)),
            pltpu.SemaphoreType.DMA((NB,)),
            pltpu.SemaphoreType.DMA((NB,)),
            pltpu.SemaphoreType.DMA((NB,)),
            pltpu.SemaphoreType.DMA((NB,)),
            pltpu.SemaphoreType.DMA((1,)),
            pltpu.SemaphoreType.DMA((NB,)),
        ],
        compiler_params=pltpu.CompilerParams(vmem_limit_bytes=100 * 2**20),
    )(A_q.reshape(S, D), A_k.reshape(S, D), A_v.reshape(S, D), A_ssm_k, B_wqkv, B_wo,
      A_shift_k.T, A_ssm_D, gate_w, jnp.asarray(_DFT, BF16))
    return out.reshape(1, S, D)
```

```python
import functools

import numpy as np
import jax
import jax.numpy as jnp
import jax.experimental.pallas as pl
import jax.experimental.pallas.tpu as pltpu

S, D = 2048, 640
H, DH = 32, 20
WIN, DIL = 8, 2
KS = 4
LT = D // 128
BLK = 256
NB = S // BLK
HS = 64
PM = 128
HALO = 16
SQRT2 = float(np.sqrt(2.0))
F32, BF16, U32 = jnp.float32, jnp.bfloat16, jnp.uint32


def _dft_matrices():
    n = np.arange(128)[None, :]
    m = np.arange(64)[:, None]
    idx = np.arange(128)
    bins = idx.reshape(2, 8, 8).transpose(1, 0, 2).reshape(-1)
    pairs = idx.reshape(2, 64).T.reshape(-1)
    slabs = idx.reshape(2, 4, 16).transpose(1, 0, 2).reshape(-1)
    filt, sig, inv = [], [], []
    for f in (4 * m, 4 * m + 2, 8 * m + 1, 8 * m + 3):
        ang = 2.0 * np.pi * ((f * n) % 512) / 512.0
        a = np.concatenate([np.cos(ang), -np.sin(ang)], axis=0)
        wgt = np.full((128, 1), 2.0 / 512.0)
        if not filt:
            a[64] = np.cos(np.pi * n[0])
            wgt[0] = wgt[64] = 1.0 / 512.0
        filt.append(a[bins])
        sig.append(a[bins][:, pairs])
        inv.append((a * wgt)[pairs].T[slabs])
    same_head = idx[:, None] % H == idx[None, :] % H
    return np.stack(filt + inv + [same_head] + sig).astype(np.float32)


_DFT = _dft_matrices()


def _nt(a, b):
    return jax.lax.dot_general(a, b, (((1,), (1,)), ((), ())),
                               preferred_element_type=F32)


def _nn(a, b):
    return jnp.dot(a, b, preferred_element_type=F32)


def _pack_rows(even, odd):
    return pltpu.pack_elementwise([even, odd], packed_dtype=BF16)


def _unpack(x):
    return pltpu.bitcast(x, BF16)


def _interleave(*streams):
    items = []
    for s in streams:
        total, done = sum(c for c, _ in s), 0.0
        for c, f in s:
            items.append(((done + 0.5 * c) / total, f))
            done += c
    for _, f in sorted(items, key=lambda e: e[0]):
        f()


def _kernel(x_hbm, k_hbm, v_hbm, h_hbm, w_hbm, wo_hbm,
            shift_ref, dvec_ref, gate_ref, dft_ref,
            out_hbm,
            x_v, k_v, v_v, h_v, w_v, wo_v,
            tmp_s, dft_s, xp_s, q0_s, q1_s, k0_s, k1_s, v0_s, v1_s,
            kf_s, lg_s, o0_s, o1_s, gq_s, u_s, g_s, out_s,
            w_sem, x_sem, k_sem, v_sem, h_sem, wo_sem, out_sem):
    part_fn = functools.partial

    def rows_copy(src, dst, sem, n):
        rows = pl.ds(n * BLK, BLK)
        return pltpu.make_async_copy(src.at[rows], dst.at[rows], sem.at[n])

    def cols_copy(src, dst, sem, n, size):
        cols = pl.ds(n * size, size)
        return pltpu.make_async_copy(src.at[:, cols], dst.at[:, cols], sem.at[n])

    cp_w = [cols_copy(w_hbm, w_v, w_sem, n, D) for n in range(3)]
    cp_x = [rows_copy(x_hbm, x_v, x_sem, n) for n in range(NB)]
    cp_k = [rows_copy(k_hbm, k_v, k_sem, n) for n in range(NB)]
    cp_v = [rows_copy(v_hbm, v_v, v_sem, n) for n in range(NB)]
    cp_h = [cols_copy(h_hbm, h_v, h_sem, n, BLK) for n in range(NB)]
    cp_wo = pltpu.make_async_copy(wo_hbm, wo_v, wo_sem.at[0])
    cp_out = [rows_copy(out_s, out_hbm, out_sem, n) for n in range(NB)]

    for c in (cp_w[0], cp_x[0], cp_w[1], cp_w[2], cp_k[0], cp_v[0], cp_h[0]):
        c.start()

    qkv_s = ((q0_s, k0_s, v0_s), (q1_s, k1_s, v1_s))
    o_s = (o0_s, o1_s)
    zeros = jnp.zeros((HALO, 128), F32)
    for t in range(LT):
        k0_s[t, 0:HALO, :] = zeros
        v0_s[t, 0:HALO, :] = zeros
        kf_s[t, 0:8, :] = zeros[0:8]
    for n in range(13):
        dft_s[n] = pltpu.bitcast(dft_ref[n], U32)
    shift = shift_ref[...].astype(F32)
    gate = gate_ref[...].astype(F32).reshape(1, D)
    dvec = dvec_ref[...].astype(F32).reshape(1, D)
    qscale = float(DH ** -0.5 * np.log2(np.e))

    def lanes(t):
        return slice(t * 128, (t + 1) * 128)

    w_tiles, wo_tiles, spectra = {}, {}, {}

    def permute_w_items(p):
        def ktile(kt):
            for t in range(LT):
                blk = w_v[lanes(kt), lanes(p * LT + t)].astype(F32)
                tmp_s[kt, lanes(t), :] = blk.T
            for t in range(LT):
                w_tiles[p, t, kt] = jnp.concatenate([
                    _pack_rows(*(tmp_s[kt, pl.ds(d + odd * DH, H // 2, stride=2 * DH), :]
                                 for odd in (0, 1)))
                    for d in range(4 * t, 4 * t + 4)], axis=0)

        return [(1, part_fn(ktile, kt)) for kt in range(LT)]

    def permute_wo_items():
        def ntile(t):
            tmp_s[t] = wo_v[:, lanes(t)].astype(F32)
            rows = [tmp_s[t, pl.ds(d, H, stride=DH), :] for d in range(DH)]
            wo_tiles[t] = jnp.concatenate(rows, axis=0).astype(BF16)

        return [(1, part_fn(ntile, t)) for t in range(LT)]

    def stage_x(i):
        xp_s[...] = pltpu.bitcast(x_v[i * BLK:(i + 1) * BLK, :], U32)

    def project_items(i, parts=(0, 1, 2)):
        def tile(p, t, row):
            wt = jnp.concatenate([w_tiles[p, t, kt] for kt in range(LT)], axis=1)
            acc = _nt(_unpack(xp_s[row // 2:(row + PM) // 2, :]), _unpack(wt))
            if p == 0:
                qkv_s[i % 2][0][t, row:row + PM, :] = acc * qscale
            else:
                qkv_s[i % 2][p][t, HALO + row:HALO + row + PM, :] = acc

        return [(1, part_fn(tile, p, t, row)) for p in parts for t in range(LT)
                for row in range(0, BLK, PM)]

    def halo_copy(i):
        for src, dst in zip(qkv_s[i % 2][1:], qkv_s[(i + 1) % 2][1:]):
            for t in range(LT):
                dst[t, 0:HALO, :] = src[t, BLK:BLK + HALO, :]

    def attend_items(i):
        q_s, ka_s, va_s = qkv_s[i % 2]
        rc, part = 16, 64
        keep, pending = {}, []

        def scores(row):
            sums = {}
            for sub in (0, 8):
                qs = [q_s[t, row + sub:row + sub + 8, :] for t in range(LT)]
                for w in range(WIN):
                    lo = row + sub + HALO - DIL * w
                    a = qs[0] * ka_s[0, lo:lo + 8, :]
                    for t in range(1, LT):
                        a = a + qs[t] * ka_s[t, lo:lo + 8, :]
                    sums[sub, w] = a
            sums = [sums[sub, w] for sub in (0, 8) for w in range(WIN)]
            pending.extend(sums)
            if (row + rc) % HS == 0:
                lo = (row + rc - HS) * WIN
                lg_s[lo:lo + HS * WIN, :] = _nn(
                    jnp.concatenate(pending, axis=0).astype(BF16), _unpack(dft_s[8]))
                pending.clear()

        def gating(row):
            r0 = i * BLK + row
            xs = [x_v[r0:r0 + rc, lanes(t)].astype(F32) for t in range(LT)]
            z = xs[0] * gate[:, lanes(0)]
            for t in range(1, LT):
                z = z + xs[t] * gate[:, lanes(t)]
            th = 0.5 * jnp.tanh(0.5 * jnp.sum(z, axis=-1, keepdims=True))
            g = 0.5 + th
            for t in range(LT):
                gq_s[t, r0:r0 + rc, :] = xs[t] * g
            keep[row] = 0.5 - th

        def mix(row):
            r0 = i * BLK + row
            outs = []
            for sub in (0, 8):
                logits = []
                for w in range(WIN):
                    at = (row + sub + w) * WIN
                    a = lg_s[at:at + 8, :]
                    if r0 + sub < DIL * w:
                        pos = r0 + sub + jax.lax.broadcasted_iota(jnp.int32, (8, 128), 0)
                        a = jnp.where(pos >= DIL * w, a, -1e9)
                    logits.append(a)
                m = logits[0]
                for w in range(1, WIN):
                    m = jnp.maximum(m, logits[w])
                es = [jnp.exp2(a - m) for a in logits]
                den = es[0]
                for w in range(1, WIN):
                    den = den + es[w]
                inv = pl.reciprocal(den, approx=True)
                inv = inv * (2.0 - den * inv)
                norm = keep[row][sub:sub + 8] * inv
                for t in range(LT):
                    a = None
                    for w in range(WIN):
                        lo = row + sub + HALO - DIL * w
                        term = es[w] * va_s[t, lo:lo + 8, :]
                        a = term if a is None else a + term
                    outs.append(a * norm)
            for t in range(LT):
                both = jnp.concatenate([outs[t], outs[LT + t]], axis=0).astype(BF16)
                o_s[i % 2][row // 2:(row + rc) // 2, lanes(t)] = pltpu.bitcast(both, U32)

        items = []
        for row in range(0, BLK + part, rc):
            if row < BLK:
                items.append((75, part_fn(gating, row)))
                items.append((155, part_fn(scores, row)))
            if row >= part:
                items.append((215, part_fn(mix, row - part)))
        return items

    def signal_items(i):
        r0 = i * BLK

        def tile(t):
            kf_s[t, r0 + 8:r0 + 8 + BLK, :] = k_v[r0:r0 + BLK, lanes(t)].astype(F32)
            pieces = [[] for _ in range(4)]
            for r in range(8):
                xs = []
                for b in range(4):
                    at = r0 + 64 * b + 8 * r
                    ks = None
                    for j in range(KS):
                        term = kf_s[t, at + 8 - j:at + 16 - j, :] * shift[j:j + 1, lanes(t)]
                        ks = term if ks is None else ks + term
                    xs.append(ks * v_v[at:at + 8, lanes(t)].astype(F32))
                x0, x1, x2, x3 = xs
                t0, t1 = x0 - x2, x1 + x3
                w0, w1 = SQRT2 * x3, SQRT2 * x2
                res = ((x0 + x2, t1), (t0, x1 - x3),
                       (t0 - w0, t1 + w1), (t0 + w0, t1 - w1))
                for cl in range(4):
                    pieces[cl].append(_pack_rows(*res[cl]))
            for cl in range(4):
                rhs = _unpack(jnp.concatenate(pieces[cl], axis=0))
                u_s[i, t, cl] = _nn(_unpack(dft_s[9 + cl]), rhs)

        return [(450, part_fn(tile, t)) for t in range(LT)]

    def filter_items(a):
        def tile(t):
            lane = jax.lax.broadcasted_iota(jnp.int32, (16, 128), 1)
            sign = jnp.where(lane < 64, -1.0, 1.0).astype(F32)
            pieces = [[] for _ in range(4)]
            for r in range(8):
                rows = slice(t * 128 + 16 * r, t * 128 + 16 * (r + 1))
                lo, hi = (h_v[rows, lanes(2 * a + n)].astype(F32) for n in (0, 1))
                if a == 0:
                    elo, ehi, olo, ohi = lo, hi, lo, hi
                else:
                    plo, phi = (h_v[rows, lanes(2 * a - 2 + n)].astype(F32) for n in (0, 1))
                    elo, ehi, olo, ohi = lo + plo, hi + phi, lo - plo, hi - phi
                tt = olo + sign * ohi
                ww = (SQRT2 * sign) * pltpu.roll(ohi, 64, 1)
                for cl, res in enumerate((elo + ehi, elo - ehi, tt + ww, tt - ww)):
                    pieces[cl].append(res)
            for cl in range(4):
                spec = _nt(_unpack(dft_s[cl]), jnp.concatenate(pieces[cl], axis=0).astype(BF16))
                if a < 2:
                    row = jax.lax.broadcasted_iota(jnp.int32, (128, 128), 0)
                    real = (row & 8) == 0
                    if cl == 0:
                        real = real | (row == 8)
                    dd = dvec[:, lanes(t)] if (a == 0 or cl < 2) else -dvec[:, lanes(t)]
                    spec = spec + jnp.where(real, dd, 0.0)
                g_s[a, t, cl] = spec

        return [(300, part_fn(tile, t)) for t in range(LT)]

    def spectrum_items(m):
        def group(t, cl):
            out = []
            for r in range(8):
                re, im = slice(16 * r, 16 * r + 8), slice(16 * r + 8, 16 * r + 16)
                yr = yi = None
                for a in range(m + 1):
                    gr, gi = g_s[a, t, cl, re, :], g_s[a, t, cl, im, :]
                    ur, ui = u_s[m - a, t, cl, re, :], u_s[m - a, t, cl, im, :]
                    ga, gb = gi, gr
                    if cl == 0 and r == 0:
                        slot0 = jax.lax.broadcasted_iota(jnp.int32, (8, 128), 0) == 0
                        ga, gb = jnp.where(slot0, 0.0, gi), jnp.where(slot0, gi, gr)
                    pr = ur * gr - ui * ga
                    pi = ur * ga + ui * gb
                    yr = pr if yr is None else yr + pr
                    yi = pi if yi is None else yi + pi
                out.append(_pack_rows(yr, yi))
            spectra[m, t, cl] = jnp.concatenate(out, axis=0)

        return [(64 * (m + 1), part_fn(group, t, cl)) for t in range(LT) for cl in range(4)]

    def finish_items(m):
        def tile(t):
            rho = [_nn(_unpack(dft_s[4 + cl]), _unpack(spectra[m, t, cl])) for cl in range(4)]
            for r0 in range(0, 4, PM // 64):
                lhs = jnp.concatenate(
                    [o_s[m % 2][32 * b + 8 * r:32 * b + 8 * (r + 1), :]
                     for r in range(r0, r0 + PM // 64) for b in range(4)], axis=0)
                bb = _nn(_unpack(lhs), wo_tiles[t])
                for r in range(r0, r0 + PM // 64):
                    (a0, a1), (b0, b1), (p0, p1), (n0, n1) = [
                        (z[32 * r:32 * r + 16], z[32 * r + 16:32 * (r + 1)]) for z in rho]
                    s0, s1, d0, d1 = p0 + n0, p1 + n1, p0 - n0, p1 - n1
                    ys = (a0 + b0 + s0, a1 + b1 + s1,
                          a0 - b0 - s0 + SQRT2 * d1, a1 - b1 + s1 - SQRT2 * d0)
                    for b in range(4):
                        lo = m * BLK + 64 * b + 16 * r
                        at = 64 * (r - r0) + 16 * b
                        res = gq_s[t, lo:lo + 16, :] * ys[b] + bb[at:at + 16]
                        out_s[lo:lo + 16, lanes(t)] = res.astype(BF16)

        return [(1, part_fn(tile, t)) for t in range(LT)]

    def fetch(n):
        for c in (cp_x[n], cp_k[n], cp_v[n], cp_h[n]):
            c.start()

    for i in range(NB + 2):
        streams = []
        if i == 0:
            cp_w[0].wait()
            _interleave(permute_w_items(0))
            cp_x[0].wait()
            stage_x(0)
            cp_w[1].wait()
            _interleave(project_items(0, (0,)), permute_w_items(1))
            cp_w[2].wait()
            fetch(1)
            _interleave(project_items(0, (1,)), permute_w_items(2))
            for c in (cp_k[0], cp_v[0], cp_h[0]):
                c.wait()
            cp_wo.start()
            streams.append(project_items(0, (2,)))
        elif i < NB:
            for c in (cp_x[i], cp_k[i], cp_v[i], cp_h[i]):
                c.wait()
            if i + 1 < NB:
                fetch(i + 1)
            stage_x(i)
            streams.append(project_items(i))
        if i < NB:
            sig, fil, spec = signal_items(i), filter_items(i), spectrum_items(i)
            conv = []
            for t in range(LT + 1):
                if t < LT:
                    conv += [sig[t], fil[t]]
                if t > 0:
                    conv += spec[4 * (t - 1):4 * t]
            streams.append(conv)
        if i == 1:
            cp_wo.wait()
            streams.append(permute_wo_items())
        if 1 <= i <= NB:
            streams.append(attend_items(i - 1))
        if i >= 2:
            streams.append(finish_items(i - 2))
        _interleave(*streams)
        if i + 1 < NB:
            halo_copy(i)
        if i >= 2:
            cp_out[i - 2].start()
    for c in cp_out:
        c.wait()


@jax.jit
def pallas_gated_mix__ssm_conv_h3__sliding_local_dilated__prompt_kernel(
    A_q: jax.Array,
    A_k: jax.Array,
    A_v: jax.Array,
    A_shift_k: jax.Array,
    A_ssm_k: jax.Array,
    A_ssm_D: jax.Array,
    B_x: jax.Array,
    B_wqkv: jax.Array,
    B_wo: jax.Array,
    gate_w: jax.Array,
):
    del B_x
    hbm = pl.BlockSpec(memory_space=pl.ANY)
    vmem = pl.BlockSpec(memory_space=pltpu.VMEM)
    qkv = [pltpu.VMEM((LT, BLK, 128), F32)] * 2 + [pltpu.VMEM((LT, HALO + BLK, 128), F32)] * 4
    out = pl.pallas_call(
        _kernel,
        out_shape=jax.ShapeDtypeStruct((S, D), BF16),
        in_specs=[hbm] * 6 + [vmem] * 4,
        out_specs=hbm,
        scratch_shapes=[
            pltpu.VMEM((S, D), BF16),
            pltpu.VMEM((S, D), BF16),
            pltpu.VMEM((S, D), BF16),
            pltpu.VMEM((D, S), BF16),
            pltpu.VMEM((D, 3 * D), BF16),
            pltpu.VMEM((D, D), BF16),
            pltpu.VMEM((LT, D, 128), F32),
            pltpu.VMEM((13, 64, 128), U32),
            pltpu.VMEM((BLK // 2, D), U32),
            *qkv,
            pltpu.VMEM((LT, 8 + S, 128), F32),
            pltpu.VMEM((BLK * WIN, 128), F32),
            pltpu.VMEM((BLK // 2, D), U32),
            pltpu.VMEM((BLK // 2, D), U32),
            pltpu.VMEM((LT, S, 128), F32),
            pltpu.VMEM((NB, LT, 4, 128, 128), F32),
            pltpu.VMEM((NB, LT, 4, 128, 128), F32),
            pltpu.VMEM((S, D), BF16),
            pltpu.SemaphoreType.DMA((3,)),
            pltpu.SemaphoreType.DMA((NB,)),
            pltpu.SemaphoreType.DMA((NB,)),
            pltpu.SemaphoreType.DMA((NB,)),
            pltpu.SemaphoreType.DMA((NB,)),
            pltpu.SemaphoreType.DMA((1,)),
            pltpu.SemaphoreType.DMA((NB,)),
        ],
        compiler_params=pltpu.CompilerParams(vmem_limit_bytes=100 * 2**20),
    )(A_q.reshape(S, D), A_k.reshape(S, D), A_v.reshape(S, D), A_ssm_k, B_wqkv, B_wo,
      A_shift_k.T, A_ssm_D, gate_w, jnp.asarray(_DFT, BF16))
    return out.reshape(1, S, D)
```

```python
import functools

import numpy as np
import jax
import jax.numpy as jnp
import jax.experimental.pallas as pl
import jax.experimental.pallas.tpu as pltpu

S, D = 2048, 640
H, DH = 32, 20
WIN, DIL = 8, 2
KS = 4
LT = D // 128
BLK = 256
NB = S // BLK
REGIONS = 1
SPAN_PROJECT = (0.0, 1.0)
SPAN_CONV = (0.0, 1.05)
SPAN_ATTEND = (0.05, 1.05)
SPAN_FINISH = (0.0, 1.0)
HS = 64
PM = 128
HALO = 16
SQRT2 = float(np.sqrt(2.0))
F32, BF16, U32 = jnp.float32, jnp.bfloat16, jnp.uint32


def _dft_matrices():
    n = np.arange(128)[None, :]
    m = np.arange(64)[:, None]
    idx = np.arange(128)
    bins = idx.reshape(2, 8, 8).transpose(1, 0, 2).reshape(-1)
    pairs = idx.reshape(2, 64).T.reshape(-1)
    slabs = idx.reshape(2, 4, 16).transpose(1, 0, 2).reshape(-1)
    filt, sig, inv = [], [], []
    for f in (4 * m, 4 * m + 2, 8 * m + 1, 8 * m + 3):
        ang = 2.0 * np.pi * ((f * n) % 512) / 512.0
        a = np.concatenate([np.cos(ang), -np.sin(ang)], axis=0)
        wgt = np.full((128, 1), 2.0 / 512.0)
        if not filt:
            a[64] = np.cos(np.pi * n[0])
            wgt[0] = wgt[64] = 1.0 / 512.0
        filt.append(a[bins])
        sig.append(a[bins][:, pairs])
        inv.append((a * wgt)[pairs].T[slabs])
    same_head = idx[:, None] % H == idx[None, :] % H
    return np.stack(filt + inv + [same_head] + sig).astype(np.float32)


_DFT = _dft_matrices()


def _nt(a, b):
    return jax.lax.dot_general(a, b, (((1,), (1,)), ((), ())),
                               preferred_element_type=F32)


def _nn(a, b):
    return jnp.dot(a, b, preferred_element_type=F32)


def _pack_rows(even, odd):
    return pltpu.pack_elementwise([even, odd], packed_dtype=BF16)


def _unpack(x):
    return pltpu.bitcast(x, BF16)


def _interleave(*streams, spans=None):
    items = []
    for n, s in enumerate(streams):
        lo, hi = (spans or {}).get(n, (0.0, 1.0))
        total, done = sum(c for c, _ in s), 0.0
        for c, f in s:
            items.append((lo + (hi - lo) * (done + 0.5 * c) / total, f))
            done += c
    for _, f in sorted(items, key=lambda e: e[0]):
        f()


def _kernel(x_hbm, k_hbm, v_hbm, h_hbm, w_hbm, wo_hbm,
            shift_ref, dvec_ref, gate_ref, dft_ref,
            out_hbm,
            x_v, k_v, v_v, h_v, w_v, wo_v,
            tmp_s, dft_s, xp_s, q_s, ka_s, va_s,
            kf_s, lg_s, o0_s, o1_s, gq_s, u_s, g_s, out_s,
            w_sem, x_sem, k_sem, v_sem, h_sem, wo_sem, out_sem, fence_sem):
    part_fn = functools.partial

    def rows_copy(src, dst, sem, n):
        rows = pl.ds(n * BLK, BLK)
        return pltpu.make_async_copy(src.at[rows], dst.at[rows], sem.at[n])

    def cols_copy(src, dst, sem, n, size):
        cols = pl.ds(n * size, size)
        return pltpu.make_async_copy(src.at[:, cols], dst.at[:, cols], sem.at[n])

    cp_w = [cols_copy(w_hbm, w_v, w_sem, n, D) for n in range(3)]
    cp_x = [rows_copy(x_hbm, x_v, x_sem, n) for n in range(NB)]
    cp_k = [rows_copy(k_hbm, k_v, k_sem, n) for n in range(NB)]
    cp_v = [rows_copy(v_hbm, v_v, v_sem, n) for n in range(NB)]
    cp_h = [cols_copy(h_hbm, h_v, h_sem, n, BLK) for n in range(NB)]
    cp_wo = pltpu.make_async_copy(wo_hbm, wo_v, wo_sem.at[0])
    cp_out = [rows_copy(out_s, out_hbm, out_sem, n) for n in range(NB)]

    for c in (cp_w[0], cp_x[0], cp_w[1], cp_w[2], cp_k[0], cp_v[0], cp_h[0]):
        c.start()

    o_s = (o0_s, o1_s)
    zeros = jnp.zeros((HALO, 128), F32)
    for t in range(LT):
        ka_s[t, 0:HALO, :] = zeros
        va_s[t, 0:HALO, :] = zeros
        kf_s[t, 0:8, :] = zeros[0:8]
    for n in range(13):
        dft_s[n] = pltpu.bitcast(dft_ref[n], U32)
    shift = shift_ref[...].astype(F32)
    gate = gate_ref[...].astype(F32).reshape(1, D)
    dvec = dvec_ref[...].astype(F32).reshape(1, D)
    qscale = float(DH ** -0.5 * np.log2(np.e))

    def lanes(t):
        return slice(t * 128, (t + 1) * 128)

    w_tiles, wo_tiles, spectra = {}, {}, {}

    def permute_w_items(p):
        def ktile(kt):
            for t in range(LT):
                blk = w_v[lanes(kt), lanes(p * LT + t)].astype(F32)
                tmp_s[kt, lanes(t), :] = blk.T
            for t in range(LT):
                w_tiles[p, t, kt] = jnp.concatenate([
                    _pack_rows(*(tmp_s[kt, pl.ds(d + odd * DH, H // 2, stride=2 * DH), :]
                                 for odd in (0, 1)))
                    for d in range(4 * t, 4 * t + 4)], axis=0)

        return [(1, part_fn(ktile, kt)) for kt in range(LT)]

    def permute_wo_items():
        def ntile(t):
            tmp_s[t] = wo_v[:, lanes(t)].astype(F32)
            rows = [tmp_s[t, pl.ds(d, H, stride=DH), :] for d in range(DH)]
            wo_tiles[t] = jnp.concatenate(rows, axis=0).astype(BF16)

        return [(1, part_fn(ntile, t)) for t in range(LT)]

    def stage_x(i):
        xp_s[i % 2] = pltpu.bitcast(x_v[i * BLK:(i + 1) * BLK, :], U32)

    def project_items(i, parts=(0, 1, 2)):
        def tile(p, t, row):
            wt = jnp.concatenate([w_tiles[p, t, kt] for kt in range(LT)], axis=1)
            acc = _nt(_unpack(xp_s[i % 2, row // 2:(row + PM) // 2, :]), _unpack(wt))
            at = i * BLK + row
            if p == 0:
                q_s[t, at:at + PM, :] = acc * qscale
            else:
                (ka_s, va_s)[p - 1][t, HALO + at:HALO + at + PM, :] = acc

        return [(1, part_fn(tile, p, t, row)) for p in parts for t in range(LT)
                for row in range(0, BLK, PM)]

    def attend_items(i):
        rc, part = 16, 64
        keep, pending = {}, []

        def scores(row):
            sums = {}
            for sub in (0, 8):
                at = i * BLK + row + sub
                qs = [q_s[t, at:at + 8, :] for t in range(LT)]
                for w in range(WIN):
                    lo = at + HALO - DIL * w
                    a = qs[0] * ka_s[0, lo:lo + 8, :]
                    for t in range(1, LT):
                        a = a + qs[t] * ka_s[t, lo:lo + 8, :]
                    sums[sub, w] = a
            sums = [sums[sub, w] for sub in (0, 8) for w in range(WIN)]
            pending.extend(sums)
            if (row + rc) % HS == 0:
                lo = (row + rc - HS) * WIN
                lg_s[lo:lo + HS * WIN, :] = _nn(
                    jnp.concatenate(pending, axis=0).astype(BF16), _unpack(dft_s[8]))
                pending.clear()

        def gating(row):
            r0 = i * BLK + row
            xs = [x_v[r0:r0 + rc, lanes(t)].astype(F32) for t in range(LT)]
            z = xs[0] * gate[:, lanes(0)]
            for t in range(1, LT):
                z = z + xs[t] * gate[:, lanes(t)]
            th = 0.5 * jnp.tanh(0.5 * jnp.sum(z, axis=-1, keepdims=True))
            g = 0.5 + th
            for t in range(LT):
                gq_s[t, r0:r0 + rc, :] = xs[t] * g
            keep[row] = 0.5 - th

        def mix(row):
            r0 = i * BLK + row
            outs = []
            for sub in (0, 8):
                logits = []
                for w in range(WIN):
                    at = (row + sub + w) * WIN
                    a = lg_s[at:at + 8, :]
                    if r0 + sub < DIL * w:
                        pos = r0 + sub + jax.lax.broadcasted_iota(jnp.int32, (8, 128), 0)
                        a = jnp.where(pos >= DIL * w, a, -1e9)
                    logits.append(a)
                m = logits[0]
                for w in range(1, WIN):
                    m = jnp.maximum(m, logits[w])
                es = [jnp.exp2(a - m) for a in logits]
                den = es[0]
                for w in range(1, WIN):
                    den = den + es[w]
                inv = pl.reciprocal(den, approx=True)
                inv = inv * (2.0 - den * inv)
                norm = keep[row][sub:sub + 8] * inv
                for t in range(LT):
                    a = None
                    for w in range(WIN):
                        lo = r0 + sub + HALO - DIL * w
                        term = es[w] * va_s[t, lo:lo + 8, :]
                        a = term if a is None else a + term
                    outs.append(a * norm)
            for t in range(LT):
                both = jnp.concatenate([outs[t], outs[LT + t]], axis=0).astype(BF16)
                o_s[i % 2][row // 2:(row + rc) // 2, lanes(t)] = pltpu.bitcast(both, U32)

        items = []
        for row in range(0, BLK + part, rc):
            if row < BLK:
                items.append((75, part_fn(gating, row)))
                items.append((155, part_fn(scores, row)))
            if row >= part:
                items.append((215, part_fn(mix, row - part)))
        return items

    def signal_items(i):
        r0 = i * BLK

        def tile(t):
            kf_s[t, r0 + 8:r0 + 8 + BLK, :] = k_v[r0:r0 + BLK, lanes(t)].astype(F32)
            pieces = [[] for _ in range(4)]
            for r in range(8):
                xs = []
                for b in range(4):
                    at = r0 + 64 * b + 8 * r
                    ks = None
                    for j in range(KS):
                        term = kf_s[t, at + 8 - j:at + 16 - j, :] * shift[j:j + 1, lanes(t)]
                        ks = term if ks is None else ks + term
                    xs.append(ks * v_v[at:at + 8, lanes(t)].astype(F32))
                x0, x1, x2, x3 = xs
                t0, t1 = x0 - x2, x1 + x3
                w0, w1 = SQRT2 * x3, SQRT2 * x2
                res = ((x0 + x2, t1), (t0, x1 - x3),
                       (t0 - w0, t1 + w1), (t0 + w0, t1 - w1))
                for cl in range(4):
                    pieces[cl].append(_pack_rows(*res[cl]))
            for cl in range(4):
                rhs = _unpack(jnp.concatenate(pieces[cl], axis=0))
                u_s[i, t, cl] = _nn(_unpack(dft_s[9 + cl]), rhs)

        return [(450, part_fn(tile, t)) for t in range(LT)]

    def filter_items(a):
        def tile(t):
            lane = jax.lax.broadcasted_iota(jnp.int32, (16, 128), 1)
            sign = jnp.where(lane < 64, -1.0, 1.0).astype(F32)
            pieces = [[] for _ in range(4)]
            for r in range(8):
                rows = slice(t * 128 + 16 * r, t * 128 + 16 * (r + 1))
                lo, hi = (h_v[rows, lanes(2 * a + n)].astype(F32) for n in (0, 1))
                if a == 0:
                    elo, ehi, olo, ohi = lo, hi, lo, hi
                else:
                    plo, phi = (h_v[rows, lanes(2 * a - 2 + n)].astype(F32) for n in (0, 1))
                    elo, ehi, olo, ohi = lo + plo, hi + phi, lo - plo, hi - phi
                tt = olo + sign * ohi
                ww = (SQRT2 * sign) * pltpu.roll(ohi, 64, 1)
                for cl, res in enumerate((elo + ehi, elo - ehi, tt + ww, tt - ww)):
                    pieces[cl].append(res)
            for cl in range(4):
                spec = _nt(_unpack(dft_s[cl]), jnp.concatenate(pieces[cl], axis=0).astype(BF16))
                if a < 2:
                    row = jax.lax.broadcasted_iota(jnp.int32, (128, 128), 0)
                    real = (row & 8) == 0
                    if cl == 0:
                        real = real | (row == 8)
                    dd = dvec[:, lanes(t)] if (a == 0 or cl < 2) else -dvec[:, lanes(t)]
                    spec = spec + jnp.where(real, dd, 0.0)
                g_s[a, t, cl] = spec

        return [(300, part_fn(tile, t)) for t in range(LT)]

    def spectrum_items(m):
        def group(t, cl):
            out = []
            for r in range(8):
                re, im = slice(16 * r, 16 * r + 8), slice(16 * r + 8, 16 * r + 16)
                yr = yi = None
                for a in range(m + 1):
                    gr, gi = g_s[a, t, cl, re, :], g_s[a, t, cl, im, :]
                    ur, ui = u_s[m - a, t, cl, re, :], u_s[m - a, t, cl, im, :]
                    ga, gb = gi, gr
                    if cl == 0 and r == 0:
                        slot0 = jax.lax.broadcasted_iota(jnp.int32, (8, 128), 0) == 0
                        ga, gb = jnp.where(slot0, 0.0, gi), jnp.where(slot0, gi, gr)
                    pr = ur * gr - ui * ga
                    pi = ur * ga + ui * gb
                    yr = pr if yr is None else yr + pr
                    yi = pi if yi is None else yi + pi
                out.append(_pack_rows(yr, yi))
            spectra[m, t, cl] = jnp.concatenate(out, axis=0)

        return [(64 * (m + 1), part_fn(group, t, cl)) for t in range(LT) for cl in range(4)]

    def finish_items(m):
        def tile(t):
            rho = [_nn(_unpack(dft_s[4 + cl]), _unpack(spectra[m, t, cl])) for cl in range(4)]
            for r0 in range(0, 4, PM // 64):
                lhs = jnp.concatenate(
                    [o_s[m % 2][32 * b + 8 * r:32 * b + 8 * (r + 1), :]
                     for r in range(r0, r0 + PM // 64) for b in range(4)], axis=0)
                bb = _nn(_unpack(lhs), wo_tiles[t])
                for r in range(r0, r0 + PM // 64):
                    (a0, a1), (b0, b1), (p0, p1), (n0, n1) = [
                        (z[32 * r:32 * r + 16], z[32 * r + 16:32 * (r + 1)]) for z in rho]
                    s0, s1, d0, d1 = p0 + n0, p1 + n1, p0 - n0, p1 - n1
                    ys = (a0 + b0 + s0, a1 + b1 + s1,
                          a0 - b0 - s0 + SQRT2 * d1, a1 - b1 + s1 - SQRT2 * d0)
                    for b in range(4):
                        lo = m * BLK + 64 * b + 16 * r
                        at = 64 * (r - r0) + 16 * b
                        res = gq_s[t, lo:lo + 16, :] * ys[b] + bb[at:at + 16]
                        out_s[lo:lo + 16, lanes(t)] = res.astype(BF16)

        return [(1, part_fn(tile, t)) for t in range(LT)]

    batches = {n: (n,) for n in range(1, NB)}
    stores = {n + 2: (n,) for n in range(NB)}

    def fence():
        pl.semaphore_signal(fence_sem, 1)
        pl.semaphore_wait(fence_sem, 1)

    def batch(i):
        return [c[n] for n in batches[i] for c in (cp_x, cp_k, cp_v, cp_h)]

    for i in range(NB + 2):
        streams, spans = [], {}
        if i == 0:
            cp_w[0].wait()
            _interleave(permute_w_items(0))
            cp_x[0].wait()
            stage_x(0)
            cp_w[1].wait()
            _interleave(project_items(0, (0,)), permute_w_items(1))
            cp_w[2].wait()
            for c in batch(1):
                c.start()
            _interleave(project_items(0, (1,)), permute_w_items(2))
            for c in (cp_k[0], cp_v[0], cp_h[0]):
                c.wait()
            cp_wo.start()
            streams.append(project_items(0, (2,)))
        elif i < NB:
            if i in batches:
                for c in batch(i):
                    c.wait()
                later = [j for j in sorted(batches) if j > i]
                if later:
                    for c in batch(later[0]):
                        c.start()
                stage_x(i)
            spans[len(streams)] = SPAN_PROJECT
            streams.append(project_items(i))
            if i + 1 < NB and i + 1 not in batches:
                streams[0].insert(len(streams[0]) * 3 // 4, (0.2, part_fn(stage_x, i + 1)))
        if i < NB:
            sig, fil, spec = signal_items(i), filter_items(i), spectrum_items(i)
            conv = []
            for t in range(LT + 1):
                if t < LT:
                    conv += [sig[t], fil[t]]
                if t > 0:
                    conv += spec[4 * (t - 1):4 * t]
            spans[len(streams)] = SPAN_CONV
            streams.append(conv)
        if i == 1:
            cp_wo.wait()
            streams.append(permute_wo_items())
        if 1 <= i <= NB:
            spans[len(streams)] = SPAN_ATTEND
            streams.append(attend_items(i - 1))
        if i >= 2:
            spans[len(streams)] = SPAN_FINISH
            streams.append(finish_items(i - 2))
        if REGIONS > 1 and 1 <= i < NB:
            streams.append([(0.5, lambda: None)] + [(1, fence)] * (REGIONS - 1) + [(0.5, lambda: None)])
        _interleave(*streams, spans=spans)
        for n in stores.get(i, ()):
            cp_out[n].start()
    for c in cp_out:
        c.wait()


@jax.jit
def pallas_gated_mix__ssm_conv_h3__sliding_local_dilated__prompt_kernel(
    A_q: jax.Array,
    A_k: jax.Array,
    A_v: jax.Array,
    A_shift_k: jax.Array,
    A_ssm_k: jax.Array,
    A_ssm_D: jax.Array,
    B_x: jax.Array,
    B_wqkv: jax.Array,
    B_wo: jax.Array,
    gate_w: jax.Array,
):
    del B_x
    hbm = pl.BlockSpec(memory_space=pl.ANY)
    vmem = pl.BlockSpec(memory_space=pltpu.VMEM)
    out = pl.pallas_call(
        _kernel,
        out_shape=jax.ShapeDtypeStruct((S, D), BF16),
        in_specs=[hbm] * 6 + [vmem] * 4,
        out_specs=hbm,
        scratch_shapes=[
            pltpu.VMEM((S, D), BF16),
            pltpu.VMEM((S, D), BF16),
            pltpu.VMEM((S, D), BF16),
            pltpu.VMEM((D, S), BF16),
            pltpu.VMEM((D, 3 * D), BF16),
            pltpu.VMEM((D, D), BF16),
            pltpu.VMEM((LT, D, 128), F32),
            pltpu.VMEM((13, 64, 128), U32),
            pltpu.VMEM((2, BLK // 2, D), U32),
            pltpu.VMEM((LT, S, 128), F32),
            pltpu.VMEM((LT, HALO + S, 128), F32),
            pltpu.VMEM((LT, HALO + S, 128), F32),
            pltpu.VMEM((LT, 8 + S, 128), F32),
            pltpu.VMEM((BLK * WIN, 128), F32),
            pltpu.VMEM((BLK // 2, D), U32),
            pltpu.VMEM((BLK // 2, D), U32),
            pltpu.VMEM((LT, S, 128), F32),
            pltpu.VMEM((NB, LT, 4, 128, 128), F32),
            pltpu.VMEM((NB, LT, 4, 128, 128), F32),
            pltpu.VMEM((S, D), BF16),
            pltpu.SemaphoreType.DMA((3,)),
            pltpu.SemaphoreType.DMA((NB,)),
            pltpu.SemaphoreType.DMA((NB,)),
            pltpu.SemaphoreType.DMA((NB,)),
            pltpu.SemaphoreType.DMA((NB,)),
            pltpu.SemaphoreType.DMA((1,)),
            pltpu.SemaphoreType.DMA((NB,)),
            pltpu.SemaphoreType.REGULAR,
        ],
        compiler_params=pltpu.CompilerParams(vmem_limit_bytes=100 * 2**20),
    )(A_q.reshape(S, D), A_k.reshape(S, D), A_v.reshape(S, D), A_ssm_k, B_wqkv, B_wo,
      A_shift_k.T, A_ssm_D, gate_w, jnp.asarray(_DFT, BF16))
    return out.reshape(1, S, D)
```

```python
import functools

import numpy as np
import jax
import jax.numpy as jnp
import jax.experimental.pallas as pl
import jax.experimental.pallas.tpu as pltpu

S, D = 2048, 640
H, DH = 32, 20
WIN, DIL = 8, 2
KS = 4
LT = D // 128
BLK = 256
NB = S // BLK
SPAN_PROJECT = (0.0, 1.0)
SPAN_CONV = (0.0, 1.05)
SPAN_ATTEND = (0.05, 1.05)
SPAN_FINISH = (0.0, 1.0)
HS = 64
PM = 128
HALO = 16
SQRT2 = float(np.sqrt(2.0))
F32, BF16, U32 = jnp.float32, jnp.bfloat16, jnp.uint32


def _dft_matrices():
    n = np.arange(128)[None, :]
    m = np.arange(64)[:, None]
    idx = np.arange(128)
    bins = idx.reshape(2, 8, 8).transpose(1, 0, 2).reshape(-1)
    pairs = idx.reshape(2, 64).T.reshape(-1)
    slabs = idx.reshape(2, 4, 16).transpose(1, 0, 2).reshape(-1)
    filt, sig, inv = [], [], []
    for f in (4 * m, 4 * m + 2, 8 * m + 1, 8 * m + 3):
        ang = 2.0 * np.pi * ((f * n) % 512) / 512.0
        a = np.concatenate([np.cos(ang), -np.sin(ang)], axis=0)
        wgt = np.full((128, 1), 2.0 / 512.0)
        if not filt:
            a[64] = np.cos(np.pi * n[0])
            wgt[0] = wgt[64] = 1.0 / 512.0
        filt.append(a[bins])
        sig.append(a[bins][:, pairs])
        inv.append((a * wgt)[pairs].T[slabs])
    same_head = idx[:, None] % H == idx[None, :] % H
    return np.stack(filt + inv + [same_head] + sig).astype(np.float32)


_DFT = _dft_matrices()


def _nt(a, b):
    return jax.lax.dot_general(a, b, (((1,), (1,)), ((), ())),
                               preferred_element_type=F32)


def _nn(a, b):
    return jnp.dot(a, b, preferred_element_type=F32)


def _pack_rows(even, odd):
    return pltpu.pack_elementwise([even, odd], packed_dtype=BF16)


def _unpack(x):
    return pltpu.bitcast(x, BF16)


def _interleave(*streams, spans=None):
    items = []
    for n, s in enumerate(streams):
        lo, hi = (spans or {}).get(n, (0.0, 1.0))
        total, done = sum(c for c, _ in s), 0.0
        for c, f in s:
            items.append((lo + (hi - lo) * (done + 0.5 * c) / total, f))
            done += c
    for _, f in sorted(items, key=lambda e: e[0]):
        f()


def _kernel(x_hbm, k_hbm, v_hbm, h_hbm, w_hbm, wo_hbm,
            shift_hbm, dvec_hbm, gate_hbm, dft_hbm,
            out_hbm,
            x_v, k_v, v_v, h_v, w_v, wo_v, shift_ref, dvec_ref, gate_ref, dft_ref,
            tmp_s, dft_s, xp_s, q_s, ka_s, va_s,
            kf_s, lg_s, o0_s, o1_s, gq_s, u_s, g_s, out_s,
            w_sem, x_sem, k_sem, v_sem, h_sem, wo_sem, out_sem, small_sem):
    part_fn = functools.partial

    def rows_copy(src, dst, sem, n):
        rows = pl.ds(n * BLK, BLK)
        return pltpu.make_async_copy(src.at[rows], dst.at[rows], sem.at[n])

    def cols_copy(src, dst, sem, n, size):
        cols = pl.ds(n * size, size)
        return pltpu.make_async_copy(src.at[:, cols], dst.at[:, cols], sem.at[n])

    cp_w = [cols_copy(w_hbm, w_v, w_sem, n, D) for n in range(3)]
    cp_x = [rows_copy(x_hbm, x_v, x_sem, n) for n in range(NB)]
    cp_k = [rows_copy(k_hbm, k_v, k_sem, n) for n in range(NB)]
    cp_v = [rows_copy(v_hbm, v_v, v_sem, n) for n in range(NB)]
    cp_h = [cols_copy(h_hbm, h_v, h_sem, n, BLK) for n in range(NB)]
    cp_wo = pltpu.make_async_copy(wo_hbm, wo_v, wo_sem.at[0])
    cp_out = [rows_copy(out_s, out_hbm, out_sem, n) for n in range(NB)]

    cp_small = [
        pltpu.make_async_copy(src, dst, small_sem.at[n])
        for n, (src, dst) in enumerate(((shift_hbm, shift_ref), (dvec_hbm, dvec_ref),
                                        (gate_hbm, gate_ref), (dft_hbm, dft_ref)))]

    cp_w[0].start()
    cp_x[0].start()
    cp_w[1].start()

    o_s = (o0_s, o1_s)
    zeros = jnp.zeros((HALO, 128), F32)
    for t in range(LT):
        ka_s[t, 0:HALO, :] = zeros
        va_s[t, 0:HALO, :] = zeros
        kf_s[t, 0:8, :] = zeros[0:8]
    vec = {}

    def load_constants():
        for n in range(_DFT.shape[0]):
            dft_s[n] = pltpu.bitcast(dft_ref[n], U32)
        vec["shift"] = shift_ref[...].astype(F32)
        vec["gate"] = gate_ref[...].astype(F32).reshape(1, D)
        vec["skip"] = dvec_ref[...].astype(F32).reshape(1, D)

    qscale = float(DH ** -0.5 * np.log2(np.e))

    def lanes(t):
        return slice(t * 128, (t + 1) * 128)

    w_tiles, wo_tiles, spectra = {}, {}, {}

    def permute_w_items(p):
        def ktile(kt):
            for t in range(LT):
                blk = w_v[lanes(kt), lanes(p * LT + t)].astype(F32)
                tmp_s[kt, lanes(t), :] = blk.T
            for t in range(LT):
                w_tiles[p, t, kt] = jnp.concatenate([
                    _pack_rows(*(tmp_s[kt, pl.ds(d + odd * DH, H // 2, stride=2 * DH), :]
                                 for odd in (0, 1)))
                    for d in range(4 * t, 4 * t + 4)], axis=0)

        return [(1, part_fn(ktile, kt)) for kt in range(LT)]

    def permute_wo_items():
        def ntile(t):
            tmp_s[t] = wo_v[:, lanes(t)].astype(F32)
            rows = [tmp_s[t, pl.ds(d, H, stride=DH), :] for d in range(DH)]
            wo_tiles[t] = jnp.concatenate(rows, axis=0).astype(BF16)

        return [(1, part_fn(ntile, t)) for t in range(LT)]

    def stage_x(i):
        xp_s[i % 2] = pltpu.bitcast(x_v[i * BLK:(i + 1) * BLK, :], U32)

    def project_items(i, parts=(0, 1, 2)):
        def tile(p, t, row):
            wt = jnp.concatenate([w_tiles[p, t, kt] for kt in range(LT)], axis=1)
            acc = _nt(_unpack(xp_s[i % 2, row // 2:(row + PM) // 2, :]), _unpack(wt))
            at = i * BLK + row
            if p == 0:
                q_s[t, at:at + PM, :] = acc * qscale
            else:
                (ka_s, va_s)[p - 1][t, HALO + at:HALO + at + PM, :] = acc

        return [(1, part_fn(tile, p, t, row)) for p in parts for t in range(LT)
                for row in range(0, BLK, PM)]

    def attend_items(i):
        rc, part = 16, 64
        keep, pending = {}, []

        def scores(row):
            sums = {}
            for sub in (0, 8):
                at = i * BLK + row + sub
                qs = [q_s[t, at:at + 8, :] for t in range(LT)]
                for w in range(WIN):
                    lo = at + HALO - DIL * w
                    a = qs[0] * ka_s[0, lo:lo + 8, :]
                    for t in range(1, LT):
                        a = a + qs[t] * ka_s[t, lo:lo + 8, :]
                    sums[sub, w] = a
            sums = [sums[sub, w] for sub in (0, 8) for w in range(WIN)]
            pending.extend(sums)
            if (row + rc) % HS == 0:
                lo = (row + rc - HS) * WIN
                lg_s[lo:lo + HS * WIN, :] = _nn(
                    jnp.concatenate(pending, axis=0).astype(BF16), _unpack(dft_s[8]))
                pending.clear()

        def gating(row):
            r0 = i * BLK + row
            xs = [x_v[r0:r0 + rc, lanes(t)].astype(F32) for t in range(LT)]
            z = xs[0] * vec["gate"][:, lanes(0)]
            for t in range(1, LT):
                z = z + xs[t] * vec["gate"][:, lanes(t)]
            th = 0.5 * jnp.tanh(0.5 * jnp.sum(z, axis=-1, keepdims=True))
            g = 0.5 + th
            for t in range(LT):
                gq_s[t, r0:r0 + rc, :] = xs[t] * g
            keep[row] = 0.5 - th

        def mix(row):
            r0 = i * BLK + row
            outs = []
            for sub in (0, 8):
                logits = []
                for w in range(WIN):
                    at = (row + sub + w) * WIN
                    a = lg_s[at:at + 8, :]
                    if r0 + sub < DIL * w:
                        pos = r0 + sub + jax.lax.broadcasted_iota(jnp.int32, (8, 128), 0)
                        a = jnp.where(pos >= DIL * w, a, -1e9)
                    logits.append(a)
                m = logits[0]
                for w in range(1, WIN):
                    m = jnp.maximum(m, logits[w])
                es = [jnp.exp2(a - m) for a in logits]
                den = es[0]
                for w in range(1, WIN):
                    den = den + es[w]
                inv = pl.reciprocal(den, approx=True)
                inv = inv * (2.0 - den * inv)
                norm = keep[row][sub:sub + 8] * inv
                for t in range(LT):
                    a = None
                    for w in range(WIN):
                        lo = r0 + sub + HALO - DIL * w
                        term = es[w] * va_s[t, lo:lo + 8, :]
                        a = term if a is None else a + term
                    outs.append(a * norm)
            for t in range(LT):
                both = jnp.concatenate([outs[t], outs[LT + t]], axis=0).astype(BF16)
                o_s[i % 2][row // 2:(row + rc) // 2, lanes(t)] = pltpu.bitcast(both, U32)

        items = []
        for row in range(0, BLK + part, rc):
            if row < BLK:
                items.append((75, part_fn(gating, row)))
                items.append((155, part_fn(scores, row)))
            if row >= part:
                items.append((215, part_fn(mix, row - part)))
        return items

    def signal_items(i):
        r0 = i * BLK

        def tile(t):
            kf_s[t, r0 + 8:r0 + 8 + BLK, :] = k_v[r0:r0 + BLK, lanes(t)].astype(F32)
            pieces = [[] for _ in range(4)]
            for r in range(8):
                xs = []
                for b in range(4):
                    at = r0 + 64 * b + 8 * r
                    ks = None
                    for j in range(KS):
                        term = kf_s[t, at + 8 - j:at + 16 - j, :] * vec["shift"][j:j + 1, lanes(t)]
                        ks = term if ks is None else ks + term
                    xs.append(ks * v_v[at:at + 8, lanes(t)].astype(F32))
                x0, x1, x2, x3 = xs
                t0, t1 = x0 - x2, x1 + x3
                w0, w1 = SQRT2 * x3, SQRT2 * x2
                res = ((x0 + x2, t1), (t0, x1 - x3),
                       (t0 - w0, t1 + w1), (t0 + w0, t1 - w1))
                for cl in range(4):
                    pieces[cl].append(_pack_rows(*res[cl]))
            for cl in range(4):
                rhs = _unpack(jnp.concatenate(pieces[cl], axis=0))
                u_s[i, t, cl] = _nn(_unpack(dft_s[9 + cl]), rhs)

        return [(450, part_fn(tile, t)) for t in range(LT)]

    def filter_items(a):
        def tile(t):
            lane = jax.lax.broadcasted_iota(jnp.int32, (16, 128), 1)
            sign = jnp.where(lane < 64, -1.0, 1.0).astype(F32)
            pieces = [[] for _ in range(4)]
            for r in range(8):
                rows = slice(t * 128 + 16 * r, t * 128 + 16 * (r + 1))
                lo, hi = (h_v[rows, lanes(2 * a + n)].astype(F32) for n in (0, 1))
                if a == 0:
                    elo, ehi, olo, ohi = lo, hi, lo, hi
                else:
                    plo, phi = (h_v[rows, lanes(2 * a - 2 + n)].astype(F32) for n in (0, 1))
                    elo, ehi, olo, ohi = lo + plo, hi + phi, lo - plo, hi - phi
                tt = olo + sign * ohi
                ww = (SQRT2 * sign) * pltpu.roll(ohi, 64, 1)
                for cl, res in enumerate((elo + ehi, elo - ehi, tt + ww, tt - ww)):
                    pieces[cl].append(res)
            for cl in range(4):
                spec = _nt(_unpack(dft_s[cl]), jnp.concatenate(pieces[cl], axis=0).astype(BF16))
                if a < 2:
                    row = jax.lax.broadcasted_iota(jnp.int32, (128, 128), 0)
                    real = (row & 8) == 0
                    if cl == 0:
                        real = real | (row == 8)
                    dd = vec["skip"][:, lanes(t)]
                    dd = dd if (a == 0 or cl < 2) else -dd
                    spec = spec + jnp.where(real, dd, 0.0)
                g_s[a, t, cl] = spec

        return [(300, part_fn(tile, t)) for t in range(LT)]

    def spectrum_items(m):
        def group(t, cl):
            out = []
            for r in range(8):
                re, im = slice(16 * r, 16 * r + 8), slice(16 * r + 8, 16 * r + 16)
                yr = yi = None
                for a in range(m + 1):
                    gr, gi = g_s[a, t, cl, re, :], g_s[a, t, cl, im, :]
                    ur, ui = u_s[m - a, t, cl, re, :], u_s[m - a, t, cl, im, :]
                    ga, gb = gi, gr
                    if cl == 0 and r == 0:
                        slot0 = jax.lax.broadcasted_iota(jnp.int32, (8, 128), 0) == 0
                        ga, gb = jnp.where(slot0, 0.0, gi), jnp.where(slot0, gi, gr)
                    pr = ur * gr - ui * ga
                    pi = ur * ga + ui * gb
                    yr = pr if yr is None else yr + pr
                    yi = pi if yi is None else yi + pi
                out.append(_pack_rows(yr, yi))
            spectra[m, t, cl] = jnp.concatenate(out, axis=0)

        return [(64 * (m + 1), part_fn(group, t, cl)) for t in range(LT) for cl in range(4)]

    def finish_items(m):
        def tile(t):
            rho = [_nn(_unpack(dft_s[4 + cl]), _unpack(spectra[m, t, cl])) for cl in range(4)]
            for r0 in range(0, 4, PM // 64):
                lhs = jnp.concatenate(
                    [o_s[m % 2][32 * b + 8 * r:32 * b + 8 * (r + 1), :]
                     for r in range(r0, r0 + PM // 64) for b in range(4)], axis=0)
                bb = _nn(_unpack(lhs), wo_tiles[t])
                for r in range(r0, r0 + PM // 64):
                    (a0, a1), (b0, b1), (p0, p1), (n0, n1) = [
                        (z[32 * r:32 * r + 16], z[32 * r + 16:32 * (r + 1)]) for z in rho]
                    s0, s1, d0, d1 = p0 + n0, p1 + n1, p0 - n0, p1 - n1
                    ys = (a0 + b0 + s0, a1 + b1 + s1,
                          a0 - b0 - s0 + SQRT2 * d1, a1 - b1 + s1 - SQRT2 * d0)
                    for b in range(4):
                        lo = m * BLK + 64 * b + 16 * r
                        at = 64 * (r - r0) + 16 * b
                        res = gq_s[t, lo:lo + 16, :] * ys[b] + bb[at:at + 16]
                        out_s[lo:lo + 16, lanes(t)] = res.astype(BF16)

        return [(1, part_fn(tile, t)) for t in range(LT)]

    batches = {n: (n,) for n in range(1, NB)}
    stores = {n + 2: (n,) for n in range(NB)}

    def batch(i):
        return [c[n] for n in batches[i] for c in (cp_x, cp_k, cp_v, cp_h)]

    for i in range(NB + 2):
        streams, spans = [], {}
        if i == 0:
            cp_w[0].wait()
            cp_w[2].start()
            _interleave(permute_w_items(0))
            cp_x[0].wait()
            stage_x(0)
            first = [cp_k[0], cp_v[0], cp_h[0]] + cp_small
            cp_w[1].wait()
            for c in first:
                c.start()
            _interleave(project_items(0, (0,)), permute_w_items(1))
            cp_w[2].wait()
            for c in batch(1):
                c.start()
            _interleave(project_items(0, (1,)), permute_w_items(2))
            for c in first:
                c.wait()
            cp_wo.start()
            load_constants()
            streams.append(project_items(0, (2,)))
        elif i < NB:
            if i in batches:
                for c in batch(i):
                    c.wait()
                later = [j for j in sorted(batches) if j > i]
                if later:
                    for c in batch(later[0]):
                        c.start()
                stage_x(i)
            spans[len(streams)] = SPAN_PROJECT
            streams.append(project_items(i))
            if i + 1 < NB and i + 1 not in batches:
                streams[0].insert(len(streams[0]) * 3 // 4, (0.2, part_fn(stage_x, i + 1)))
        if i < NB:
            sig, fil, spec = signal_items(i), filter_items(i), spectrum_items(i)
            conv = []
            for t in range(LT + 1):
                if t < LT:
                    conv += [sig[t], fil[t]]
                if t > 0:
                    conv += spec[4 * (t - 1):4 * t]
            spans[len(streams)] = SPAN_CONV
            streams.append(conv)
        if i == 1:
            cp_wo.wait()
            streams.append(permute_wo_items())
        if 1 <= i <= NB:
            spans[len(streams)] = SPAN_ATTEND
            streams.append(attend_items(i - 1))
        if i >= 2:
            spans[len(streams)] = SPAN_FINISH
            streams.append(finish_items(i - 2))
        _interleave(*streams, spans=spans)
        for n in stores.get(i, ()):
            cp_out[n].start()
    for c in cp_out:
        c.wait()


@jax.jit
def pallas_gated_mix__ssm_conv_h3__sliding_local_dilated__prompt_kernel(
    A_q: jax.Array,
    A_k: jax.Array,
    A_v: jax.Array,
    A_shift_k: jax.Array,
    A_ssm_k: jax.Array,
    A_ssm_D: jax.Array,
    B_x: jax.Array,
    B_wqkv: jax.Array,
    B_wo: jax.Array,
    gate_w: jax.Array,
):
    del B_x
    hbm = pl.BlockSpec(memory_space=pl.ANY)
    out = pl.pallas_call(
        _kernel,
        out_shape=jax.ShapeDtypeStruct((S, D), BF16),
        in_specs=[hbm] * 10,
        out_specs=hbm,
        scratch_shapes=[
            pltpu.VMEM((S, D), BF16),
            pltpu.VMEM((S, D), BF16),
            pltpu.VMEM((S, D), BF16),
            pltpu.VMEM((D, S), BF16),
            pltpu.VMEM((D, 3 * D), BF16),
            pltpu.VMEM((D, D), BF16),
            pltpu.VMEM((KS, D), BF16),
            pltpu.VMEM((D,), BF16),
            pltpu.VMEM((D,), BF16),
            pltpu.VMEM(_DFT.shape, BF16),
            pltpu.VMEM((LT, D, 128), F32),
            pltpu.VMEM((13, 64, 128), U32),
            pltpu.VMEM((2, BLK // 2, D), U32),
            pltpu.VMEM((LT, S, 128), F32),
            pltpu.VMEM((LT, HALO + S, 128), F32),
            pltpu.VMEM((LT, HALO + S, 128), F32),
            pltpu.VMEM((LT, 8 + S, 128), F32),
            pltpu.VMEM((BLK * WIN, 128), F32),
            pltpu.VMEM((BLK // 2, D), U32),
            pltpu.VMEM((BLK // 2, D), U32),
            pltpu.VMEM((LT, S, 128), F32),
            pltpu.VMEM((NB, LT, 4, 128, 128), F32),
            pltpu.VMEM((NB, LT, 4, 128, 128), F32),
            pltpu.VMEM((S, D), BF16),
            pltpu.SemaphoreType.DMA((3,)),
            pltpu.SemaphoreType.DMA((NB,)),
            pltpu.SemaphoreType.DMA((NB,)),
            pltpu.SemaphoreType.DMA((NB,)),
            pltpu.SemaphoreType.DMA((NB,)),
            pltpu.SemaphoreType.DMA((1,)),
            pltpu.SemaphoreType.DMA((NB,)),
            pltpu.SemaphoreType.DMA((4,)),
        ],
        compiler_params=pltpu.CompilerParams(vmem_limit_bytes=100 * 2**20),
    )(A_q.reshape(S, D), A_k.reshape(S, D), A_v.reshape(S, D), A_ssm_k, B_wqkv, B_wo,
      A_shift_k.T, A_ssm_D, gate_w, jnp.asarray(_DFT, BF16))
    return out.reshape(1, S, D)
```

```python
import functools

import numpy as np
import jax
import jax.numpy as jnp
import jax.experimental.pallas as pl
import jax.experimental.pallas.tpu as pltpu

S, D = 2048, 640
H, DH = 32, 20
WIN, DIL = 8, 2
KS = 4
LT = D // 128
BLK = 256
NB = S // BLK
SPAN_PROJECT = (0.0, 1.0)
SPAN_CONV = (0.0, 1.05)
SPAN_ATTEND = (0.05, 1.05)
SPAN_FINISH = (0.0, 1.0)
HS = 64
PM = 128
HALO = 16
SQRT2 = float(np.sqrt(2.0))
F32, BF16, U32 = jnp.float32, jnp.bfloat16, jnp.uint32


def _dft_matrices():
    n = np.arange(128)[None, :]
    m = np.arange(64)[:, None]
    idx = np.arange(128)
    bins = idx.reshape(2, 8, 8).transpose(1, 0, 2).reshape(-1)
    pairs = idx.reshape(2, 64).T.reshape(-1)
    slabs = idx.reshape(2, 4, 16).transpose(1, 0, 2).reshape(-1)
    filt, sig, inv = [], [], []
    for f in (4 * m, 4 * m + 2, 8 * m + 1, 8 * m + 3):
        ang = 2.0 * np.pi * ((f * n) % 512) / 512.0
        a = np.concatenate([np.cos(ang), -np.sin(ang)], axis=0)
        wgt = np.full((128, 1), 2.0 / 512.0)
        if not filt:
            a[64] = np.cos(np.pi * n[0])
            wgt[0] = wgt[64] = 1.0 / 512.0
        filt.append(a[bins])
        sig.append(a[bins][:, pairs])
        inv.append((a * wgt)[pairs].T[slabs])
    same_head = idx[:, None] % H == idx[None, :] % H
    return np.stack(filt + inv + [same_head] + sig).astype(np.float32)


_DFT = _dft_matrices()


def _nt(a, b):
    return jax.lax.dot_general(a, b, (((1,), (1,)), ((), ())),
                               preferred_element_type=F32)


def _nn(a, b):
    return jnp.dot(a, b, preferred_element_type=F32)


def _pack_rows(even, odd):
    return pltpu.pack_elementwise([even, odd], packed_dtype=BF16)


def _unpack(x):
    return pltpu.bitcast(x, BF16)


def _interleave(*streams, spans=None):
    items = []
    for n, s in enumerate(streams):
        lo, hi = (spans or {}).get(n, (0.0, 1.0))
        total, done = sum(c for c, _ in s), 0.0
        for c, f in s:
            items.append((lo + (hi - lo) * (done + 0.5 * c) / total, f))
            done += c
    for _, f in sorted(items, key=lambda e: e[0]):
        f()


def _kernel(x_hbm, k_hbm, v_hbm, h_hbm, w_hbm, wo_hbm,
            shift_hbm, dvec_hbm, gate_hbm, dft_hbm,
            out_hbm,
            x_v, k_v, v_v, h_v, w_v, wo_v, shift_ref, dvec_ref, gate_ref, dft_ref,
            tmp_s, dft_s, xp_s, q_s, ka_s, va_s,
            kf_s, lg_s, o0_s, o1_s, gq_s, u_s, g_s, out_s,
            w_sem, x_sem, k_sem, v_sem, h_sem, wo_sem, out_sem, small_sem):
    part_fn = functools.partial

    def rows_copy(src, dst, sem, n):
        rows = pl.ds(n * BLK, BLK)
        return pltpu.make_async_copy(src.at[rows], dst.at[rows], sem.at[n])

    def cols_copy(src, dst, sem, n, size):
        cols = pl.ds(n * size, size)
        return pltpu.make_async_copy(src.at[:, cols], dst.at[:, cols], sem.at[n])

    cp_w = [cols_copy(w_hbm, w_v, w_sem, n, D) for n in range(3)]
    cp_x = [rows_copy(x_hbm, x_v, x_sem, n) for n in range(NB)]
    cp_k = [rows_copy(k_hbm, k_v, k_sem, n) for n in range(NB)]
    cp_v = [rows_copy(v_hbm, v_v, v_sem, n) for n in range(NB)]
    cp_h = [cols_copy(h_hbm, h_v, h_sem, n, BLK) for n in range(NB)]
    cp_wo = pltpu.make_async_copy(wo_hbm, wo_v, wo_sem.at[0])
    cp_out = [rows_copy(out_s, out_hbm, out_sem, n) for n in range(NB)]

    cp_small = [
        pltpu.make_async_copy(src, dst, small_sem.at[n])
        for n, (src, dst) in enumerate(((shift_hbm, shift_ref), (dvec_hbm, dvec_ref),
                                        (gate_hbm, gate_ref), (dft_hbm, dft_ref)))]

    cp_w[0].start()
    cp_x[0].start()
    cp_x[1].start()
    cp_w[1].start()

    o_s = (o0_s, o1_s)
    zeros = jnp.zeros((HALO, 128), F32)
    for t in range(LT):
        ka_s[t, 0:HALO, :] = zeros
        va_s[t, 0:HALO, :] = zeros
        kf_s[t, 0:8, :] = zeros[0:8]
    vec = {}

    def load_constants():
        for n in range(_DFT.shape[0]):
            dft_s[n] = pltpu.bitcast(dft_ref[n], U32)
        vec["shift"] = shift_ref[...].astype(F32)
        vec["gate"] = gate_ref[...].astype(F32).reshape(1, D)
        vec["skip"] = dvec_ref[...].astype(F32).reshape(1, D)

    qscale = float(DH ** -0.5 * np.log2(np.e))

    def lanes(t):
        return slice(t * 128, (t + 1) * 128)

    w_tiles, wo_tiles, spectra = {}, {}, {}

    def permute_w_items(p):
        def ktile(kt):
            for t in range(LT):
                blk = w_v[lanes(kt), lanes(p * LT + t)].astype(F32)
                tmp_s[kt, lanes(t), :] = blk.T
            for t in range(LT):
                w_tiles[p, t, kt] = jnp.concatenate([
                    _pack_rows(*(tmp_s[kt, pl.ds(d + odd * DH, H // 2, stride=2 * DH), :]
                                 for odd in (0, 1)))
                    for d in range(4 * t, 4 * t + 4)], axis=0)

        return [(1, part_fn(ktile, kt)) for kt in range(LT)]

    def permute_wo_items():
        def ntile(t):
            tmp_s[t] = wo_v[:, lanes(t)].astype(F32)
            rows = [tmp_s[t, pl.ds(d, H, stride=DH), :] for d in range(DH)]
            wo_tiles[t] = jnp.concatenate(rows, axis=0).astype(BF16)

        return [(1, part_fn(ntile, t)) for t in range(LT)]

    def stage_x(i):
        xp_s[i % 2] = pltpu.bitcast(x_v[i * BLK:(i + 1) * BLK, :], U32)

    def project_items(i, parts=(0, 1, 2)):
        def tile(p, t, row):
            wt = jnp.concatenate([w_tiles[p, t, kt] for kt in range(LT)], axis=1)
            acc = _nt(_unpack(xp_s[i % 2, row // 2:(row + PM) // 2, :]), _unpack(wt))
            at = i * BLK + row
            if p == 0:
                q_s[t, at:at + PM, :] = acc * qscale
            else:
                (ka_s, va_s)[p - 1][t, HALO + at:HALO + at + PM, :] = acc

        return [(1, part_fn(tile, p, t, row)) for p in parts for t in range(LT)
                for row in range(0, BLK, PM)]

    def attend_items(i):
        rc, part = 16, 64
        keep, pending = {}, []

        def scores(row):
            sums = {}
            for sub in (0, 8):
                at = i * BLK + row + sub
                qs = [q_s[t, at:at + 8, :] for t in range(LT)]
                for w in range(WIN):
                    lo = at + HALO - DIL * w
                    a = qs[0] * ka_s[0, lo:lo + 8, :]
                    for t in range(1, LT):
                        a = a + qs[t] * ka_s[t, lo:lo + 8, :]
                    sums[sub, w] = a
            sums = [sums[sub, w] for sub in (0, 8) for w in range(WIN)]
            pending.extend(sums)
            if (row + rc) % HS == 0:
                lo = (row + rc - HS) * WIN
                lg_s[lo:lo + HS * WIN, :] = _nn(
                    jnp.concatenate(pending, axis=0).astype(BF16), _unpack(dft_s[8]))
                pending.clear()

        def gating(row):
            r0 = i * BLK + row
            xs = [x_v[r0:r0 + rc, lanes(t)].astype(F32) for t in range(LT)]
            z = xs[0] * vec["gate"][:, lanes(0)]
            for t in range(1, LT):
                z = z + xs[t] * vec["gate"][:, lanes(t)]
            th = 0.5 * jnp.tanh(0.5 * jnp.sum(z, axis=-1, keepdims=True))
            g = 0.5 + th
            for t in range(LT):
                gq_s[t, r0:r0 + rc, :] = xs[t] * g
            keep[row] = 0.5 - th

        def mix(row):
            r0 = i * BLK + row
            outs = []
            for sub in (0, 8):
                logits = []
                for w in range(WIN):
                    at = (row + sub + w) * WIN
                    a = lg_s[at:at + 8, :]
                    if r0 + sub < DIL * w:
                        pos = r0 + sub + jax.lax.broadcasted_iota(jnp.int32, (8, 128), 0)
                        a = jnp.where(pos >= DIL * w, a, -1e9)
                    logits.append(a)
                m = logits[0]
                for w in range(1, WIN):
                    m = jnp.maximum(m, logits[w])
                es = [jnp.exp2(a - m) for a in logits]
                den = es[0]
                for w in range(1, WIN):
                    den = den + es[w]
                inv = pl.reciprocal(den, approx=True)
                inv = inv * (2.0 - den * inv)
                norm = keep[row][sub:sub + 8] * inv
                for t in range(LT):
                    a = None
                    for w in range(WIN):
                        lo = r0 + sub + HALO - DIL * w
                        term = es[w] * va_s[t, lo:lo + 8, :]
                        a = term if a is None else a + term
                    outs.append(a * norm)
            for t in range(LT):
                both = jnp.concatenate([outs[t], outs[LT + t]], axis=0).astype(BF16)
                o_s[i % 2][row // 2:(row + rc) // 2, lanes(t)] = pltpu.bitcast(both, U32)

        items = []
        for row in range(0, BLK + part, rc):
            if row < BLK:
                items.append((75, part_fn(gating, row)))
                items.append((155, part_fn(scores, row)))
            if row >= part:
                items.append((215, part_fn(mix, row - part)))
        return items

    def signal_items(i):
        r0 = i * BLK

        def tile(t):
            kf_s[t, r0 + 8:r0 + 8 + BLK, :] = k_v[r0:r0 + BLK, lanes(t)].astype(F32)
            pieces = [[] for _ in range(4)]
            for r in range(8):
                xs = []
                for b in range(4):
                    at = r0 + 64 * b + 8 * r
                    ks = None
                    for j in range(KS):
                        term = kf_s[t, at + 8 - j:at + 16 - j, :] * vec["shift"][j:j + 1, lanes(t)]
                        ks = term if ks is None else ks + term
                    xs.append(ks * v_v[at:at + 8, lanes(t)].astype(F32))
                x0, x1, x2, x3 = xs
                t0, t1 = x0 - x2, x1 + x3
                w0, w1 = SQRT2 * x3, SQRT2 * x2
                res = ((x0 + x2, t1), (t0, x1 - x3),
                       (t0 - w0, t1 + w1), (t0 + w0, t1 - w1))
                for cl in range(4):
                    pieces[cl].append(_pack_rows(*res[cl]))
            for cl in range(4):
                rhs = _unpack(jnp.concatenate(pieces[cl], axis=0))
                u_s[i, t, cl] = _nn(_unpack(dft_s[9 + cl]), rhs)

        return [(450, part_fn(tile, t)) for t in range(LT)]

    def filter_items(a):
        def tile(t):
            lane = jax.lax.broadcasted_iota(jnp.int32, (16, 128), 1)
            sign = jnp.where(lane < 64, -1.0, 1.0).astype(F32)
            pieces = [[] for _ in range(4)]
            for r in range(8):
                rows = slice(t * 128 + 16 * r, t * 128 + 16 * (r + 1))
                lo, hi = (h_v[rows, lanes(2 * a + n)].astype(F32) for n in (0, 1))
                if a == 0:
                    elo, ehi, olo, ohi = lo, hi, lo, hi
                else:
                    plo, phi = (h_v[rows, lanes(2 * a - 2 + n)].astype(F32) for n in (0, 1))
                    elo, ehi, olo, ohi = lo + plo, hi + phi, lo - plo, hi - phi
                tt = olo + sign * ohi
                ww = (SQRT2 * sign) * pltpu.roll(ohi, 64, 1)
                for cl, res in enumerate((elo + ehi, elo - ehi, tt + ww, tt - ww)):
                    pieces[cl].append(res)
            for cl in range(4):
                spec = _nt(_unpack(dft_s[cl]), jnp.concatenate(pieces[cl], axis=0).astype(BF16))
                if a < 2:
                    row = jax.lax.broadcasted_iota(jnp.int32, (128, 128), 0)
                    real = (row & 8) == 0
                    if cl == 0:
                        real = real | (row == 8)
                    dd = vec["skip"][:, lanes(t)]
                    dd = dd if (a == 0 or cl < 2) else -dd
                    spec = spec + jnp.where(real, dd, 0.0)
                g_s[a, t, cl] = spec

        return [(300, part_fn(tile, t)) for t in range(LT)]

    def spectrum_items(m):
        def group(t, cl):
            out = []
            for r in range(8):
                re, im = slice(16 * r, 16 * r + 8), slice(16 * r + 8, 16 * r + 16)
                yr = yi = None
                for a in range(m + 1):
                    gr, gi = g_s[a, t, cl, re, :], g_s[a, t, cl, im, :]
                    ur, ui = u_s[m - a, t, cl, re, :], u_s[m - a, t, cl, im, :]
                    ga, gb = gi, gr
                    if cl == 0 and r == 0:
                        slot0 = jax.lax.broadcasted_iota(jnp.int32, (8, 128), 0) == 0
                        ga, gb = jnp.where(slot0, 0.0, gi), jnp.where(slot0, gi, gr)
                    pr = ur * gr - ui * ga
                    pi = ur * ga + ui * gb
                    yr = pr if yr is None else yr + pr
                    yi = pi if yi is None else yi + pi
                out.append(_pack_rows(yr, yi))
            spectra[m, t, cl] = jnp.concatenate(out, axis=0)

        return [(64 * (m + 1), part_fn(group, t, cl)) for t in range(LT) for cl in range(4)]

    def finish_items(m):
        def tile(t):
            rho = [_nn(_unpack(dft_s[4 + cl]), _unpack(spectra[m, t, cl])) for cl in range(4)]
            for r0 in range(0, 4, PM // 64):
                lhs = jnp.concatenate(
                    [o_s[m % 2][32 * b + 8 * r:32 * b + 8 * (r + 1), :]
                     for r in range(r0, r0 + PM // 64) for b in range(4)], axis=0)
                bb = _nn(_unpack(lhs), wo_tiles[t])
                for r in range(r0, r0 + PM // 64):
                    (a0, a1), (b0, b1), (p0, p1), (n0, n1) = [
                        (z[32 * r:32 * r + 16], z[32 * r + 16:32 * (r + 1)]) for z in rho]
                    s0, s1, d0, d1 = p0 + n0, p1 + n1, p0 - n0, p1 - n1
                    ys = (a0 + b0 + s0, a1 + b1 + s1,
                          a0 - b0 - s0 + SQRT2 * d1, a1 - b1 + s1 - SQRT2 * d0)
                    for b in range(4):
                        lo = m * BLK + 64 * b + 16 * r
                        at = 64 * (r - r0) + 16 * b
                        res = gq_s[t, lo:lo + 16, :] * ys[b] + bb[at:at + 16]
                        out_s[lo:lo + 16, lanes(t)] = res.astype(BF16)

        return [(1, part_fn(tile, t)) for t in range(LT)]

    for i in range(NB + 2):
        streams, spans = [], {}
        if i == 0:
            first = [cp_k[0], cp_v[0], cp_h[0]] + cp_small
            cp_w[0].wait()
            cp_w[2].start()
            _interleave(permute_w_items(0))
            for n in (0, 1):
                cp_x[n].wait()
            for n in (0, 1):
                stage_x(n)
            _interleave(project_items(0, (0,)))
            cp_w[1].wait()
            for c in first:
                c.start()
            _interleave(project_items(1, (0,)), permute_w_items(1))
            cp_w[2].wait()
            for c in (cp_k[1], cp_v[1], cp_h[1], cp_wo):
                c.start()
            _interleave(project_items(0, (1,)), permute_w_items(2))
            for c in first:
                c.wait()
            load_constants()
            streams.append(project_items(0, (2,)))
        elif i < NB:
            for c in (cp_k, cp_v, cp_h) + ((cp_x,) if i > 1 else ()):
                c[i].wait()
            if i + 1 < NB:
                for c in (cp_x, cp_k, cp_v, cp_h):
                    c[i + 1].start()
            if i > 1:
                stage_x(i)
            spans[len(streams)] = SPAN_PROJECT
            streams.append(project_items(i, (0, 1, 2) if i > 1 else (1, 2)))
        if i < NB:
            sig, fil, spec = signal_items(i), filter_items(i), spectrum_items(i)
            conv = []
            for t in range(LT + 1):
                if t < LT:
                    conv += [sig[t], fil[t]]
                if t > 0:
                    conv += spec[4 * (t - 1):4 * t]
            spans[len(streams)] = SPAN_CONV
            streams.append(conv)
        if i == 1:
            cp_wo.wait()
            streams.append(permute_wo_items())
        if 1 <= i <= NB:
            spans[len(streams)] = SPAN_ATTEND
            streams.append(attend_items(i - 1))
        if i >= 2:
            spans[len(streams)] = SPAN_FINISH
            streams.append(finish_items(i - 2))
        _interleave(*streams, spans=spans)
        if i >= 2:
            cp_out[i - 2].start()
    for c in cp_out:
        c.wait()


@jax.jit
def pallas_gated_mix__ssm_conv_h3__sliding_local_dilated__prompt_kernel(
    A_q: jax.Array,
    A_k: jax.Array,
    A_v: jax.Array,
    A_shift_k: jax.Array,
    A_ssm_k: jax.Array,
    A_ssm_D: jax.Array,
    B_x: jax.Array,
    B_wqkv: jax.Array,
    B_wo: jax.Array,
    gate_w: jax.Array,
):
    del B_x
    hbm = pl.BlockSpec(memory_space=pl.ANY)
    out = pl.pallas_call(
        _kernel,
        out_shape=jax.ShapeDtypeStruct((S, D), BF16),
        in_specs=[hbm] * 10,
        out_specs=hbm,
        scratch_shapes=[
            pltpu.VMEM((S, D), BF16),
            pltpu.VMEM((S, D), BF16),
            pltpu.VMEM((S, D), BF16),
            pltpu.VMEM((D, S), BF16),
            pltpu.VMEM((D, 3 * D), BF16),
            pltpu.VMEM((D, D), BF16),
            pltpu.VMEM((KS, D), BF16),
            pltpu.VMEM((D,), BF16),
            pltpu.VMEM((D,), BF16),
            pltpu.VMEM(_DFT.shape, BF16),
            pltpu.VMEM((LT, D, 128), F32),
            pltpu.VMEM((13, 64, 128), U32),
            pltpu.VMEM((2, BLK // 2, D), U32),
            pltpu.VMEM((LT, S, 128), F32),
            pltpu.VMEM((LT, HALO + S, 128), F32),
            pltpu.VMEM((LT, HALO + S, 128), F32),
            pltpu.VMEM((LT, 8 + S, 128), F32),
            pltpu.VMEM((BLK * WIN, 128), F32),
            pltpu.VMEM((BLK // 2, D), U32),
            pltpu.VMEM((BLK // 2, D), U32),
            pltpu.VMEM((LT, S, 128), F32),
            pltpu.VMEM((NB, LT, 4, 128, 128), F32),
            pltpu.VMEM((NB, LT, 4, 128, 128), F32),
            pltpu.VMEM((S, D), BF16),
            pltpu.SemaphoreType.DMA((3,)),
            pltpu.SemaphoreType.DMA((NB,)),
            pltpu.SemaphoreType.DMA((NB,)),
            pltpu.SemaphoreType.DMA((NB,)),
            pltpu.SemaphoreType.DMA((NB,)),
            pltpu.SemaphoreType.DMA((1,)),
            pltpu.SemaphoreType.DMA((NB,)),
            pltpu.SemaphoreType.DMA((4,)),
        ],
        compiler_params=pltpu.CompilerParams(vmem_limit_bytes=100 * 2**20),
    )(A_q.reshape(S, D), A_k.reshape(S, D), A_v.reshape(S, D), A_ssm_k, B_wqkv, B_wo,
      A_shift_k.T, A_ssm_D, gate_w, jnp.asarray(_DFT, BF16))
    return out.reshape(1, S, D)
```

```python
import functools

import numpy as np
import jax
import jax.numpy as jnp
import jax.experimental.pallas as pl
import jax.experimental.pallas.tpu as pltpu

S, D = 2048, 640
H, DH = 32, 20
WIN, DIL = 8, 2
KS = 4
LT = D // 128
BLK = 256
NB = S // BLK
SPAN_PROJECT = (0.0, 1.0)
SPAN_CONV = (0.0, 1.05)
SPAN_ATTEND = (0.05, 1.05)
SPAN_FINISH = (0.0, 1.0)
HS = 64
PM = 128
HALO = 16
SQRT2 = float(np.sqrt(2.0))
F32, BF16, U32 = jnp.float32, jnp.bfloat16, jnp.uint32


def _dft_matrices():
    n = np.arange(128)[None, :]
    m = np.arange(64)[:, None]
    idx = np.arange(128)
    bins = idx.reshape(2, 8, 8).transpose(1, 0, 2).reshape(-1)
    pairs = idx.reshape(2, 64).T.reshape(-1)
    slabs = idx.reshape(2, 4, 16).transpose(1, 0, 2).reshape(-1)
    filt, sig, inv = [], [], []
    for f in (4 * m, 4 * m + 2, 8 * m + 1, 8 * m + 3):
        ang = 2.0 * np.pi * ((f * n) % 512) / 512.0
        a = np.concatenate([np.cos(ang), -np.sin(ang)], axis=0)
        wgt = np.full((128, 1), 2.0 / 512.0)
        if not filt:
            a[64] = np.cos(np.pi * n[0])
            wgt[0] = wgt[64] = 1.0 / 512.0
        filt.append(a[bins])
        sig.append(a[bins][:, pairs])
        inv.append((a * wgt)[pairs].T[slabs])
    same_head = idx[:, None] % H == idx[None, :] % H
    return np.stack(filt + inv + [same_head] + sig).astype(np.float32)


_DFT = _dft_matrices()


def _nt(a, b):
    return jax.lax.dot_general(a, b, (((1,), (1,)), ((), ())),
                               preferred_element_type=F32)


def _nn(a, b):
    return jnp.dot(a, b, preferred_element_type=F32)


def _pack_rows(even, odd):
    return pltpu.pack_elementwise([even, odd], packed_dtype=BF16)


def _unpack(x):
    return pltpu.bitcast(x, BF16)


def _interleave(*streams, spans=None):
    items = []
    for n, s in enumerate(streams):
        lo, hi = (spans or {}).get(n, (0.0, 1.0))
        total, done = sum(c for c, _ in s), 0.0
        for c, f in s:
            items.append((lo + (hi - lo) * (done + 0.5 * c) / total, f))
            done += c
    for _, f in sorted(items, key=lambda e: e[0]):
        f()


def _kernel(x_hbm, k_hbm, v_hbm, h_hbm, w_hbm, wo_hbm,
            shift_hbm, dvec_hbm, gate_hbm, dft_hbm,
            out_hbm,
            x_v, k_v, v_v, h_v, w_v, wo_v, shift_ref, dvec_ref, gate_ref, dft_ref,
            tmp_s, dft_s, xp_s, q_s, ka_s, va_s,
            kf_s, lg_s, o0_s, o1_s, gq_s, u_s, g_s, out_s,
            w_sem, x_sem, k_sem, v_sem, h_sem, wo_sem, out_sem, small_sem, wq_sem):
    part_fn = functools.partial

    def rows_copy(src, dst, sem, n):
        rows = pl.ds(n * BLK, BLK)
        return pltpu.make_async_copy(src.at[rows], dst.at[rows], sem.at[n])

    def cols_copy(src, dst, sem, n, size):
        cols = pl.ds(n * size, size)
        return pltpu.make_async_copy(src.at[:, cols], dst.at[:, cols], sem.at[n])

    cp_w = [None] + [cols_copy(w_hbm, w_v, w_sem, n, D) for n in (1, 2)]
    cp_wq = [pltpu.make_async_copy(w_hbm.at[pl.ds(n * 128, 128), pl.ds(0, D)],
                                   w_v.at[pl.ds(n * 128, 128), pl.ds(0, D)], wq_sem.at[n])
             for n in range(LT)]
    cp_x = [rows_copy(x_hbm, x_v, x_sem, n) for n in range(NB)]
    cp_k = [rows_copy(k_hbm, k_v, k_sem, n) for n in range(NB)]
    cp_v = [rows_copy(v_hbm, v_v, v_sem, n) for n in range(NB)]
    cp_h = [cols_copy(h_hbm, h_v, h_sem, n, BLK) for n in range(NB)]
    cp_wo = pltpu.make_async_copy(wo_hbm, wo_v, wo_sem.at[0])
    cp_out = [rows_copy(out_s, out_hbm, out_sem, n) for n in range(NB)]

    cp_small = [
        pltpu.make_async_copy(src, dst, small_sem.at[n])
        for n, (src, dst) in enumerate(((shift_hbm, shift_ref), (dvec_hbm, dvec_ref),
                                        (gate_hbm, gate_ref), (dft_hbm, dft_ref)))]

    for c in cp_wq:
        c.start()
    cp_x[0].start()
    cp_x[1].start()
    cp_w[1].start()

    o_s = (o0_s, o1_s)
    zeros = jnp.zeros((HALO, 128), F32)
    for t in range(LT):
        ka_s[t, 0:HALO, :] = zeros
        va_s[t, 0:HALO, :] = zeros
        kf_s[t, 0:8, :] = zeros[0:8]
    vec = {}

    def load_constants():
        for n in range(_DFT.shape[0]):
            dft_s[n] = pltpu.bitcast(dft_ref[n], U32)
        vec["shift"] = shift_ref[...].astype(F32)
        vec["gate"] = gate_ref[...].astype(F32).reshape(1, D)
        vec["skip"] = dvec_ref[...].astype(F32).reshape(1, D)

    qscale = float(DH ** -0.5 * np.log2(np.e))

    def lanes(t):
        return slice(t * 128, (t + 1) * 128)

    w_tiles, wo_tiles, spectra = {}, {}, {}

    def permute_w_items(p):
        def ktile(kt):
            for t in range(LT):
                blk = w_v[lanes(kt), lanes(p * LT + t)].astype(F32)
                tmp_s[kt, lanes(t), :] = blk.T
            for t in range(LT):
                w_tiles[p, t, kt] = jnp.concatenate([
                    _pack_rows(*(tmp_s[kt, pl.ds(d + odd * DH, H // 2, stride=2 * DH), :]
                                 for odd in (0, 1)))
                    for d in range(4 * t, 4 * t + 4)], axis=0)

        return [(1, part_fn(ktile, kt)) for kt in range(LT)]

    def permute_wo_items():
        def ntile(t):
            tmp_s[t] = wo_v[:, lanes(t)].astype(F32)
            rows = [tmp_s[t, pl.ds(d, H, stride=DH), :] for d in range(DH)]
            wo_tiles[t] = jnp.concatenate(rows, axis=0).astype(BF16)

        return [(1, part_fn(ntile, t)) for t in range(LT)]

    def stage_x(i):
        xp_s[i % 2] = pltpu.bitcast(x_v[i * BLK:(i + 1) * BLK, :], U32)

    def project_items(i, parts=(0, 1, 2)):
        def tile(p, t, row):
            wt = jnp.concatenate([w_tiles[p, t, kt] for kt in range(LT)], axis=1)
            acc = _nt(_unpack(xp_s[i % 2, row // 2:(row + PM) // 2, :]), _unpack(wt))
            at = i * BLK + row
            if p == 0:
                q_s[t, at:at + PM, :] = acc * qscale
            else:
                (ka_s, va_s)[p - 1][t, HALO + at:HALO + at + PM, :] = acc

        return [(1, part_fn(tile, p, t, row)) for p in parts for t in range(LT)
                for row in range(0, BLK, PM)]

    def attend_items(i):
        rc, part = 16, 64
        keep, pending = {}, []

        def scores(row):
            sums = {}
            for sub in (0, 8):
                at = i * BLK + row + sub
                qs = [q_s[t, at:at + 8, :] for t in range(LT)]
                for w in range(WIN):
                    lo = at + HALO - DIL * w
                    a = qs[0] * ka_s[0, lo:lo + 8, :]
                    for t in range(1, LT):
                        a = a + qs[t] * ka_s[t, lo:lo + 8, :]
                    sums[sub, w] = a
            sums = [sums[sub, w] for sub in (0, 8) for w in range(WIN)]
            pending.extend(sums)
            if (row + rc) % HS == 0:
                lo = (row + rc - HS) * WIN
                lg_s[lo:lo + HS * WIN, :] = _nn(
                    jnp.concatenate(pending, axis=0).astype(BF16), _unpack(dft_s[8]))
                pending.clear()

        def gating(row):
            r0 = i * BLK + row
            xs = [x_v[r0:r0 + rc, lanes(t)].astype(F32) for t in range(LT)]
            z = xs[0] * vec["gate"][:, lanes(0)]
            for t in range(1, LT):
                z = z + xs[t] * vec["gate"][:, lanes(t)]
            th = 0.5 * jnp.tanh(0.5 * jnp.sum(z, axis=-1, keepdims=True))
            g = 0.5 + th
            for t in range(LT):
                gq_s[t, r0:r0 + rc, :] = xs[t] * g
            keep[row] = 0.5 - th

        def mix(row):
            r0 = i * BLK + row
            outs = []
            for sub in (0, 8):
                logits = []
                for w in range(WIN):
                    at = (row + sub + w) * WIN
                    a = lg_s[at:at + 8, :]
                    if r0 + sub < DIL * w:
                        pos = r0 + sub + jax.lax.broadcasted_iota(jnp.int32, (8, 128), 0)
                        a = jnp.where(pos >= DIL * w, a, -1e9)
                    logits.append(a)
                m = logits[0]
                for w in range(1, WIN):
                    m = jnp.maximum(m, logits[w])
                es = [jnp.exp2(a - m) for a in logits]
                den = es[0]
                for w in range(1, WIN):
                    den = den + es[w]
                inv = pl.reciprocal(den, approx=True)
                inv = inv * (2.0 - den * inv)
                norm = keep[row][sub:sub + 8] * inv
                for t in range(LT):
                    a = None
                    for w in range(WIN):
                        lo = r0 + sub + HALO - DIL * w
                        term = es[w] * va_s[t, lo:lo + 8, :]
                        a = term if a is None else a + term
                    outs.append(a * norm)
            for t in range(LT):
                both = jnp.concatenate([outs[t], outs[LT + t]], axis=0).astype(BF16)
                o_s[i % 2][row // 2:(row + rc) // 2, lanes(t)] = pltpu.bitcast(both, U32)

        items = []
        for row in range(0, BLK + part, rc):
            if row < BLK:
                items.append((75, part_fn(gating, row)))
                items.append((155, part_fn(scores, row)))
            if row >= part:
                items.append((215, part_fn(mix, row - part)))
        return items

    def signal_items(i):
        r0 = i * BLK

        def tile(t):
            kf_s[t, r0 + 8:r0 + 8 + BLK, :] = k_v[r0:r0 + BLK, lanes(t)].astype(F32)
            pieces = [[] for _ in range(4)]
            for r in range(8):
                xs = []
                for b in range(4):
                    at = r0 + 64 * b + 8 * r
                    ks = None
                    for j in range(KS):
                        term = kf_s[t, at + 8 - j:at + 16 - j, :] * vec["shift"][j:j + 1, lanes(t)]
                        ks = term if ks is None else ks + term
                    xs.append(ks * v_v[at:at + 8, lanes(t)].astype(F32))
                x0, x1, x2, x3 = xs
                t0, t1 = x0 - x2, x1 + x3
                w0, w1 = SQRT2 * x3, SQRT2 * x2
                res = ((x0 + x2, t1), (t0, x1 - x3),
                       (t0 - w0, t1 + w1), (t0 + w0, t1 - w1))
                for cl in range(4):
                    pieces[cl].append(_pack_rows(*res[cl]))
            for cl in range(4):
                rhs = _unpack(jnp.concatenate(pieces[cl], axis=0))
                u_s[i, t, cl] = _nn(_unpack(dft_s[9 + cl]), rhs)

        return [(450, part_fn(tile, t)) for t in range(LT)]

    def filter_items(a):
        def tile(t):
            lane = jax.lax.broadcasted_iota(jnp.int32, (16, 128), 1)
            sign = jnp.where(lane < 64, -1.0, 1.0).astype(F32)
            pieces = [[] for _ in range(4)]
            for r in range(8):
                rows = slice(t * 128 + 16 * r, t * 128 + 16 * (r + 1))
                lo, hi = (h_v[rows, lanes(2 * a + n)].astype(F32) for n in (0, 1))
                if a == 0:
                    elo, ehi, olo, ohi = lo, hi, lo, hi
                else:
                    plo, phi = (h_v[rows, lanes(2 * a - 2 + n)].astype(F32) for n in (0, 1))
                    elo, ehi, olo, ohi = lo + plo, hi + phi, lo - plo, hi - phi
                tt = olo + sign * ohi
                ww = (SQRT2 * sign) * pltpu.roll(ohi, 64, 1)
                for cl, res in enumerate((elo + ehi, elo - ehi, tt + ww, tt - ww)):
                    pieces[cl].append(res)
            for cl in range(4):
                spec = _nt(_unpack(dft_s[cl]), jnp.concatenate(pieces[cl], axis=0).astype(BF16))
                if a < 2:
                    row = jax.lax.broadcasted_iota(jnp.int32, (128, 128), 0)
                    real = (row & 8) == 0
                    if cl == 0:
                        real = real | (row == 8)
                    dd = vec["skip"][:, lanes(t)]
                    dd = dd if (a == 0 or cl < 2) else -dd
                    spec = spec + jnp.where(real, dd, 0.0)
                g_s[a, t, cl] = spec

        return [(300, part_fn(tile, t)) for t in range(LT)]

    def spectrum_items(m):
        def group(t, cl):
            out = []
            for r in range(8):
                re, im = slice(16 * r, 16 * r + 8), slice(16 * r + 8, 16 * r + 16)
                yr = yi = None
                for a in range(m + 1):
                    gr, gi = g_s[a, t, cl, re, :], g_s[a, t, cl, im, :]
                    ur, ui = u_s[m - a, t, cl, re, :], u_s[m - a, t, cl, im, :]
                    ga, gb = gi, gr
                    if cl == 0 and r == 0:
                        slot0 = jax.lax.broadcasted_iota(jnp.int32, (8, 128), 0) == 0
                        ga, gb = jnp.where(slot0, 0.0, gi), jnp.where(slot0, gi, gr)
                    pr = ur * gr - ui * ga
                    pi = ur * ga + ui * gb
                    yr = pr if yr is None else yr + pr
                    yi = pi if yi is None else yi + pi
                out.append(_pack_rows(yr, yi))
            spectra[m, t, cl] = jnp.concatenate(out, axis=0)

        return [(64 * (m + 1), part_fn(group, t, cl)) for t in range(LT) for cl in range(4)]

    def finish_items(m):
        def tile(t):
            rho = [_nn(_unpack(dft_s[4 + cl]), _unpack(spectra[m, t, cl])) for cl in range(4)]
            for r0 in range(0, 4, PM // 64):
                lhs = jnp.concatenate(
                    [o_s[m % 2][32 * b + 8 * r:32 * b + 8 * (r + 1), :]
                     for r in range(r0, r0 + PM // 64) for b in range(4)], axis=0)
                bb = _nn(_unpack(lhs), wo_tiles[t])
                for r in range(r0, r0 + PM // 64):
                    (a0, a1), (b0, b1), (p0, p1), (n0, n1) = [
                        (z[32 * r:32 * r + 16], z[32 * r + 16:32 * (r + 1)]) for z in rho]
                    s0, s1, d0, d1 = p0 + n0, p1 + n1, p0 - n0, p1 - n1
                    ys = (a0 + b0 + s0, a1 + b1 + s1,
                          a0 - b0 - s0 + SQRT2 * d1, a1 - b1 + s1 - SQRT2 * d0)
                    for b in range(4):
                        lo = m * BLK + 64 * b + 16 * r
                        at = 64 * (r - r0) + 16 * b
                        res = gq_s[t, lo:lo + 16, :] * ys[b] + bb[at:at + 16]
                        out_s[lo:lo + 16, lanes(t)] = res.astype(BF16)

        return [(1, part_fn(tile, t)) for t in range(LT)]

    for i in range(NB + 2):
        streams, spans = [], {}
        if i == 0:
            first = [cp_k[0], cp_v[0], cp_h[0]] + cp_small
            for c, (_, permute) in zip(cp_wq, permute_w_items(0)):
                c.wait()
                permute()
            cp_w[2].start()
            for n in (0, 1):
                cp_x[n].wait()
            for n in (0, 1):
                stage_x(n)
            _interleave(project_items(0, (0,)))
            cp_w[1].wait()
            for c in first:
                c.start()
            _interleave(project_items(1, (0,)), permute_w_items(1))
            cp_w[2].wait()
            for c in (cp_k[1], cp_v[1], cp_h[1], cp_wo):
                c.start()
            _interleave(project_items(0, (1,)), permute_w_items(2))
            for c in first:
                c.wait()
            load_constants()
            streams.append(project_items(0, (2,)))
        elif i < NB:
            for c in (cp_k, cp_v, cp_h) + ((cp_x,) if i > 1 else ()):
                c[i].wait()
            if i + 1 < NB:
                for c in (cp_x, cp_k, cp_v, cp_h):
                    c[i + 1].start()
            if i > 1:
                stage_x(i)
            spans[len(streams)] = SPAN_PROJECT
            streams.append(project_items(i, (0, 1, 2) if i > 1 else (1, 2)))
        if i < NB:
            sig, fil, spec = signal_items(i), filter_items(i), spectrum_items(i)
            conv = []
            for t in range(LT + 1):
                if t < LT:
                    conv += [sig[t], fil[t]]
                if t > 0:
                    conv += spec[4 * (t - 1):4 * t]
            spans[len(streams)] = SPAN_CONV
            streams.append(conv)
        if i == 2:
            cp_wo.wait()
            _interleave(permute_wo_items())
        if 1 <= i <= NB:
            spans[len(streams)] = SPAN_ATTEND
            streams.append(attend_items(i - 1))
        if i >= 2:
            spans[len(streams)] = SPAN_FINISH
            streams.append(finish_items(i - 2))
        _interleave(*streams, spans=spans)
        if i >= 2:
            cp_out[i - 2].start()
    for c in cp_out:
        c.wait()


@jax.jit
def pallas_gated_mix__ssm_conv_h3__sliding_local_dilated__prompt_kernel(
    A_q: jax.Array,
    A_k: jax.Array,
    A_v: jax.Array,
    A_shift_k: jax.Array,
    A_ssm_k: jax.Array,
    A_ssm_D: jax.Array,
    B_x: jax.Array,
    B_wqkv: jax.Array,
    B_wo: jax.Array,
    gate_w: jax.Array,
):
    del B_x
    hbm = pl.BlockSpec(memory_space=pl.ANY)
    out = pl.pallas_call(
        _kernel,
        out_shape=jax.ShapeDtypeStruct((S, D), BF16),
        in_specs=[hbm] * 10,
        out_specs=hbm,
        scratch_shapes=[
            pltpu.VMEM((S, D), BF16),
            pltpu.VMEM((S, D), BF16),
            pltpu.VMEM((S, D), BF16),
            pltpu.VMEM((D, S), BF16),
            pltpu.VMEM((D, 3 * D), BF16),
            pltpu.VMEM((D, D), BF16),
            pltpu.VMEM((KS, D), BF16),
            pltpu.VMEM((D,), BF16),
            pltpu.VMEM((D,), BF16),
            pltpu.VMEM(_DFT.shape, BF16),
            pltpu.VMEM((LT, D, 128), F32),
            pltpu.VMEM((13, 64, 128), U32),
            pltpu.VMEM((2, BLK // 2, D), U32),
            pltpu.VMEM((LT, S, 128), F32),
            pltpu.VMEM((LT, HALO + S, 128), F32),
            pltpu.VMEM((LT, HALO + S, 128), F32),
            pltpu.VMEM((LT, 8 + S, 128), F32),
            pltpu.VMEM((BLK * WIN, 128), F32),
            pltpu.VMEM((BLK // 2, D), U32),
            pltpu.VMEM((BLK // 2, D), U32),
            pltpu.VMEM((LT, S, 128), F32),
            pltpu.VMEM((NB, LT, 4, 128, 128), F32),
            pltpu.VMEM((NB, LT, 4, 128, 128), F32),
            pltpu.VMEM((S, D), BF16),
            pltpu.SemaphoreType.DMA((3,)),
            pltpu.SemaphoreType.DMA((NB,)),
            pltpu.SemaphoreType.DMA((NB,)),
            pltpu.SemaphoreType.DMA((NB,)),
            pltpu.SemaphoreType.DMA((NB,)),
            pltpu.SemaphoreType.DMA((1,)),
            pltpu.SemaphoreType.DMA((NB,)),
            pltpu.SemaphoreType.DMA((4,)),
            pltpu.SemaphoreType.DMA((LT,)),
        ],
        compiler_params=pltpu.CompilerParams(vmem_limit_bytes=100 * 2**20),
    )(A_q.reshape(S, D), A_k.reshape(S, D), A_v.reshape(S, D), A_ssm_k, B_wqkv, B_wo,
      A_shift_k.T, A_ssm_D, gate_w, jnp.asarray(_DFT, BF16))
    return out.reshape(1, S, D)
```

```python
import functools

import numpy as np
import jax
import jax.numpy as jnp
import jax.experimental.pallas as pl
import jax.experimental.pallas.tpu as pltpu

S, D = 2048, 640
H, DH = 32, 20
WIN, DIL = 8, 2
KS = 4
LT = D // 128
BLK = 256
NB = S // BLK
SPAN_PROJECT = (0.0, 1.0)
SPAN_CONV = (0.0, 1.05)
SPAN_ATTEND = (0.05, 1.05)
SPAN_FINISH = (0.0, 1.0)
HS = 64
PM = 128
HALO = 16
SQRT2 = float(np.sqrt(2.0))
F32, BF16, U32 = jnp.float32, jnp.bfloat16, jnp.uint32


def _dft_matrices():
    n = np.arange(128)[None, :]
    m = np.arange(64)[:, None]
    idx = np.arange(128)
    bins = idx.reshape(2, 8, 8).transpose(1, 0, 2).reshape(-1)
    slabs = idx.reshape(2, 4, 16).transpose(1, 0, 2).reshape(-1)
    filt, sig, inv = [], [], []
    for f in (4 * m, 4 * m + 2, 8 * m + 1, 8 * m + 3):
        ang = 2.0 * np.pi * ((f * n) % 512) / 512.0
        a = np.concatenate([np.cos(ang), -np.sin(ang)], axis=0)
        wgt = np.full((128, 1), 2.0 / 512.0)
        if not filt:
            a[64] = np.cos(np.pi * n[0])
            wgt[0] = wgt[64] = 1.0 / 512.0
        filt.append(a[bins])
        sig.append(a[bins][:, bins])
        inv.append((a * wgt)[bins].T[slabs])
    same_head = idx[:, None] % H == idx[None, :] % H
    return np.stack(filt + inv + [same_head] + sig).astype(np.float32)


_DFT = _dft_matrices()


def _nt(a, b):
    return jax.lax.dot_general(a, b, (((1,), (1,)), ((), ())),
                               preferred_element_type=F32)


def _nn(a, b):
    return jnp.dot(a, b, preferred_element_type=F32)


def _unpack(x):
    return pltpu.bitcast(x, BF16)


def _interleave(*streams, spans=None):
    items = []
    for n, s in enumerate(streams):
        lo, hi = (spans or {}).get(n, (0.0, 1.0))
        total, done = sum(c for c, _ in s), 0.0
        for c, f in s:
            items.append((lo + (hi - lo) * (done + 0.5 * c) / total, f))
            done += c
    for _, f in sorted(items, key=lambda e: e[0]):
        f()


def _kernel(x_hbm, k_hbm, v_hbm, h_hbm, w_hbm, wo_hbm,
            shift_hbm, dvec_hbm, gate_hbm, dft_hbm,
            out_hbm,
            x_v, k_v, v_v, h_v, w_v, wo_v, shift_ref, dvec_ref, gate_ref, dft_ref,
            tmp_s, dft_s, xp_s, q_s, ka_s, va_s,
            kf_s, lg_s, o0_s, o1_s, gq_s, u_s, g_s, out_s,
            w_sem, x_sem, k_sem, v_sem, h_sem, wo_sem, out_sem, small_sem, wq_sem):
    part_fn = functools.partial

    def rows_copy(src, dst, sem, n):
        rows = pl.ds(n * BLK, BLK)
        return pltpu.make_async_copy(src.at[rows], dst.at[rows], sem.at[n])

    def cols_copy(src, dst, sem, n, size):
        cols = pl.ds(n * size, size)
        return pltpu.make_async_copy(src.at[:, cols], dst.at[:, cols], sem.at[n])

    cp_w = [None] + [cols_copy(w_hbm, w_v, w_sem, n, D) for n in (1, 2)]
    cp_wq = [pltpu.make_async_copy(w_hbm.at[pl.ds(n * 128, 128), pl.ds(0, D)],
                                   w_v.at[pl.ds(n * 128, 128), pl.ds(0, D)], wq_sem.at[n])
             for n in range(LT)]
    cp_x = [rows_copy(x_hbm, x_v, x_sem, n) for n in range(NB)]
    cp_k = [rows_copy(k_hbm, k_v, k_sem, n) for n in range(NB)]
    cp_v = [rows_copy(v_hbm, v_v, v_sem, n) for n in range(NB)]
    cp_h = [cols_copy(h_hbm, h_v, h_sem, n, BLK) for n in range(NB)]
    cp_wo = pltpu.make_async_copy(wo_hbm, wo_v, wo_sem.at[0])
    cp_out = [rows_copy(out_s, out_hbm, out_sem, n) for n in range(NB)]

    cp_small = [
        pltpu.make_async_copy(src, dst, small_sem.at[n])
        for n, (src, dst) in enumerate(((shift_hbm, shift_ref), (dvec_hbm, dvec_ref),
                                        (gate_hbm, gate_ref), (dft_hbm, dft_ref)))]

    for c in cp_wq:
        c.start()
    cp_x[0].start()
    cp_x[1].start()
    cp_w[1].start()

    o_s = (o0_s, o1_s)
    zeros = jnp.zeros((HALO, 128), F32)
    for t in range(LT):
        ka_s[t, 0:HALO, :] = zeros
        va_s[t, 0:HALO, :] = zeros
        kf_s[t, 0:8, :] = zeros[0:8]
    vec = {}

    def load_constants():
        for n in range(_DFT.shape[0]):
            dft_s[n] = pltpu.bitcast(dft_ref[n], U32)
        vec["shift"] = shift_ref[...].astype(F32)
        vec["gate"] = gate_ref[...].astype(F32).reshape(1, D)
        vec["skip"] = dvec_ref[...].astype(F32).reshape(1, D)

    qscale = float(DH ** -0.5 * np.log2(np.e))

    def lanes(t):
        return slice(t * 128, (t + 1) * 128)

    w_tiles, wo_tiles, spectra = {}, {}, {}

    def permute_w_items(p):
        def transpose(kt):
            for t in range(LT):
                blk = w_v[lanes(kt), lanes(p * LT + t)].astype(F32)
                tmp_s[kt, lanes(t), :] = blk.T

        def gather(t):
            w_tiles[p, t] = jnp.concatenate([
                jnp.concatenate([tmp_s[kt, pl.ds(d, H, stride=DH), :]
                                 for d in range(4 * t, 4 * t + 4)], axis=0)
                for kt in range(LT)], axis=1).astype(BF16)

        return ([(2, part_fn(transpose, kt)) for kt in range(LT)]
                + [(1, part_fn(gather, t)) for t in range(LT)])

    def permute_wo_items():
        def ntile(t):
            tmp_s[t] = wo_v[:, lanes(t)].astype(F32)
            rows = [tmp_s[t, pl.ds(d, H, stride=DH), :] for d in range(DH)]
            wo_tiles[t] = jnp.concatenate(rows, axis=0).astype(BF16)

        return [(1, part_fn(ntile, t)) for t in range(LT)]

    def stage_x(i):
        xp_s[i % 2] = pltpu.bitcast(x_v[i * BLK:(i + 1) * BLK, :], U32)

    def project_items(i, parts=(0, 1, 2)):
        def tile(p, t, row):
            acc = _nt(_unpack(xp_s[i % 2, row // 2:(row + PM) // 2, :]), w_tiles[p, t])
            at = i * BLK + row
            if p == 0:
                q_s[t, at:at + PM, :] = acc * qscale
            else:
                (ka_s, va_s)[p - 1][t, HALO + at:HALO + at + PM, :] = acc

        return [(1, part_fn(tile, p, t, row)) for p in parts for t in range(LT)
                for row in range(0, BLK, PM)]

    def attend_items(i):
        rc, part = 16, 64
        keep, pending = {}, []

        def scores(row):
            sums = {}
            for sub in (0, 8):
                at = i * BLK + row + sub
                qs = [q_s[t, at:at + 8, :] for t in range(LT)]
                for w in range(WIN):
                    lo = at + HALO - DIL * w
                    a = qs[0] * ka_s[0, lo:lo + 8, :]
                    for t in range(1, LT):
                        a = a + qs[t] * ka_s[t, lo:lo + 8, :]
                    sums[sub, w] = a
            sums = [sums[sub, w] for sub in (0, 8) for w in range(WIN)]
            pending.extend(sums)
            if (row + rc) % HS == 0:
                lo = (row + rc - HS) * WIN
                lg_s[lo:lo + HS * WIN, :] = _nn(
                    jnp.concatenate(pending, axis=0).astype(BF16), _unpack(dft_s[8]))
                pending.clear()

        def gating(row):
            r0 = i * BLK + row
            xs = [x_v[r0:r0 + rc, lanes(t)].astype(F32) for t in range(LT)]
            z = xs[0] * vec["gate"][:, lanes(0)]
            for t in range(1, LT):
                z = z + xs[t] * vec["gate"][:, lanes(t)]
            th = 0.5 * jnp.tanh(0.5 * jnp.sum(z, axis=-1, keepdims=True))
            g = 0.5 + th
            for t in range(LT):
                gq_s[t, r0:r0 + rc, :] = xs[t] * g
            keep[row] = 0.5 - th

        def mix(row):
            r0 = i * BLK + row
            outs = []
            for sub in (0, 8):
                logits = []
                for w in range(WIN):
                    at = (row + sub + w) * WIN
                    a = lg_s[at:at + 8, :]
                    if r0 + sub < DIL * w:
                        pos = r0 + sub + jax.lax.broadcasted_iota(jnp.int32, (8, 128), 0)
                        a = jnp.where(pos >= DIL * w, a, -1e9)
                    logits.append(a)
                m = logits[0]
                for w in range(1, WIN):
                    m = jnp.maximum(m, logits[w])
                es = [jnp.exp2(a - m) for a in logits]
                den = es[0]
                for w in range(1, WIN):
                    den = den + es[w]
                inv = pl.reciprocal(den, approx=True)
                inv = inv * (2.0 - den * inv)
                norm = keep[row][sub:sub + 8] * inv
                for t in range(LT):
                    a = None
                    for w in range(WIN):
                        lo = r0 + sub + HALO - DIL * w
                        term = es[w] * va_s[t, lo:lo + 8, :]
                        a = term if a is None else a + term
                    outs.append(a * norm)
            for t in range(LT):
                both = jnp.concatenate([outs[t], outs[LT + t]], axis=0).astype(BF16)
                o_s[i % 2][row // 2:(row + rc) // 2, lanes(t)] = pltpu.bitcast(both, U32)

        items = []
        for row in range(0, BLK + part, rc):
            if row < BLK:
                items.append((75, part_fn(gating, row)))
                items.append((155, part_fn(scores, row)))
            if row >= part:
                items.append((215, part_fn(mix, row - part)))
        return items

    def signal_items(i):
        r0 = i * BLK

        def tile(t):
            kf_s[t, r0 + 8:r0 + 8 + BLK, :] = k_v[r0:r0 + BLK, lanes(t)].astype(F32)
            pieces = [[] for _ in range(4)]
            for r in range(8):
                xs = []
                for b in range(4):
                    at = r0 + 64 * b + 8 * r
                    ks = None
                    for j in range(KS):
                        term = kf_s[t, at + 8 - j:at + 16 - j, :] * vec["shift"][j:j + 1, lanes(t)]
                        ks = term if ks is None else ks + term
                    xs.append(ks * v_v[at:at + 8, lanes(t)].astype(F32))
                x0, x1, x2, x3 = xs
                t0, t1 = x0 - x2, x1 + x3
                w0, w1 = SQRT2 * x3, SQRT2 * x2
                res = ((x0 + x2, t1), (t0, x1 - x3),
                       (t0 - w0, t1 + w1), (t0 + w0, t1 - w1))
                for cl in range(4):
                    pieces[cl].extend(res[cl])
            for cl in range(4):
                rhs = jnp.concatenate(pieces[cl], axis=0).astype(BF16)
                u_s[i, t, cl] = _nn(_unpack(dft_s[9 + cl]), rhs)

        return [(450, part_fn(tile, t)) for t in range(LT)]

    def filter_items(a):
        def tile(t):
            lane = jax.lax.broadcasted_iota(jnp.int32, (16, 128), 1)
            sign = jnp.where(lane < 64, -1.0, 1.0).astype(F32)
            pieces = [[] for _ in range(4)]
            for r in range(8):
                rows = slice(t * 128 + 16 * r, t * 128 + 16 * (r + 1))
                lo, hi = (h_v[rows, lanes(2 * a + n)].astype(F32) for n in (0, 1))
                if a == 0:
                    elo, ehi, olo, ohi = lo, hi, lo, hi
                else:
                    plo, phi = (h_v[rows, lanes(2 * a - 2 + n)].astype(F32) for n in (0, 1))
                    elo, ehi, olo, ohi = lo + plo, hi + phi, lo - plo, hi - phi
                tt = olo + sign * ohi
                ww = (SQRT2 * sign) * pltpu.roll(ohi, 64, 1)
                for cl, res in enumerate((elo + ehi, elo - ehi, tt + ww, tt - ww)):
                    pieces[cl].append(res)
            for cl in range(4):
                spec = _nt(_unpack(dft_s[cl]), jnp.concatenate(pieces[cl], axis=0).astype(BF16))
                if a < 2:
                    row = jax.lax.broadcasted_iota(jnp.int32, (128, 128), 0)
                    real = (row & 8) == 0
                    if cl == 0:
                        real = real | (row == 8)
                    dd = vec["skip"][:, lanes(t)]
                    dd = dd if (a == 0 or cl < 2) else -dd
                    spec = spec + jnp.where(real, dd, 0.0)
                g_s[a, t, cl] = spec

        return [(300, part_fn(tile, t)) for t in range(LT)]

    def spectrum_items(m):
        def group(t, cl):
            out = []
            for r in range(8):
                re, im = slice(16 * r, 16 * r + 8), slice(16 * r + 8, 16 * r + 16)
                yr = yi = None
                for a in range(m + 1):
                    gr, gi = g_s[a, t, cl, re, :], g_s[a, t, cl, im, :]
                    ur, ui = u_s[m - a, t, cl, re, :], u_s[m - a, t, cl, im, :]
                    ga, gb = gi, gr
                    if cl == 0 and r == 0:
                        slot0 = jax.lax.broadcasted_iota(jnp.int32, (8, 128), 0) == 0
                        ga, gb = jnp.where(slot0, 0.0, gi), jnp.where(slot0, gi, gr)
                    pr = ur * gr - ui * ga
                    pi = ur * ga + ui * gb
                    yr = pr if yr is None else yr + pr
                    yi = pi if yi is None else yi + pi
                out += [yr, yi]
            spectra[m, t, cl] = jnp.concatenate(out, axis=0).astype(BF16)

        return [(64 * (m + 1), part_fn(group, t, cl)) for t in range(LT) for cl in range(4)]

    def finish_items(m):
        def tile(t):
            rho = [_nn(_unpack(dft_s[4 + cl]), spectra[m, t, cl]) for cl in range(4)]
            for r0 in range(0, 4, PM // 64):
                lhs = jnp.concatenate(
                    [o_s[m % 2][32 * b + 8 * r:32 * b + 8 * (r + 1), :]
                     for r in range(r0, r0 + PM // 64) for b in range(4)], axis=0)
                bb = _nn(_unpack(lhs), wo_tiles[t])
                for r in range(r0, r0 + PM // 64):
                    (a0, a1), (b0, b1), (p0, p1), (n0, n1) = [
                        (z[32 * r:32 * r + 16], z[32 * r + 16:32 * (r + 1)]) for z in rho]
                    s0, s1, d0, d1 = p0 + n0, p1 + n1, p0 - n0, p1 - n1
                    ys = (a0 + b0 + s0, a1 + b1 + s1,
                          a0 - b0 - s0 + SQRT2 * d1, a1 - b1 + s1 - SQRT2 * d0)
                    for b in range(4):
                        lo = m * BLK + 64 * b + 16 * r
                        at = 64 * (r - r0) + 16 * b
                        res = gq_s[t, lo:lo + 16, :] * ys[b] + bb[at:at + 16]
                        out_s[lo:lo + 16, lanes(t)] = res.astype(BF16)

        return [(1, part_fn(tile, t)) for t in range(LT)]

    for i in range(NB + 2):
        streams, spans = [], {}
        if i == 0:
            first = [cp_k[0], cp_v[0], cp_h[0]] + cp_small
            for n, (_, permute) in enumerate(permute_w_items(0)):
                if n < LT:
                    cp_wq[n].wait()
                permute()
            cp_w[2].start()
            for n in (0, 1):
                cp_x[n].wait()
            for n in (0, 1):
                stage_x(n)
            _interleave(project_items(0, (0,)))
            cp_w[1].wait()
            for c in first:
                c.start()
            _interleave(project_items(1, (0,)), permute_w_items(1))
            cp_w[2].wait()
            for c in (cp_k[1], cp_v[1], cp_h[1], cp_wo):
                c.start()
            _interleave(project_items(0, (1,)), permute_w_items(2))
            for c in first:
                c.wait()
            load_constants()
            streams.append(project_items(0, (2,)))
        elif i < NB:
            for c in (cp_k, cp_v, cp_h) + ((cp_x,) if i > 1 else ()):
                c[i].wait()
            if i + 1 < NB:
                for c in (cp_x, cp_k, cp_v, cp_h):
                    c[i + 1].start()
            if i > 1:
                stage_x(i)
            spans[len(streams)] = SPAN_PROJECT
            streams.append(project_items(i, (0, 1, 2) if i > 1 else (1, 2)))
        if i < NB:
            sig, fil, spec = signal_items(i), filter_items(i), spectrum_items(i)
            conv = []
            for t in range(LT + 1):
                if t < LT:
                    conv += [sig[t], fil[t]]
                if t > 0:
                    conv += spec[4 * (t - 1):4 * t]
            spans[len(streams)] = SPAN_CONV
            streams.append(conv)
        if i == 2:
            cp_wo.wait()
            _interleave(permute_wo_items())
        if 1 <= i <= NB:
            spans[len(streams)] = SPAN_ATTEND
            streams.append(attend_items(i - 1))
        if i >= 2:
            spans[len(streams)] = SPAN_FINISH
            streams.append(finish_items(i - 2))
        _interleave(*streams, spans=spans)
        if i >= 2:
            cp_out[i - 2].start()
    for c in cp_out:
        c.wait()


@jax.jit
def pallas_gated_mix__ssm_conv_h3__sliding_local_dilated__prompt_kernel(
    A_q: jax.Array,
    A_k: jax.Array,
    A_v: jax.Array,
    A_shift_k: jax.Array,
    A_ssm_k: jax.Array,
    A_ssm_D: jax.Array,
    B_x: jax.Array,
    B_wqkv: jax.Array,
    B_wo: jax.Array,
    gate_w: jax.Array,
):
    del B_x
    hbm = pl.BlockSpec(memory_space=pl.ANY)
    out = pl.pallas_call(
        _kernel,
        out_shape=jax.ShapeDtypeStruct((S, D), BF16),
        in_specs=[hbm] * 10,
        out_specs=hbm,
        scratch_shapes=[
            pltpu.VMEM((S, D), BF16),
            pltpu.VMEM((S, D), BF16),
            pltpu.VMEM((S, D), BF16),
            pltpu.VMEM((D, S), BF16),
            pltpu.VMEM((D, 3 * D), BF16),
            pltpu.VMEM((D, D), BF16),
            pltpu.VMEM((KS, D), BF16),
            pltpu.VMEM((D,), BF16),
            pltpu.VMEM((D,), BF16),
            pltpu.VMEM(_DFT.shape, BF16),
            pltpu.VMEM((LT, D, 128), F32),
            pltpu.VMEM((13, 64, 128), U32),
            pltpu.VMEM((2, BLK // 2, D), U32),
            pltpu.VMEM((LT, S, 128), F32),
            pltpu.VMEM((LT, HALO + S, 128), F32),
            pltpu.VMEM((LT, HALO + S, 128), F32),
            pltpu.VMEM((LT, 8 + S, 128), F32),
            pltpu.VMEM((BLK * WIN, 128), F32),
            pltpu.VMEM((BLK // 2, D), U32),
            pltpu.VMEM((BLK // 2, D), U32),
            pltpu.VMEM((LT, S, 128), F32),
            pltpu.VMEM((NB, LT, 4, 128, 128), F32),
            pltpu.VMEM((NB, LT, 4, 128, 128), F32),
            pltpu.VMEM((S, D), BF16),
            pltpu.SemaphoreType.DMA((3,)),
            pltpu.SemaphoreType.DMA((NB,)),
            pltpu.SemaphoreType.DMA((NB,)),
            pltpu.SemaphoreType.DMA((NB,)),
            pltpu.SemaphoreType.DMA((NB,)),
            pltpu.SemaphoreType.DMA((1,)),
            pltpu.SemaphoreType.DMA((NB,)),
            pltpu.SemaphoreType.DMA((4,)),
            pltpu.SemaphoreType.DMA((LT,)),
        ],
        compiler_params=pltpu.CompilerParams(vmem_limit_bytes=100 * 2**20),
    )(A_q.reshape(S, D), A_k.reshape(S, D), A_v.reshape(S, D), A_ssm_k, B_wqkv, B_wo,
      A_shift_k.T, A_ssm_D, gate_w, jnp.asarray(_DFT, BF16))
    return out.reshape(1, S, D)
```

```python
import functools

import numpy as np
import jax
import jax.numpy as jnp
import jax.experimental.pallas as pl
import jax.experimental.pallas.tpu as pltpu

S, D = 2048, 640
H, DH = 32, 20
WIN, DIL = 8, 2
KS = 4
LT = D // 128
BLK = 256
NB = S // BLK
SPAN_PROJECT = (0.0, 1.0)
SPAN_CONV = (0.0, 1.05)
SPAN_ATTEND = (0.05, 1.05)
SPAN_FINISH = (0.0, 1.0)
AHEAD = {7: (5, (3, 4)), 6: (4, (3,))}
HS = 64
PM = 128
HALO = 16
SQRT2 = float(np.sqrt(2.0))
F32, BF16, U32 = jnp.float32, jnp.bfloat16, jnp.uint32


def _dft_matrices():
    n = np.arange(128)[None, :]
    m = np.arange(64)[:, None]
    idx = np.arange(128)
    bins = idx.reshape(2, 8, 8).transpose(1, 0, 2).reshape(-1)
    slabs = idx.reshape(2, 4, 16).transpose(1, 0, 2).reshape(-1)
    filt, sig, inv = [], [], []
    for f in (4 * m, 4 * m + 2, 8 * m + 1, 8 * m + 3):
        ang = 2.0 * np.pi * ((f * n) % 512) / 512.0
        a = np.concatenate([np.cos(ang), -np.sin(ang)], axis=0)
        wgt = np.full((128, 1), 2.0 / 512.0)
        if not filt:
            a[64] = np.cos(np.pi * n[0])
            wgt[0] = wgt[64] = 1.0 / 512.0
        filt.append(a[bins])
        sig.append(a[bins][:, bins])
        inv.append((a * wgt)[bins].T[slabs])
    same_head = idx[:, None] % H == idx[None, :] % H
    return np.stack(filt + inv + [same_head] + sig).astype(np.float32)


_DFT = _dft_matrices()


def _nt(a, b):
    return jax.lax.dot_general(a, b, (((1,), (1,)), ((), ())),
                               preferred_element_type=F32)


def _nn(a, b):
    return jnp.dot(a, b, preferred_element_type=F32)


def _unpack(x):
    return pltpu.bitcast(x, BF16)


def _interleave(*streams, spans=None):
    items = []
    for n, s in enumerate(streams):
        lo, hi = (spans or {}).get(n, (0.0, 1.0))
        total, done = sum(c for c, _ in s), 0.0
        for c, f in s:
            items.append((lo + (hi - lo) * (done + 0.5 * c) / total, f))
            done += c
    for _, f in sorted(items, key=lambda e: e[0]):
        f()


def _kernel(x_hbm, k_hbm, v_hbm, h_hbm, w_hbm, wo_hbm,
            shift_hbm, dvec_hbm, gate_hbm, dft_hbm,
            out_hbm,
            x_v, k_v, v_v, h_v, w_v, wo_v, shift_ref, dvec_ref, gate_ref, dft_ref,
            tmp_s, dft_s, xp_s, q_s, ka_s, va_s,
            kf_s, lg_s, o0_s, o1_s, gq_s, u_s, g_s, out_s,
            w_sem, x_sem, k_sem, v_sem, h_sem, wo_sem, out_sem, small_sem, wq_sem):
    part_fn = functools.partial

    def rows_copy(src, dst, sem, n):
        rows = pl.ds(n * BLK, BLK)
        return pltpu.make_async_copy(src.at[rows], dst.at[rows], sem.at[n])

    def cols_copy(src, dst, sem, n, size):
        cols = pl.ds(n * size, size)
        return pltpu.make_async_copy(src.at[:, cols], dst.at[:, cols], sem.at[n])

    cp_w = [None] + [cols_copy(w_hbm, w_v, w_sem, n, D) for n in (1, 2)]
    cp_wq = [pltpu.make_async_copy(w_hbm.at[pl.ds(n * 128, 128), pl.ds(0, D)],
                                   w_v.at[pl.ds(n * 128, 128), pl.ds(0, D)], wq_sem.at[n])
             for n in range(LT)]
    cp_x = [rows_copy(x_hbm, x_v, x_sem, n) for n in range(NB)]
    cp_k = [rows_copy(k_hbm, k_v, k_sem, n) for n in range(NB)]
    cp_v = [rows_copy(v_hbm, v_v, v_sem, n) for n in range(NB)]
    cp_h = [cols_copy(h_hbm, h_v, h_sem, n, BLK) for n in range(NB)]
    cp_wo = pltpu.make_async_copy(wo_hbm, wo_v, wo_sem.at[0])
    cp_out = [rows_copy(out_s, out_hbm, out_sem, n) for n in range(NB)]

    cp_small = [
        pltpu.make_async_copy(src, dst, small_sem.at[n])
        for n, (src, dst) in enumerate(((shift_hbm, shift_ref), (dvec_hbm, dvec_ref),
                                        (gate_hbm, gate_ref), (dft_hbm, dft_ref)))]

    for c in cp_wq:
        c.start()
    cp_x[0].start()
    cp_x[1].start()
    cp_w[1].start()

    o_s = (o0_s, o1_s)
    zeros = jnp.zeros((HALO, 128), F32)
    for t in range(LT):
        ka_s[t, 0:HALO, :] = zeros
        va_s[t, 0:HALO, :] = zeros
        kf_s[t, 0:8, :] = zeros[0:8]
    vec = {}

    def load_constants():
        for n in range(_DFT.shape[0]):
            dft_s[n] = pltpu.bitcast(dft_ref[n], U32)
        vec["shift"] = shift_ref[...].astype(F32)
        vec["gate"] = gate_ref[...].astype(F32).reshape(1, D)
        vec["skip"] = dvec_ref[...].astype(F32).reshape(1, D)

    qscale = float(DH ** -0.5 * np.log2(np.e))

    def lanes(t):
        return slice(t * 128, (t + 1) * 128)

    w_tiles, wo_tiles, spectra, carried = {}, {}, {}, {}

    def permute_w_items(p):
        def transpose(kt):
            for t in range(LT):
                blk = w_v[lanes(kt), lanes(p * LT + t)].astype(F32)
                tmp_s[kt, lanes(t), :] = blk.T

        def gather(t):
            w_tiles[p, t] = jnp.concatenate([
                jnp.concatenate([tmp_s[kt, pl.ds(d, H, stride=DH), :]
                                 for d in range(4 * t, 4 * t + 4)], axis=0)
                for kt in range(LT)], axis=1).astype(BF16)

        return ([(2, part_fn(transpose, kt)) for kt in range(LT)]
                + [(1, part_fn(gather, t)) for t in range(LT)])

    def permute_wo_items():
        def ntile(t):
            tmp_s[t] = wo_v[:, lanes(t)].astype(F32)
            rows = [tmp_s[t, pl.ds(d, H, stride=DH), :] for d in range(DH)]
            wo_tiles[t] = jnp.concatenate(rows, axis=0).astype(BF16)

        return [(1, part_fn(ntile, t)) for t in range(LT)]

    def stage_x(i):
        xp_s[i % 2] = pltpu.bitcast(x_v[i * BLK:(i + 1) * BLK, :], U32)

    def project_items(i, parts=(0, 1, 2)):
        def tile(p, t, row):
            acc = _nt(_unpack(xp_s[i % 2, row // 2:(row + PM) // 2, :]), w_tiles[p, t])
            at = i * BLK + row
            if p == 0:
                q_s[t, at:at + PM, :] = acc * qscale
            else:
                (ka_s, va_s)[p - 1][t, HALO + at:HALO + at + PM, :] = acc

        return [(1, part_fn(tile, p, t, row)) for p in parts for t in range(LT)
                for row in range(0, BLK, PM)]

    def attend_items(i):
        rc, part = 16, 64
        keep, pending = {}, []

        def scores(row):
            sums = {}
            for sub in (0, 8):
                at = i * BLK + row + sub
                qs = [q_s[t, at:at + 8, :] for t in range(LT)]
                for w in range(WIN):
                    lo = at + HALO - DIL * w
                    a = qs[0] * ka_s[0, lo:lo + 8, :]
                    for t in range(1, LT):
                        a = a + qs[t] * ka_s[t, lo:lo + 8, :]
                    sums[sub, w] = a
            sums = [sums[sub, w] for sub in (0, 8) for w in range(WIN)]
            pending.extend(sums)
            if (row + rc) % HS == 0:
                lo = (row + rc - HS) * WIN
                lg_s[lo:lo + HS * WIN, :] = _nn(
                    jnp.concatenate(pending, axis=0).astype(BF16), _unpack(dft_s[8]))
                pending.clear()

        def gating(row):
            r0 = i * BLK + row
            xs = [x_v[r0:r0 + rc, lanes(t)].astype(F32) for t in range(LT)]
            z = xs[0] * vec["gate"][:, lanes(0)]
            for t in range(1, LT):
                z = z + xs[t] * vec["gate"][:, lanes(t)]
            th = 0.5 * jnp.tanh(0.5 * jnp.sum(z, axis=-1, keepdims=True))
            g = 0.5 + th
            for t in range(LT):
                gq_s[t, r0:r0 + rc, :] = xs[t] * g
            keep[row] = 0.5 - th

        def mix(row):
            r0 = i * BLK + row
            outs = []
            for sub in (0, 8):
                logits = []
                for w in range(WIN):
                    at = (row + sub + w) * WIN
                    a = lg_s[at:at + 8, :]
                    if r0 + sub < DIL * w:
                        pos = r0 + sub + jax.lax.broadcasted_iota(jnp.int32, (8, 128), 0)
                        a = jnp.where(pos >= DIL * w, a, -1e9)
                    logits.append(a)
                m = logits[0]
                for w in range(1, WIN):
                    m = jnp.maximum(m, logits[w])
                es = [jnp.exp2(a - m) for a in logits]
                den = es[0]
                for w in range(1, WIN):
                    den = den + es[w]
                inv = pl.reciprocal(den, approx=True)
                inv = inv * (2.0 - den * inv)
                norm = keep[row][sub:sub + 8] * inv
                for t in range(LT):
                    a = None
                    for w in range(WIN):
                        lo = r0 + sub + HALO - DIL * w
                        term = es[w] * va_s[t, lo:lo + 8, :]
                        a = term if a is None else a + term
                    outs.append(a * norm)
            for t in range(LT):
                both = jnp.concatenate([outs[t], outs[LT + t]], axis=0).astype(BF16)
                o_s[i % 2][row // 2:(row + rc) // 2, lanes(t)] = pltpu.bitcast(both, U32)

        items = []
        for row in range(0, BLK + part, rc):
            if row < BLK:
                items.append((75, part_fn(gating, row)))
                items.append((155, part_fn(scores, row)))
            if row >= part:
                items.append((215, part_fn(mix, row - part)))
        return items

    def signal_items(i):
        r0 = i * BLK

        def tile(t):
            kf_s[t, r0 + 8:r0 + 8 + BLK, :] = k_v[r0:r0 + BLK, lanes(t)].astype(F32)
            pieces = [[] for _ in range(4)]
            for r in range(8):
                xs = []
                for b in range(4):
                    at = r0 + 64 * b + 8 * r
                    ks = None
                    for j in range(KS):
                        term = kf_s[t, at + 8 - j:at + 16 - j, :] * vec["shift"][j:j + 1, lanes(t)]
                        ks = term if ks is None else ks + term
                    xs.append(ks * v_v[at:at + 8, lanes(t)].astype(F32))
                x0, x1, x2, x3 = xs
                t0, t1 = x0 - x2, x1 + x3
                w0, w1 = SQRT2 * x3, SQRT2 * x2
                res = ((x0 + x2, t1), (t0, x1 - x3),
                       (t0 - w0, t1 + w1), (t0 + w0, t1 - w1))
                for cl in range(4):
                    pieces[cl].extend(res[cl])
            for cl in range(4):
                rhs = jnp.concatenate(pieces[cl], axis=0).astype(BF16)
                u_s[i, t, cl] = _nn(_unpack(dft_s[9 + cl]), rhs)

        return [(450, part_fn(tile, t)) for t in range(LT)]

    def filter_items(a):
        def tile(t):
            lane = jax.lax.broadcasted_iota(jnp.int32, (16, 128), 1)
            sign = jnp.where(lane < 64, -1.0, 1.0).astype(F32)
            pieces = [[] for _ in range(4)]
            for r in range(8):
                rows = slice(t * 128 + 16 * r, t * 128 + 16 * (r + 1))
                lo, hi = (h_v[rows, lanes(2 * a + n)].astype(F32) for n in (0, 1))
                if a == 0:
                    elo, ehi, olo, ohi = lo, hi, lo, hi
                else:
                    plo, phi = (h_v[rows, lanes(2 * a - 2 + n)].astype(F32) for n in (0, 1))
                    elo, ehi, olo, ohi = lo + plo, hi + phi, lo - plo, hi - phi
                tt = olo + sign * ohi
                ww = (SQRT2 * sign) * pltpu.roll(ohi, 64, 1)
                for cl, res in enumerate((elo + ehi, elo - ehi, tt + ww, tt - ww)):
                    pieces[cl].append(res)
            for cl in range(4):
                spec = _nt(_unpack(dft_s[cl]), jnp.concatenate(pieces[cl], axis=0).astype(BF16))
                if a < 2:
                    row = jax.lax.broadcasted_iota(jnp.int32, (128, 128), 0)
                    real = (row & 8) == 0
                    if cl == 0:
                        real = real | (row == 8)
                    dd = vec["skip"][:, lanes(t)]
                    dd = dd if (a == 0 or cl < 2) else -dd
                    spec = spec + jnp.where(real, dd, 0.0)
                g_s[a, t, cl] = spec

        return [(300, part_fn(tile, t)) for t in range(LT)]

    def spectrum_items(m, lags, last=True):
        def group(t, cl):
            out = []
            for r in range(8):
                re, im = slice(16 * r, 16 * r + 8), slice(16 * r + 8, 16 * r + 16)
                yr, yi = carried.pop((m, t, cl, r), (None, None))
                for a in lags:
                    gr, gi = g_s[a, t, cl, re, :], g_s[a, t, cl, im, :]
                    ur, ui = u_s[m - a, t, cl, re, :], u_s[m - a, t, cl, im, :]
                    ga, gb = gi, gr
                    if cl == 0 and r == 0:
                        slot0 = jax.lax.broadcasted_iota(jnp.int32, (8, 128), 0) == 0
                        ga, gb = jnp.where(slot0, 0.0, gi), jnp.where(slot0, gi, gr)
                    pr = ur * gr - ui * ga
                    pi = ur * ga + ui * gb
                    yr = pr if yr is None else yr + pr
                    yi = pi if yi is None else yi + pi
                out += [yr, yi]
                if not last:
                    carried[m, t, cl, r] = (yr, yi)
            if last:
                spectra[m, t, cl] = jnp.concatenate(out, axis=0).astype(BF16)

        return [(64 * len(lags), part_fn(group, t, cl)) for t in range(LT) for cl in range(4)]

    def finish_items(m):
        def tile(t):
            rho = [_nn(_unpack(dft_s[4 + cl]), spectra[m, t, cl]) for cl in range(4)]
            for r0 in range(0, 4, PM // 64):
                lhs = jnp.concatenate(
                    [o_s[m % 2][32 * b + 8 * r:32 * b + 8 * (r + 1), :]
                     for r in range(r0, r0 + PM // 64) for b in range(4)], axis=0)
                bb = _nn(_unpack(lhs), wo_tiles[t])
                for r in range(r0, r0 + PM // 64):
                    (a0, a1), (b0, b1), (p0, p1), (n0, n1) = [
                        (z[32 * r:32 * r + 16], z[32 * r + 16:32 * (r + 1)]) for z in rho]
                    s0, s1, d0, d1 = p0 + n0, p1 + n1, p0 - n0, p1 - n1
                    ys = (a0 + b0 + s0, a1 + b1 + s1,
                          a0 - b0 - s0 + SQRT2 * d1, a1 - b1 + s1 - SQRT2 * d0)
                    for b in range(4):
                        lo = m * BLK + 64 * b + 16 * r
                        at = 64 * (r - r0) + 16 * b
                        res = gq_s[t, lo:lo + 16, :] * ys[b] + bb[at:at + 16]
                        out_s[lo:lo + 16, lanes(t)] = res.astype(BF16)

        return [(1, part_fn(tile, t)) for t in range(LT)]

    for i in range(NB + 2):
        streams, spans = [], {}
        if i == 0:
            first = [cp_k[0], cp_v[0], cp_h[0]] + cp_small
            for n, (_, permute) in enumerate(permute_w_items(0)):
                if n < LT:
                    cp_wq[n].wait()
                permute()
            cp_w[2].start()
            for n in (0, 1):
                cp_x[n].wait()
            for n in (0, 1):
                stage_x(n)
            _interleave(project_items(0, (0,)))
            cp_w[1].wait()
            for c in first:
                c.start()
            _interleave(project_items(1, (0,)), permute_w_items(1))
            cp_w[2].wait()
            for c in (cp_k[1], cp_v[1], cp_h[1], cp_wo):
                c.start()
            _interleave(project_items(0, (1,)), permute_w_items(2))
            for c in first:
                c.wait()
            load_constants()
            streams.append(project_items(0, (2,)))
        elif i < NB:
            for c in (cp_k, cp_v, cp_h) + ((cp_x,) if i > 1 else ()):
                c[i].wait()
            if i + 1 < NB:
                for c in (cp_x, cp_k, cp_v, cp_h):
                    c[i + 1].start()
            if i > 1:
                stage_x(i)
            spans[len(streams)] = SPAN_PROJECT
            streams.append(project_items(i, (0, 1, 2) if i > 1 else (1, 2)))
        if i < NB:
            sig, fil, spec = signal_items(i), filter_items(i), spectrum_items(
                i, [a for a in range(i + 1) if a not in AHEAD.get(i, (0, ()))[1]])
            conv = []
            for t in range(LT + 1):
                if t < LT:
                    conv += [sig[t], fil[t]]
                if t > 0:
                    conv += spec[4 * (t - 1):4 * t]
            for m, (step, lags) in AHEAD.items():
                if step == i:
                    streams.append(spectrum_items(m, lags, last=False))
            spans[len(streams)] = SPAN_CONV
            streams.append(conv)
        if i == 2:
            cp_wo.wait()
            _interleave(permute_wo_items())
        if 1 <= i <= NB:
            spans[len(streams)] = SPAN_ATTEND
            streams.append(attend_items(i - 1))
        if i >= 2:
            spans[len(streams)] = SPAN_FINISH
            streams.append(finish_items(i - 2))
        _interleave(*streams, spans=spans)
        if i >= 2:
            cp_out[i - 2].start()
    for c in cp_out:
        c.wait()


@jax.jit
def pallas_gated_mix__ssm_conv_h3__sliding_local_dilated__prompt_kernel(
    A_q: jax.Array,
    A_k: jax.Array,
    A_v: jax.Array,
    A_shift_k: jax.Array,
    A_ssm_k: jax.Array,
    A_ssm_D: jax.Array,
    B_x: jax.Array,
    B_wqkv: jax.Array,
    B_wo: jax.Array,
    gate_w: jax.Array,
):
    del B_x
    hbm = pl.BlockSpec(memory_space=pl.ANY)
    out = pl.pallas_call(
        _kernel,
        out_shape=jax.ShapeDtypeStruct((S, D), BF16),
        in_specs=[hbm] * 10,
        out_specs=hbm,
        scratch_shapes=[
            pltpu.VMEM((S, D), BF16),
            pltpu.VMEM((S, D), BF16),
            pltpu.VMEM((S, D), BF16),
            pltpu.VMEM((D, S), BF16),
            pltpu.VMEM((D, 3 * D), BF16),
            pltpu.VMEM((D, D), BF16),
            pltpu.VMEM((KS, D), BF16),
            pltpu.VMEM((D,), BF16),
            pltpu.VMEM((D,), BF16),
            pltpu.VMEM(_DFT.shape, BF16),
            pltpu.VMEM((LT, D, 128), F32),
            pltpu.VMEM((13, 64, 128), U32),
            pltpu.VMEM((2, BLK // 2, D), U32),
            pltpu.VMEM((LT, S, 128), F32),
            pltpu.VMEM((LT, HALO + S, 128), F32),
            pltpu.VMEM((LT, HALO + S, 128), F32),
            pltpu.VMEM((LT, 8 + S, 128), F32),
            pltpu.VMEM((BLK * WIN, 128), F32),
            pltpu.VMEM((BLK // 2, D), U32),
            pltpu.VMEM((BLK // 2, D), U32),
            pltpu.VMEM((LT, S, 128), F32),
            pltpu.VMEM((NB, LT, 4, 128, 128), F32),
            pltpu.VMEM((NB, LT, 4, 128, 128), F32),
            pltpu.VMEM((S, D), BF16),
            pltpu.SemaphoreType.DMA((3,)),
            pltpu.SemaphoreType.DMA((NB,)),
            pltpu.SemaphoreType.DMA((NB,)),
            pltpu.SemaphoreType.DMA((NB,)),
            pltpu.SemaphoreType.DMA((NB,)),
            pltpu.SemaphoreType.DMA((1,)),
            pltpu.SemaphoreType.DMA((NB,)),
            pltpu.SemaphoreType.DMA((4,)),
            pltpu.SemaphoreType.DMA((LT,)),
        ],
        compiler_params=pltpu.CompilerParams(vmem_limit_bytes=100 * 2**20),
    )(A_q.reshape(S, D), A_k.reshape(S, D), A_v.reshape(S, D), A_ssm_k, B_wqkv, B_wo,
      A_shift_k.T, A_ssm_D, gate_w, jnp.asarray(_DFT, BF16))
    return out.reshape(1, S, D)
```

```python
import functools

import numpy as np
import jax
import jax.numpy as jnp
import jax.experimental.pallas as pl
import jax.experimental.pallas.tpu as pltpu

S, D = 2048, 640
H, DH = 32, 20
WIN, DIL = 8, 2
KS = 4
LT = D // 128
BLK = 256
NB = S // BLK
SPAN_PROJECT = (0.0, 1.0)
SPAN_CONV = (0.0, 1.05)
SPAN_ATTEND = (0.05, 1.05)
SPAN_FINISH = (0.0, 1.0)
AHEAD = {7: (5, (3, 4)), 6: (4, (3,))}
HS = 64
PM = 128
HALO = 16
SQRT2 = float(np.sqrt(2.0))
F32, BF16, U32 = jnp.float32, jnp.bfloat16, jnp.uint32


def _dft_matrices():
    n = np.arange(128)[None, :]
    m = np.arange(64)[:, None]
    idx = np.arange(128)
    bins = idx.reshape(2, 8, 8).transpose(1, 0, 2).reshape(-1)
    slabs = idx.reshape(2, 4, 16).transpose(1, 0, 2).reshape(-1)
    filt, sig, inv = [], [], []
    for f in (4 * m, 4 * m + 2, 8 * m + 1, 8 * m + 3):
        ang = 2.0 * np.pi * ((f * n) % 512) / 512.0
        a = np.concatenate([np.cos(ang), -np.sin(ang)], axis=0)
        wgt = np.full((128, 1), 2.0 / 512.0)
        if not filt:
            a[64] = np.cos(np.pi * n[0])
            wgt[0] = wgt[64] = 1.0 / 512.0
        filt.append(a[bins])
        sig.append(a[bins][:, bins])
        inv.append((a * wgt)[bins].T[slabs])
    same_head = idx[:, None] % H == idx[None, :] % H
    return np.stack(filt + inv + [same_head] + sig).astype(np.float32)


_DFT = _dft_matrices().astype(BF16)


def _nt(a, b):
    return jax.lax.dot_general(a, b, (((1,), (1,)), ((), ())),
                               preferred_element_type=F32)


def _nn(a, b):
    return jnp.dot(a, b, preferred_element_type=F32)


def _unpack(x):
    return pltpu.bitcast(x, BF16)


def _interleave(*streams, spans=None):
    items = []
    for n, s in enumerate(streams):
        lo, hi = (spans or {}).get(n, (0.0, 1.0))
        total, done = sum(c for c, _ in s), 0.0
        for c, f in s:
            items.append((lo + (hi - lo) * (done + 0.5 * c) / total, f))
            done += c
    for _, f in sorted(items, key=lambda e: e[0]):
        f()


def _kernel(x_hbm, k_hbm, v_hbm, h_hbm, w_hbm, wo_hbm,
            shift_hbm, dvec_hbm, gate_hbm, dft_hbm,
            out_hbm,
            x_v, k_v, v_v, h_v, w_v, wo_v, shift_ref, dvec_ref, gate_ref, dft_ref,
            tmp_s, dft_s, xp_s, q_s, ka_s, va_s,
            kf_s, lg_s, o0_s, o1_s, gq_s, u_s, g_s, out_s,
            w_sem, x_sem, k_sem, v_sem, h_sem, wo_sem, out_sem, small_sem, wq_sem):
    part_fn = functools.partial

    def rows_copy(src, dst, sem, n):
        rows = pl.ds(n * BLK, BLK)
        return pltpu.make_async_copy(src.at[rows], dst.at[rows], sem.at[n])

    def cols_copy(src, dst, sem, n, size):
        cols = pl.ds(n * size, size)
        return pltpu.make_async_copy(src.at[:, cols], dst.at[:, cols], sem.at[n])

    cp_w = [None] + [cols_copy(w_hbm, w_v, w_sem, n, D) for n in (1, 2)]
    cp_wq = [pltpu.make_async_copy(w_hbm.at[pl.ds(n * 128, 128), pl.ds(0, D)],
                                   w_v.at[pl.ds(n * 128, 128), pl.ds(0, D)], wq_sem.at[n])
             for n in range(LT)]
    cp_x = [rows_copy(x_hbm, x_v, x_sem, n) for n in range(NB)]
    cp_k = [rows_copy(k_hbm, k_v, k_sem, n) for n in range(NB)]
    cp_v = [rows_copy(v_hbm, v_v, v_sem, n) for n in range(NB)]
    cp_h = [cols_copy(h_hbm, h_v, h_sem, n, BLK) for n in range(NB)]
    cp_wo = pltpu.make_async_copy(wo_hbm, wo_v, wo_sem.at[0])
    cp_out = [rows_copy(out_s, out_hbm, out_sem, n) for n in range(NB)]

    cp_small = [
        pltpu.make_async_copy(src, dst, small_sem.at[n])
        for n, (src, dst) in enumerate(((shift_hbm, shift_ref), (dvec_hbm, dvec_ref),
                                        (gate_hbm, gate_ref), (dft_hbm, dft_ref)))]

    for c in cp_wq:
        c.start()
    cp_x[0].start()
    cp_x[1].start()
    cp_w[1].start()

    o_s = (o0_s, o1_s)
    zeros = jnp.zeros((HALO, 128), F32)
    for t in range(LT):
        ka_s[t, 0:HALO, :] = zeros
        va_s[t, 0:HALO, :] = zeros
        kf_s[t, 0:8, :] = zeros[0:8]
    vec = {}

    def load_constants():
        for n in range(_DFT.shape[0]):
            dft_s[n] = pltpu.bitcast(dft_ref[n], U32)
        vec["shift"] = shift_ref[...].astype(F32)
        vec["gate"] = gate_ref[...].astype(F32).reshape(1, D)
        vec["skip"] = dvec_ref[...].astype(F32).reshape(1, D)

    qscale = float(DH ** -0.5 * np.log2(np.e))

    def lanes(t):
        return slice(t * 128, (t + 1) * 128)

    w_tiles, wo_tiles, spectra, carried = {}, {}, {}, {}

    def permute_w_items(p):
        def transpose(kt):
            for t in range(LT):
                blk = w_v[lanes(kt), lanes(p * LT + t)].astype(F32)
                tmp_s[kt, lanes(t), :] = blk.T

        def gather(t):
            tile = jnp.concatenate([
                jnp.concatenate([tmp_s[kt, pl.ds(d, H, stride=DH), :]
                                 for d in range(4 * t, 4 * t + 4)], axis=0)
                for kt in range(LT)], axis=1)
            if p == 0:
                tile = tile * qscale
            w_tiles[p, t] = tile.astype(BF16)

        return ([(2, part_fn(transpose, kt)) for kt in range(LT)]
                + [(1, part_fn(gather, t)) for t in range(LT)])

    def permute_wo_items():
        def ntile(t):
            tmp_s[t] = wo_v[:, lanes(t)].astype(F32)
            rows = [tmp_s[t, pl.ds(d, H, stride=DH), :] for d in range(DH)]
            wo_tiles[t] = jnp.concatenate(rows, axis=0).astype(BF16)

        return [(1, part_fn(ntile, t)) for t in range(LT)]

    def stage_x(i):
        xp_s[i % 2] = pltpu.bitcast(x_v[i * BLK:(i + 1) * BLK, :], U32)

    def project_items(i, parts=(0, 1, 2)):
        def tile(p, t, row):
            acc = _nt(_unpack(xp_s[i % 2, row // 2:(row + PM) // 2, :]), w_tiles[p, t])
            at = i * BLK + row
            if p == 0:
                q_s[t, at:at + PM, :] = acc
            else:
                (ka_s, va_s)[p - 1][t, HALO + at:HALO + at + PM, :] = acc

        return [(1, part_fn(tile, p, t, row)) for p in parts for t in range(LT)
                for row in range(0, BLK, PM)]

    def attend_items(i):
        rc, part = 16, 64
        keep, pending = {}, []

        def scores(row):
            sums = {}
            for sub in (0, 8):
                at = i * BLK + row + sub
                qs = [q_s[t, at:at + 8, :] for t in range(LT)]
                for w in range(WIN):
                    lo = at + HALO - DIL * w
                    a = qs[0] * ka_s[0, lo:lo + 8, :]
                    for t in range(1, LT):
                        a = a + qs[t] * ka_s[t, lo:lo + 8, :]
                    sums[sub, w] = a
            sums = [sums[sub, w] for sub in (0, 8) for w in range(WIN)]
            pending.extend(sums)
            if (row + rc) % HS == 0:
                lo = (row + rc - HS) * WIN
                lg_s[lo:lo + HS * WIN, :] = _nn(
                    jnp.concatenate(pending, axis=0).astype(BF16), _unpack(dft_s[8]))
                pending.clear()

        def gating(row):
            r0 = i * BLK + row
            xs = [x_v[r0:r0 + rc, lanes(t)].astype(F32) for t in range(LT)]
            z = xs[0] * vec["gate"][:, lanes(0)]
            for t in range(1, LT):
                z = z + xs[t] * vec["gate"][:, lanes(t)]
            th = 0.5 * jnp.tanh(0.5 * jnp.sum(z, axis=-1, keepdims=True))
            g = 0.5 + th
            for t in range(LT):
                gq_s[t, r0:r0 + rc, :] = xs[t] * g
            keep[row] = 0.5 - th

        def mix(row):
            r0 = i * BLK + row
            outs = []
            for sub in (0, 8):
                logits = []
                for w in range(WIN):
                    at = (row + sub + w) * WIN
                    a = lg_s[at:at + 8, :]
                    if r0 + sub < DIL * w:
                        pos = r0 + sub + jax.lax.broadcasted_iota(jnp.int32, (8, 128), 0)
                        a = jnp.where(pos >= DIL * w, a, -1e9)
                    logits.append(a)
                m = logits[0]
                for w in range(1, WIN):
                    m = jnp.maximum(m, logits[w])
                es = [jnp.exp2(a - m) for a in logits]
                den = es[0]
                for w in range(1, WIN):
                    den = den + es[w]
                inv = pl.reciprocal(den, approx=True)
                inv = inv * (2.0 - den * inv)
                norm = keep[row][sub:sub + 8] * inv
                for t in range(LT):
                    a = None
                    for w in range(WIN):
                        lo = r0 + sub + HALO - DIL * w
                        term = es[w] * va_s[t, lo:lo + 8, :]
                        a = term if a is None else a + term
                    outs.append(a * norm)
            for t in range(LT):
                both = jnp.concatenate([outs[t], outs[LT + t]], axis=0).astype(BF16)
                o_s[i % 2][row // 2:(row + rc) // 2, lanes(t)] = pltpu.bitcast(both, U32)

        items = []
        for row in range(0, BLK + part, rc):
            if row < BLK:
                items.append((75, part_fn(gating, row)))
                items.append((155, part_fn(scores, row)))
            if row >= part:
                items.append((215, part_fn(mix, row - part)))
        return items

    def signal_items(i):
        r0 = i * BLK

        def tile(t):
            kf_s[t, r0 + 8:r0 + 8 + BLK, :] = k_v[r0:r0 + BLK, lanes(t)].astype(F32)
            pieces = [[] for _ in range(4)]
            for r in range(8):
                xs = []
                for b in range(4):
                    at = r0 + 64 * b + 8 * r
                    ks = None
                    for j in range(KS):
                        term = kf_s[t, at + 8 - j:at + 16 - j, :] * vec["shift"][j:j + 1, lanes(t)]
                        ks = term if ks is None else ks + term
                    xs.append(ks * v_v[at:at + 8, lanes(t)].astype(F32))
                x0, x1, x2, x3 = xs
                t0, t1 = x0 - x2, x1 + x3
                w0, w1 = SQRT2 * x3, SQRT2 * x2
                res = ((x0 + x2, t1), (t0, x1 - x3),
                       (t0 - w0, t1 + w1), (t0 + w0, t1 - w1))
                for cl in range(4):
                    pieces[cl].extend(res[cl])
            for cl in range(4):
                rhs = jnp.concatenate(pieces[cl], axis=0).astype(BF16)
                u_s[i, t, cl] = _nn(_unpack(dft_s[9 + cl]), rhs)

        return [(450, part_fn(tile, t)) for t in range(LT)]

    def filter_items(a):
        def tile(t):
            lane = jax.lax.broadcasted_iota(jnp.int32, (16, 128), 1)
            sign = jnp.where(lane < 64, -1.0, 1.0).astype(F32)
            pieces = [[] for _ in range(4)]
            for r in range(8):
                rows = slice(t * 128 + 16 * r, t * 128 + 16 * (r + 1))
                lo, hi = (h_v[rows, lanes(2 * a + n)].astype(F32) for n in (0, 1))
                if a == 0:
                    elo, ehi, olo, ohi = lo, hi, lo, hi
                else:
                    plo, phi = (h_v[rows, lanes(2 * a - 2 + n)].astype(F32) for n in (0, 1))
                    elo, ehi, olo, ohi = lo + plo, hi + phi, lo - plo, hi - phi
                tt = olo + sign * ohi
                ww = (SQRT2 * sign) * pltpu.roll(ohi, 64, 1)
                for cl, res in enumerate((elo + ehi, elo - ehi, tt + ww, tt - ww)):
                    pieces[cl].append(res)
            for cl in range(4):
                spec = _nt(_unpack(dft_s[cl]), jnp.concatenate(pieces[cl], axis=0).astype(BF16))
                if a < 2:
                    row = jax.lax.broadcasted_iota(jnp.int32, (128, 128), 0)
                    real = (row & 8) == 0
                    if cl == 0:
                        real = real | (row == 8)
                    dd = vec["skip"][:, lanes(t)]
                    dd = dd if (a == 0 or cl < 2) else -dd
                    spec = spec + jnp.where(real, dd, 0.0)
                g_s[a, t, cl] = spec

        return [(300, part_fn(tile, t)) for t in range(LT)]

    def spectrum_items(m, lags, last=True):
        def group(t, cl):
            out = []
            for r in range(8):
                re, im = slice(16 * r, 16 * r + 8), slice(16 * r + 8, 16 * r + 16)
                yr, yi = carried.pop((m, t, cl, r), (None, None))
                for a in lags:
                    gr, gi = g_s[a, t, cl, re, :], g_s[a, t, cl, im, :]
                    ur, ui = u_s[m - a, t, cl, re, :], u_s[m - a, t, cl, im, :]
                    ga, gb = gi, gr
                    if cl == 0 and r == 0:
                        slot0 = jax.lax.broadcasted_iota(jnp.int32, (8, 128), 0) == 0
                        ga, gb = jnp.where(slot0, 0.0, gi), jnp.where(slot0, gi, gr)
                    pr = ur * gr - ui * ga
                    pi = ur * ga + ui * gb
                    yr = pr if yr is None else yr + pr
                    yi = pi if yi is None else yi + pi
                out += [yr, yi]
                if not last:
                    carried[m, t, cl, r] = (yr, yi)
            if last:
                spectra[m, t, cl] = jnp.concatenate(out, axis=0).astype(BF16)

        return [(64 * len(lags), part_fn(group, t, cl)) for t in range(LT) for cl in range(4)]

    def finish_items(m):
        def tile(t):
            rho = [_nn(_unpack(dft_s[4 + cl]), spectra[m, t, cl]) for cl in range(4)]
            for r0 in range(0, 4, PM // 64):
                lhs = jnp.concatenate(
                    [o_s[m % 2][32 * b + 8 * r:32 * b + 8 * (r + 1), :]
                     for r in range(r0, r0 + PM // 64) for b in range(4)], axis=0)
                bb = _nn(_unpack(lhs), wo_tiles[t])
                for r in range(r0, r0 + PM // 64):
                    (a0, a1), (b0, b1), (p0, p1), (n0, n1) = [
                        (z[32 * r:32 * r + 16], z[32 * r + 16:32 * (r + 1)]) for z in rho]
                    s0, s1, d0, d1 = p0 + n0, p1 + n1, p0 - n0, p1 - n1
                    ys = (a0 + b0 + s0, a1 + b1 + s1,
                          a0 - b0 - s0 + SQRT2 * d1, a1 - b1 + s1 - SQRT2 * d0)
                    for b in range(4):
                        lo = m * BLK + 64 * b + 16 * r
                        at = 64 * (r - r0) + 16 * b
                        res = gq_s[t, lo:lo + 16, :] * ys[b] + bb[at:at + 16]
                        out_s[lo:lo + 16, lanes(t)] = res.astype(BF16)

        return [(1, part_fn(tile, t)) for t in range(LT)]

    for i in range(NB + 2):
        streams, spans = [], {}
        if i == 0:
            first = [cp_k[0], cp_v[0], cp_h[0]] + cp_small
            for n, (_, permute) in enumerate(permute_w_items(0)):
                if n < LT:
                    cp_wq[n].wait()
                permute()
            cp_w[2].start()
            for n in (0, 1):
                cp_x[n].wait()
            for n in (0, 1):
                stage_x(n)
            _interleave(project_items(0, (0,)))
            cp_w[1].wait()
            for c in first:
                c.start()
            _interleave(project_items(1, (0,)), permute_w_items(1))
            cp_w[2].wait()
            for c in (cp_k[1], cp_v[1], cp_h[1], cp_wo):
                c.start()
            _interleave(project_items(0, (1,)), permute_w_items(2))
            for c in first:
                c.wait()
            load_constants()
            streams.append(project_items(0, (2,)))
        elif i < NB:
            for c in (cp_k, cp_v, cp_h) + ((cp_x,) if i > 1 else ()):
                c[i].wait()
            if i + 1 < NB:
                for c in (cp_x, cp_k, cp_v, cp_h):
                    c[i + 1].start()
            if i > 1:
                stage_x(i)
            spans[len(streams)] = SPAN_PROJECT
            streams.append(project_items(i, (0, 1, 2) if i > 1 else (1, 2)))
        if i < NB:
            sig, fil, spec = signal_items(i), filter_items(i), spectrum_items(
                i, [a for a in range(i + 1) if a not in AHEAD.get(i, (0, ()))[1]])
            conv = []
            for t in range(LT + 1):
                if t < LT:
                    conv += [sig[t], fil[t]]
                if t > 0:
                    conv += spec[4 * (t - 1):4 * t]
            for m, (step, lags) in AHEAD.items():
                if step == i:
                    streams.append(spectrum_items(m, lags, last=False))
            spans[len(streams)] = SPAN_CONV
            streams.append(conv)
        if i == 2:
            cp_wo.wait()
            _interleave(permute_wo_items())
        if 1 <= i <= NB:
            spans[len(streams)] = SPAN_ATTEND
            streams.append(attend_items(i - 1))
        if i >= 2:
            spans[len(streams)] = SPAN_FINISH
            streams.append(finish_items(i - 2))
        _interleave(*streams, spans=spans)
        if i >= 2:
            cp_out[i - 2].start()
    for c in cp_out:
        c.wait()


@jax.jit
def pallas_gated_mix__ssm_conv_h3__sliding_local_dilated__prompt_kernel(
    A_q: jax.Array,
    A_k: jax.Array,
    A_v: jax.Array,
    A_shift_k: jax.Array,
    A_ssm_k: jax.Array,
    A_ssm_D: jax.Array,
    B_x: jax.Array,
    B_wqkv: jax.Array,
    B_wo: jax.Array,
    gate_w: jax.Array,
):
    del B_x
    hbm = pl.BlockSpec(memory_space=pl.ANY)
    out = pl.pallas_call(
        _kernel,
        out_shape=jax.ShapeDtypeStruct((S, D), BF16),
        in_specs=[hbm] * 10,
        out_specs=hbm,
        scratch_shapes=[
            pltpu.VMEM((S, D), BF16),
            pltpu.VMEM((S, D), BF16),
            pltpu.VMEM((S, D), BF16),
            pltpu.VMEM((D, S), BF16),
            pltpu.VMEM((D, 3 * D), BF16),
            pltpu.VMEM((D, D), BF16),
            pltpu.VMEM((KS, D), BF16),
            pltpu.VMEM((D,), BF16),
            pltpu.VMEM((D,), BF16),
            pltpu.VMEM(_DFT.shape, BF16),
            pltpu.VMEM((LT, D, 128), F32),
            pltpu.VMEM((13, 64, 128), U32),
            pltpu.VMEM((2, BLK // 2, D), U32),
            pltpu.VMEM((LT, S, 128), F32),
            pltpu.VMEM((LT, HALO + S, 128), F32),
            pltpu.VMEM((LT, HALO + S, 128), F32),
            pltpu.VMEM((LT, 8 + S, 128), F32),
            pltpu.VMEM((BLK * WIN, 128), F32),
            pltpu.VMEM((BLK // 2, D), U32),
            pltpu.VMEM((BLK // 2, D), U32),
            pltpu.VMEM((LT, S, 128), F32),
            pltpu.VMEM((NB, LT, 4, 128, 128), F32),
            pltpu.VMEM((NB, LT, 4, 128, 128), F32),
            pltpu.VMEM((S, D), BF16),
            pltpu.SemaphoreType.DMA((3,)),
            pltpu.SemaphoreType.DMA((NB,)),
            pltpu.SemaphoreType.DMA((NB,)),
            pltpu.SemaphoreType.DMA((NB,)),
            pltpu.SemaphoreType.DMA((NB,)),
            pltpu.SemaphoreType.DMA((1,)),
            pltpu.SemaphoreType.DMA((NB,)),
            pltpu.SemaphoreType.DMA((4,)),
            pltpu.SemaphoreType.DMA((LT,)),
        ],
        compiler_params=pltpu.CompilerParams(vmem_limit_bytes=100 * 2**20),
    )(A_q.reshape(S, D), A_k.reshape(S, D), A_v.reshape(S, D), A_ssm_k, B_wqkv, B_wo,
      A_shift_k.T, A_ssm_D, gate_w, _DFT)
    return out.reshape(1, S, D)
```
